```python
import jax
import jax.numpy as jnp

def _softmax(x, axis=-1):
    return jax.nn.softmax(x, axis=axis)
def _gelu(x):
    return jax.nn.gelu(x, approximate=True)
def _silu(x):
    return jax.nn.silu(x)
def _sigmoid(x):
    return jax.nn.sigmoid(x)
def _layernorm(x, axis=-1, eps=1e-5):
    m = jnp.mean(x, axis=axis, keepdims=True)
    v = jnp.var(x, axis=axis, keepdims=True)
    return (x - m) / jnp.sqrt(v + eps)
def _scatter_add(tgt, idx, src, axis=0):
    return tgt.at[idx].add(src)
def _segment_sum(src, seg, n):
    return jax.ops.segment_sum(src, seg, n)
class _Rng:
    def __init__(self, key):
        self._k = key
    def _next(self):
        self._k, sub = jax.random.split(self._k)
        return sub
    def normal(self, shape):
        return jax.random.normal(self._next(), shape, dtype=jnp.bfloat16)
    def randint(self, lo, hi, shape):
        return jax.random.randint(self._next(), shape, lo, hi, dtype=jnp.int32)
    def uniform(self, shape, lo=0.0, hi=1.0):
        return jax.random.uniform(self._next(), shape, jnp.bfloat16, lo, hi)
    def permutation(self, n):
        return jax.random.permutation(self._next(), n)


kernel_name = 'recurrent_scan__linear_kernel_hedgehog__moe_arch_mod__prompt'

def setup_inputs():
    _rng = _Rng(jax.random.key(int.from_bytes(__import__("os").urandom(4), "little")))
    _w = (lambda a: (lambda t: t.astype(jnp.bfloat16) if jnp.issubdtype(t.dtype, jnp.floating) else t)(jnp.asarray(a)))
    def _A_setup():
        B, S, D, H = 1, 2048, 1024, 32
        Dh = D // H
        return {
            "x": _w((lambda *s: _rng.normal(s) * 0.05)(B, S, D)),
            "wqkv": _w((lambda *s: _rng.normal(s) * 0.05)(D, 3 * D)),
            "w_phi": _w((lambda *s: _rng.normal(s) * 0.05)(H, Dh, Dh) * (Dh ** -0.5)),
            "wo": _w((lambda *s: _rng.normal(s) * 0.05)(D, D)),
        }
    _A_in = _A_setup()

    def _B_setup():
        B, S, D, F, C = 1, 2048, 1024, 3584, 1
        return {
            "x": _w((lambda *s: _rng.normal(s) * 0.05)(B, S, D)),
            "w_r": _w((lambda *s: _rng.normal(s) * 0.05)(D)),
            "w_gate": _w((lambda *s: _rng.normal(s) * 0.05)(D, F)),
            "w_up": _w((lambda *s: _rng.normal(s) * 0.05)(D, F)),
            "w_down": _w((lambda *s: _rng.normal(s) * 0.05)(F, D)),
        }
    _B_in = _B_setup()

    return {
        "A_x": _A_in["x"],
        "A_wqkv": _A_in["wqkv"],
        "A_w_phi": _A_in["w_phi"],
        "A_wo": _A_in["wo"],
        "B_x": _B_in["x"],
        "B_w_r": _B_in["w_r"],
        "B_w_gate": _B_in["w_gate"],
        "B_w_up": _B_in["w_up"],
        "B_w_down": _B_in["w_down"],
    }

def reference(A_x, A_wqkv, A_w_phi, A_wo, B_x, B_w_r, B_w_gate, B_w_up, B_w_down):
    def _A_ref(x, wqkv, w_phi, wo):
        B, S, D = x.shape
        H = 32; Dh = D // H
        qkv = (lambda x, *d: x.transpose(*d))((x @ wqkv).reshape(B, S, 3, H, Dh), 2, 0, 3, 1, 4)
        q, k, v = qkv[0], qkv[1], qkv[2]
        pq = jnp.einsum("bhsd,hdf->bhsf", q, w_phi)
        pk = jnp.einsum("bhsd,hdf->bhsf", k, w_phi)
        phi_q = jnp.concatenate([_softmax(pq, axis=-1), _softmax(-pq, axis=-1)], axis=-1)
        phi_k = jnp.concatenate([_softmax(pk, axis=-1), _softmax(-pk, axis=-1)], axis=-1)
        kv = jnp.einsum("bhsf,bhsd->bhfd", phi_k, v)
        z  = jnp.einsum("bhsf->bhf", phi_k)
        num = jnp.einsum("bhqf,bhfd->bhqd", phi_q, kv)
        den = jnp.einsum("bhqf,bhf->bhq", phi_q, z)[..., None] + 1e-6
        o = num / den
        return (lambda x, *d: x.transpose(*d))(o, 0, 2, 1, 3).reshape(B, S, D) @ wo

    def _B_ref(x, w_r, w_gate, w_up, w_down):
        B, S, D = x.shape
        C = 1
        r = x @ w_r
        idx = jnp.argsort(-r, axis=-1)[:, :C]
        idx_e = jnp.repeat(idx.reshape(B, C, 1), D, axis=2)
        x_sel = jnp.take_along_axis(x, idx_e, axis=1)
        g = _silu(x_sel @ w_gate)
        u = x_sel @ w_up
        y = (g * u) @ w_down
        r_sel = _sigmoid(jnp.take_along_axis(r, idx, axis=1))
        y = y * r_sel.reshape(B, C, 1)
        b_off = (jnp.arange(B) * S).reshape(B, 1)
        flat_idx = (idx + b_off).reshape(B * C)
        zero = (x * 0.0).reshape(B * S, D)
        upd = _scatter_add(zero, flat_idx, y.reshape(B * C, D), axis=0)
        return x + upd.reshape(B, S, D)

    x = A_x
    xn = _layernorm(x, axis=-1)
    s = _A_ref(xn, A_wqkv, A_w_phi, A_wo)
    g = _silu(_B_ref(xn, B_w_r, B_w_gate, B_w_up, B_w_down))
    return x + s * g
```

```python
import functools
import math

import jax
import jax.numpy as jnp
import numpy as np
from jax import lax
import jax.experimental.pallas as pl
import jax.experimental.pallas.tpu as pltpu

bf16, f32, u32, i32 = jnp.bfloat16, jnp.float32, jnp.uint32, jnp.int32
LOG2E = 1.4426950408889634
NT_DIMS = (((1,), (1,)), ((), ()))
TN_DIMS = (((0,), (0,)), ((), ()))


def _dot(a, b):
    return jnp.dot(a, b, preferred_element_type=f32)


def _dot_nt(a, b):
    return lax.dot_general(a, b, NT_DIMS, preferred_element_type=f32)


def _dot_tn(a, b):
    return lax.dot_general(a, b, TN_DIMS, preferred_element_type=f32)


def _pack(x):
    return pltpu.bitcast(x, u32)


def _unpack(x):
    return pltpu.bitcast(x, bf16)


def _rb(x):
    return x.astype(bf16).astype(f32)


def _head_reduce(v, op):
    v = op(v, pltpu.roll(v, 4, 0))
    return op(v, pltpu.roll(v, 2, 0))


def _dual_softmax(p):
    t = p.shape[1]
    p3 = p.reshape(8, 8, t)
    mx = _head_reduce(jnp.max(p3, axis=0), jnp.maximum)
    mn = _head_reduce(jnp.min(p3, axis=0), jnp.minimum)
    ep = jnp.exp2(p3 - mx[None])
    en = jnp.exp2(mn[None] - p3)
    sp = _head_reduce(jnp.sum(ep, axis=0), jnp.add)
    sn = _head_reduce(jnp.sum(en, axis=0), jnp.add)
    ep = ep * (1.0 / sp)[None]
    en = en * (1.0 / sn)[None]
    return ep, en


def make_kernel(S=2048, D=1024, H=32, F=3584, T=512, lag=1):
    Dh = D // H
    NT = S // T
    NG = D // 128
    NP = D // 64
    FC = F // NT
    TL = T // 128

    def kernel(x_hbm, wqkv_hbm, wphi_hbm, wo_hbm, wr_hbm, wg_hbm, wu_hbm, wd_hbm, out_hbm,
               x_v, wqkv_v, wphi_v, wo_v, wr_v, wg_v, wu_v, wd_v, out_v,
               xn_v, stage_v, wkvT_v, wqT_v, pT_v, kv_v, z_v, kvT_v, zb_v, r_v, oT_v,
               xb_v, y_v, sem_x, sem_w, sem_m, sem_f, sem_o):

        def x_copy(i):
            return pltpu.make_async_copy(x_hbm.at[pl.ds(i * T, T), :], x_v.at[pl.ds(i * T, T), :], sem_x.at[i])

        def w_copy(j):
            return pltpu.make_async_copy(wqkv_hbm.at[:, pl.ds(j * D, D)], wqkv_v.at[:, pl.ds(j * D, D)], sem_w.at[j])

        phi_copy = pltpu.make_async_copy(wphi_hbm, wphi_v, sem_m.at[0])
        wr_copy = pltpu.make_async_copy(wr_hbm, wr_v, sem_m.at[1])
        wo_copy = pltpu.make_async_copy(wo_hbm, wo_v, sem_m.at[2])
        f_copies = [pltpu.make_async_copy(s, d, sem_f.at[j])
                    for j, (s, d) in enumerate(((wg_hbm, wg_v), (wu_hbm, wu_v), (wd_hbm, wd_v)))]

        def o_copy(t):
            return pltpu.make_async_copy(out_v.at[pl.ds(t * T, T), :], out_hbm.at[pl.ds(t * T, T), :], sem_o.at[0])

        phi_copy.start()
        wr_copy.start()
        w_copy(1).start()
        x_copy(0).start()
        w_copy(2).start()
        for i in range(1, NT):
            x_copy(i).start()
        w_copy(0).start()
        wo_copy.start()

        phi_copy.wait()
        er = lax.broadcasted_iota(i32, (128, Dh), 0)
        ec = lax.broadcasted_iota(i32, (128, Dh), 1)
        eT = jnp.where((er % 64) // 2 == ec, 1.0, 0.0).astype(bf16)
        pT = _dot_nt(eT, wphi_v[...])
        rr = lax.broadcasted_iota(i32, (128, D), 0)
        cc = lax.broadcasted_iota(i32, (128, D), 1)
        head_r = (rr // 64) * 2 + rr % 2
        head_c = (cc % 128) // 32
        pT_v[...] = jnp.where(head_r == head_c, pT, 0.0).astype(bf16)

        def fold(g, j):
            w = wqkv_v[:, j * D + g * 128: j * D + (g + 1) * 128]
            return (_dot_nt(pT_v[:, g * 128:(g + 1) * 128], w) * LOG2E).astype(bf16)

        w_copy(1).wait()
        for g in range(NG):
            wkvT_v[g * 128: g * 128 + 64, :] = _pack(fold(g, 1))
        kv_v[...] = jnp.zeros(kv_v.shape, f32)
        z_v[...] = jnp.zeros(z_v.shape, f32)
        y_v[...] = jnp.zeros(y_v.shape, f32)

        wr_copy.wait()

        def layernorm(i):
            wr = wr_v[...].astype(f32).reshape(1, D)
            x = x_v[pl.ds(pl.multiple_of(i * T, T), T), :].astype(f32)
            m32 = jnp.sum(x, axis=1, keepdims=True) * (1.0 / D)
            c = x - m32
            v32 = jnp.sum(c * c, axis=1, keepdims=True) * (1.0 / D)
            sd = _rb(jnp.sqrt(_rb(_rb(v32) + float(np.asarray(1e-5, dtype=bf16)))))
            xn = (_rb(x - _rb(m32)) * (1.0 / sd)).astype(bf16)
            r = _rb(jnp.sum(xn.astype(f32) * wr, axis=1, keepdims=True))
            r_v[pl.ds(pl.multiple_of(i * T, T), T), :] = jnp.broadcast_to(r, (T, 128))
            return xn

        x_copy(0).wait()
        xn_v[0:T // 2, :] = _pack(layernorm(0))

        w_copy(2).wait()
        for g in range(NG):
            wkvT_v[g * 128 + 64:(g + 1) * 128, :] = _pack(wqkv_v[:, 2 * D + g * 128: 2 * D + (g + 1) * 128].T)

        for i in range(1, NT):
            x_copy(i).wait()
        for c in f_copies:
            c.start()

        def phase1(i, carry):
            row = pl.multiple_of(i * (T // 2), T // 2)
            nxt = jnp.minimum(i + 1, NT - 1)
            stage_v[...] = _pack(layernorm(nxt))

            def proj(g):
                return _dot_nt(_unpack(wkvT_v[g * 128:(g + 1) * 128, :]), _unpack(xn_v[pl.ds(row, T // 2), :]))

            def feats(g, pv):
                res = []
                for a in range(2):
                    pr = 2 * g + a
                    ep, en = _dual_softmax(pv[a * 64:(a + 1) * 64])
                    phi = jnp.concatenate([ep.reshape(64, T), en.reshape(64, T)], axis=0)
                    zs = phi[:, 0:128]
                    for l in range(1, TL):
                        zs = zs + phi[:, l * 128:(l + 1) * 128]
                    z_v[pr] += zs
                    res.append((pr, pv[128 + a * 64:128 + (a + 1) * 64].astype(bf16), phi.astype(bf16)))
                return res

            def accum(res):
                for pr, vT, phi in res:
                    kv_v[pr] += _dot_nt(vT, phi)

            pend = []
            for g in range(NG):
                pv = proj(g)
                pend.append(feats(g, pv))
                if len(pend) > lag:
                    accum(pend.pop(0))
            xn_v[pl.ds(pl.multiple_of(nxt * (T // 2), T // 2), T // 2), :] = stage_v[...]
            for res in pend:
                accum(res)
            return carry

        lax.fori_loop(0, NT, phase1, 0)

        w_copy(0).wait()
        for g in range(NG):
            wqT_v[g * 64:(g + 1) * 64, :] = _pack(fold(g, 0))

        kr = lax.broadcasted_iota(i32, (64, 128), 0)
        kc = lax.broadcasted_iota(i32, (64, 128), 1)
        same = (kr // 32) == (kc % 2)
        for pr in range(NP):
            kvT_v[pr] = _pack(jnp.where(same, kv_v[pr], 0.0).astype(bf16))
            zb_v[pr] = jnp.broadcast_to(jnp.sum(z_v[pr], axis=1, keepdims=True), (128, 128))

        r = r_v[...]
        r = jnp.where(r != r, -jnp.inf, r)
        rmax = jnp.max(r)
        io = lax.broadcasted_iota(i32, r.shape, 0)
        idx = jnp.clip(jnp.min(jnp.where(r == rmax, io, S)), 0, S - 1)
        t_sel = idx // T
        wrd = jnp.broadcast_to(xn_v[pl.ds(idx // 2, 1), :], (128, D))
        bits = jnp.where(idx % 2 == 1, wrd & jnp.uint32(0xFFFF0000), wrd << 16)
        xb_v[...] = pltpu.bitcast(bits, f32).T
        r_sel = r_v[pl.ds(idx, 1), :][:, 0:1]
        gate = 1.0 / (1.0 + jnp.exp(-r_sel))

        wo_copy.wait()
        for c in f_copies:
            c.wait()

        def ffn_chunk(c):
            col = pl.multiple_of(c * FC, 128)
            nb = FC // 128
            ag = jnp.zeros((8, FC), f32)
            au = jnp.zeros((8, FC), f32)
            for k in range(0, D, 16):
                xb = jnp.tile(xb_v[k:k + 16, :], (1, nb))
                pg = wg_v[k:k + 16, pl.ds(col, FC)].astype(f32) * xb
                pu = wu_v[k:k + 16, pl.ds(col, FC)].astype(f32) * xb
                ag = ag + (pg[0:8] + pg[8:16])
                au = au + (pu[0:8] + pu[8:16])
            gt = _rb(jnp.sum(ag, axis=0, keepdims=True))
            up = _rb(jnp.sum(au, axis=0, keepdims=True))
            h = _rb(_rb(gt / (1.0 + jnp.exp(-gt))) * up)
            hb = jnp.broadcast_to(h, (128, FC)).T
            ay = y_v[...]
            for k in range(0, FC, 16):
                pd = wd_v[pl.ds(col + k, 16), :].astype(f32) * jnp.tile(hb[k:k + 16], (1, D // 128))
                ay = ay + (pd[0:8] + pd[8:16])
            y_v[...] = ay

        def q_proj(t, g):
            row = pl.multiple_of(t * (T // 2), T // 2)
            return _dot_nt(_unpack(wqT_v[g * 64:(g + 1) * 64, :]), _unpack(xn_v[pl.ds(row, T // 2), :]))

        def q_feats(g, pq):
            res = []
            for a in range(2):
                pr = 2 * g + a
                ep, en = _dual_softmax(pq[a * 64:(a + 1) * 64])
                zb = jnp.tile(zb_v[pr], (1, TL))
                den = jnp.sum(ep * zb[0:64].reshape(8, 8, T) + en * zb[64:128].reshape(8, 8, T), axis=0)
                inv = 1.0 / (_head_reduce(den, jnp.add) + 1e-6)
                phi = jnp.concatenate([ep.reshape(64, T), en.reshape(64, T)], axis=0).astype(bf16)
                res.append((pr, phi, inv))
            return res

        def q_out(res, slot):
            for pr, phi, inv in res:
                num = _dot(_unpack(kvT_v[pr]), phi)
                sc = jnp.concatenate([jnp.broadcast_to(inv[0:1], (32, T)), jnp.broadcast_to(inv[1:2], (32, T))], axis=0)
                oT_v[slot, pr * 32:(pr + 1) * 32, :] = _pack((num * sc).astype(bf16))

        def out_chunk(t, slot, n0, n1, sel=None):
            s = _dot_tn(_unpack(oT_v[slot]), wo_v[:, n0:n1])
            gin = _unpack(xn_v[pl.ds(pl.multiple_of(t * (T // 2), T // 2), T // 2), n0:n1]).astype(f32)
            if sel is not None:
                rows, upd = sel
                gin = jnp.where(rows, _rb(gin + upd[:, n0:n1]), gin)
            gl = gin / (1.0 + jnp.exp(-gin))
            row = pl.multiple_of(t * T, T)
            out_v[pl.ds(row, T), n0:n1] = (x_v[pl.ds(row, T), n0:n1].astype(f32) + s * gl).astype(bf16)

        def tile_of(i):
            return lax.rem(t_sel + 1 + i, NT)

        def q_pass(t, slot, between=None):
            pend = []
            for g in range(NG):
                pq = q_proj(t, g)
                pend.append(q_feats(g, pq))
                if between is not None:
                    between(g)
                if len(pend) > lag:
                    q_out(pend.pop(0), slot)
            for res in pend:
                q_out(res, slot)

        NC = 256

        q_pass(tile_of(0), 0)
        ffn_chunk(0)

        def phase2(i, carry):
            tp = tile_of(i - 1)
            oT_v[1] = oT_v[0]

            def between(g):
                if g % 2 == 1:
                    out_chunk(tp, 1, (g // 2) * NC, (g // 2 + 1) * NC)

            q_pass(tile_of(i), 0, between)
            ffn_chunk(i)
            o_copy(tp).start()
            return carry

        lax.fori_loop(1, NT, phase2, 0)

        upd = _rb(_rb(jnp.sum(y_v[...], axis=0, keepdims=True)) * _rb(gate))
        rows = lax.broadcasted_iota(i32, (T, NC), 0) == idx - t_sel * T
        for n in range(D // NC):
            out_chunk(t_sel, 0, n * NC, (n + 1) * NC, (rows, upd))
        o_copy(t_sel).start()
        for i in range(NT):
            o_copy(i).wait()

    scratch = [
        pltpu.VMEM((S, D), bf16),
        pltpu.VMEM((D, 3 * D), bf16),
        pltpu.VMEM((D, Dh), bf16),
        pltpu.VMEM((D, D), bf16),
        pltpu.VMEM((D,), bf16),
        pltpu.VMEM((D, F), bf16),
        pltpu.VMEM((D, F), bf16),
        pltpu.VMEM((F, D), bf16),
        pltpu.VMEM((S, D), bf16),
        pltpu.VMEM((S // 2, D), u32),
        pltpu.VMEM((T // 2, D), u32),
        pltpu.VMEM((D, D), u32),
        pltpu.VMEM((D // 2, D), u32),
        pltpu.VMEM((128, D), bf16),
        pltpu.VMEM((NP, 64, 128), f32),
        pltpu.VMEM((NP, 128, 128), f32),
        pltpu.VMEM((NP, 32, 128), u32),
        pltpu.VMEM((NP, 128, 128), f32),
        pltpu.VMEM((S, 128), f32),
        pltpu.VMEM((2, D // 2, T), u32),
        pltpu.VMEM((D, 128), f32),
        pltpu.VMEM((8, D), f32),
        pltpu.SemaphoreType.DMA((NT,)),
        pltpu.SemaphoreType.DMA((3,)),
        pltpu.SemaphoreType.DMA((3,)),
        pltpu.SemaphoreType.DMA((3,)),
        pltpu.SemaphoreType.DMA((1,)),
    ]
    return kernel, scratch


@jax.jit
def pallas_recurrent_scan__linear_kernel_hedgehog__moe_arch_mod__prompt_kernel(
    A_x: jax.Array,
    A_wqkv: jax.Array,
    A_w_phi: jax.Array,
    A_wo: jax.Array,
    B_x: jax.Array,
    B_w_r: jax.Array,
    B_w_gate: jax.Array,
    B_w_up: jax.Array,
    B_w_down: jax.Array,
):
    del B_x
    B, S, D = A_x.shape
    H, Dh, _ = A_w_phi.shape
    F = B_w_gate.shape[1]
    assert B == 1
    kernel, scratch = make_kernel(S=S, D=D, H=H, F=F)
    out = pl.pallas_call(
        kernel,
        out_shape=jax.ShapeDtypeStruct((S, D), A_x.dtype),
        in_specs=[pl.BlockSpec(memory_space=pl.ANY)] * 8,
        out_specs=pl.BlockSpec(memory_space=pl.ANY),
        scratch_shapes=scratch,
        compiler_params=pltpu.CompilerParams(vmem_limit_bytes=100 * 1024 * 1024),
        name="hedgehog_mod",
    )(A_x.reshape(S, D), A_wqkv, A_w_phi.reshape(H * Dh, Dh), A_wo, B_w_r, B_w_gate, B_w_up, B_w_down)
    return out.reshape(B, S, D)
```

```python
import contextlib

import jax
import jax.numpy as jnp
import numpy as np
from jax import lax
import jax.experimental.pallas as pl
import jax.experimental.pallas.tpu as pltpu

bf16, f32, u32, i32 = jnp.bfloat16, jnp.float32, jnp.uint32, jnp.int32
LOG2E = 1.4426950408889634
LN_EPS = float(np.asarray(1e-5, dtype=bf16))
NT_DIMS = (((1,), (1,)), ((), ()))


def _dot(a, b):
    return jnp.dot(a, b, preferred_element_type=f32)


def _dot_nt(a, b):
    return lax.dot_general(a, b, NT_DIMS, preferred_element_type=f32)


def _pack(x):
    return pltpu.bitcast(x, u32)


def _unpack(x):
    return pltpu.bitcast(x, bf16)


def _rb(x):
    return x.astype(bf16).astype(f32)


def _recip(x):
    return pltpu.reciprocal(x, approx=False, full_range=False)


def _silu(x):
    h = 0.5 * x
    return h * jnp.tanh(h) + h


def _zero_after(vals, slack):
    z = None
    for v in vals:
        b = pltpu.bitcast(v, u32)
        z = b if z is None else z | b
    z = (z >> 16) >> 16
    for _ in range(slack):
        z = pltpu.roll(z, 1, 1)
    return z


def _after(op, deps):
    deps = {k: v for k, v in deps.items() if v is not None}
    if not deps:
        return op
    rows, r0 = [], 0
    for r in sorted({r for r, _ in deps}):
        if r > r0:
            rows.append(op[r0:r])
        parts, c0 = [], 0
        for c in sorted(c for rr, c in deps if rr == r):
            if c > c0:
                parts.append(op[r:r + 8, c0:c])
            parts.append(op[r:r + 8, c:c + 128] | deps[(r, c)])
            c0 = c + 128
        if c0 < op.shape[1]:
            parts.append(op[r:r + 8, c0:])
        rows.append(parts[0] if len(parts) == 1 else jnp.concatenate(parts, axis=1))
        r0 = r + 8
    if r0 < op.shape[0]:
        rows.append(op[r0:])
    return jnp.concatenate(rows, axis=0)


def _head_reduce(v, op):
    v = op(v, pltpu.roll(v, 4, 0))
    return op(v, pltpu.roll(v, 2, 0))


def _dual_softmax(p):
    t = p.shape[1]
    p3 = p.reshape(8, 8, t)
    mx = _head_reduce(jnp.max(p3, axis=0), jnp.maximum)
    mn = _head_reduce(jnp.min(p3, axis=0), jnp.minimum)
    ep = jnp.exp2(p3 - mx[None])
    en = jnp.exp2(mn[None] - p3)
    sp = _head_reduce(jnp.sum(ep, axis=0), jnp.add)
    sn = _head_reduce(jnp.sum(en, axis=0), jnp.add)
    return ep * _recip(sp)[None], en * _recip(sn)[None]


def make_kernel(S=2048, D=1024, H=32, F=3584, T=512, lag=1, NC=256, NCL=128, olag=1, ffn_end=1, ln0=4,
                anchor1=False, anchor2=True, slack=0, UK=64, UC=2, UD=64, ffn_early=True, qfold_early=True,
                scopes=False):
    Dh = D // H
    NT = S // T
    NG = D // 128
    NP = D // 64
    TL = T // 128
    FP = 256
    NF = F // FP
    n_dma = 64

    def kernel(x_hbm, wqkv_hbm, wphi_hbm, wo_hbm, wr_hbm, wg_hbm, wu_hbm, wd_hbm, out_hbm,
               x_v, wqkv_v, wphi_v, wo_v, wr_v, wg_v, wu_v, wd_v, out_v,
               xn_v, wkvT_v, wqT_v, pT_v, kv_v, z_v, kvT_v, zb_v, r_v, o_v, xb_v, sem):

        def scope(name):
            return jax.named_scope(name) if scopes else contextlib.nullcontext()

        used = []

        def dma(src, dst):
            used.append(None)
            return pltpu.make_async_copy(src, dst, sem.at[len(used) - 1])

        def cols(ref, c, n):
            return ref.at[:, pl.ds(c, n)]

        def rows(ref, r, n):
            return ref.at[pl.ds(r, n), :]

        x0_copies = [dma(rows(x_hbm, j * 128, 128), rows(x_v, j * 128, 128)) for j in range(TL)]
        x_copies = {i: dma(rows(x_hbm, i * T, T), rows(x_v, i * T, T)) for i in range(1, NT)}
        wk_copies = [dma(cols(wqkv_hbm, D + g * 128, 128), cols(wqkv_v, D + g * 128, 128)) for g in range(NG)]
        wv_copies = [dma(cols(wqkv_hbm, 2 * D + g * 128, 128), cols(wqkv_v, 2 * D + g * 128, 128)) for g in range(NG)]
        wq_copy = dma(cols(wqkv_hbm, 0, D), cols(wqkv_v, 0, D))
        phi_copy, wr_copy, wo_copy = dma(wphi_hbm, wphi_v), dma(wr_hbm, wr_v), dma(wo_hbm, wo_v)
        wg_copy, wu_copy, wd_copy = dma(wg_hbm, wg_v), dma(wu_hbm, wu_v), dma(wd_hbm, wd_v)
        out_copies = []

        order = [wr_copy, x0_copies[0], phi_copy, x0_copies[1], wk_copies[0], x0_copies[2], wv_copies[0]]
        order += x0_copies[3:]
        for g in range(1, NG):
            order += [wk_copies[g], wv_copies[g]]
            if g == 5:
                order.append(x_copies[1])
        order += [x_copies[i] for i in range(2, NT)]
        order += [wg_copy, wu_copy, wq_copy, wo_copy, wd_copy]
        for c in order:
            c.start()

        def layernorm(row, n):
            wr = wr_v[...].astype(f32).reshape(1, D)
            x = x_v[row:row + n, :].astype(f32)
            m32 = jnp.sum(x, axis=1, keepdims=True) * (1.0 / D)
            c = x - m32
            v32 = jnp.sum(c * c, axis=1, keepdims=True) * (1.0 / D)
            sd = _rb(jnp.sqrt(_rb(_rb(v32) + LN_EPS)))
            xn = (_rb(x - _rb(m32)) * (1.0 / sd)).astype(bf16)
            r = jnp.broadcast_to(_rb(jnp.sum(xn.astype(f32) * wr, axis=1, keepdims=True)), (n, 128))
            r_v[row:row + n, :] = r
            xn_v[row // 2:(row + n) // 2, :] = _pack(xn)
            return r

        with scope("w_x0"):
            wr_copy.wait()
            x0_copies[0].wait()
        layernorm(0, 128)

        with scope("w_phi"):
            phi_copy.wait()
        er = lax.broadcasted_iota(i32, (128, Dh), 0)
        ec = lax.broadcasted_iota(i32, (128, Dh), 1)
        eT = jnp.where(((er & 63) >> 1) == ec, 1.0, 0.0).astype(bf16)
        pT = _dot_nt(eT, wphi_v[...])
        rr = lax.broadcasted_iota(i32, (128, 128), 0)
        cc = lax.broadcasted_iota(i32, (128, 128), 1)
        same_head = (rr >> 6) * 2 + (rr & 1) == (cc >> 5)
        for g in range(NG):
            pT_v[:, g * 128:(g + 1) * 128] = _pack(jnp.where(same_head, pT[:, g * 128:(g + 1) * 128], 0.0).astype(bf16))

        for j in range(1, TL):
            with scope("w_x0"):
                x0_copies[j].wait()
            layernorm(j * 128, 128)

        def fold(g, j):
            w = wqkv_v[:, j * D + g * 128: j * D + (g + 1) * 128]
            return _pack((_dot_nt(_unpack(pT_v[:, g * 128:(g + 1) * 128]), w) * LOG2E).astype(bf16))

        def prepare_kv(g):
            with scope("w_kv"):
                wk_copies[g].wait()
                wv_copies[g].wait()
            wkvT_v[g * 128: g * 128 + 64, :] = fold(g, 1)
            wkvT_v[g * 128 + 64:(g + 1) * 128, :] = _pack(wqkv_v[:, 2 * D + g * 128: 2 * D + (g + 1) * 128].T)

        sel = {}

        def route():
            r = r_v[...]
            r = jnp.where(r != r, -jnp.inf, r)
            rmax = jnp.max(r)
            io = lax.broadcasted_iota(i32, r.shape, 0)
            idx = jnp.clip(jnp.min(jnp.where(r == rmax, io, S)), 0, S - 1)
            wrd = jnp.broadcast_to(xn_v[pl.ds(idx // 2, 1), :], (128, D))
            bits = jnp.where(idx % 2 == 1, wrd & jnp.uint32(0xFFFF0000), wrd << 16)
            xb_v[...] = pltpu.bitcast(bits, f32).T
            r_sel = r_v[pl.ds(idx, 1), :][:, 0:1]
            sel.update(idx=idx, gate=_rb(1.0 / (1.0 + jnp.exp(-r_sel))), y=None)
            spare = pl.multiple_of(D + (idx % 2) * 8, 8)
            wkvT_v[pl.ds(spare, 8), 0:128] = jnp.zeros((8, 128), u32)

        def ffn_units():
            with scope("w_gu"):
                wg_copy.wait()
                wu_copy.wait()
            ag = [None] * NF
            au = [None] * NF
            for k0 in range(0, D, UK):
                xbs = [jnp.tile(xb_v[k:k + 8, :], (1, FP // 128)) for k in range(k0, k0 + UK, 8)]
                for c in range(NF):
                    col = c * FP
                    for j, xb in enumerate(xbs):
                        k = k0 + 8 * j
                        pg = wg_v[k:k + 8, col:col + FP].astype(f32) * xb
                        pu = wu_v[k:k + 8, col:col + FP].astype(f32) * xb
                        ag[c] = pg if ag[c] is None else ag[c] + pg
                        au[c] = pu if au[c] is None else au[c] + pu
                    if (c + 1) % UC == 0:
                        yield [v[:, l * 128:(l + 1) * 128] for cc in range(c + 1 - UC, c + 1)
                               for v in (ag[cc], au[cc]) for l in range(FP // 128)]
            with scope("w_d"):
                wd_copy.wait()
            for c in range(NF):
                col = c * FP
                gt = _rb(jnp.sum(ag[c], axis=0, keepdims=True))
                up = _rb(jnp.sum(au[c], axis=0, keepdims=True))
                h = _rb(_rb(_silu(gt)) * up)
                hb = jnp.broadcast_to(h, (128, FP)).T
                for k in range(0, FP, 8):
                    pd = wd_v[col + k:col + k + 8, :].astype(f32) * jnp.tile(hb[k:k + 8], (1, D // 128))
                    sel["y"] = pd if sel["y"] is None else sel["y"] + pd
                    if (k + 8) % UD == 0:
                        yield [sel["y"][:, l * 128:(l + 1) * 128] for l in range(D // 128)]

        NO = D // NC
        units = ffn_units()
        n_units = (D // UK) * (NF // UC) + F // UD
        n_slots = (NT * NG - ffn_end) * TL + (NO * (NT - 1) - 1) * 4 + (NG * 2 * TL if ffn_early else 0)
        count = {"slot": 0, "unit": 0}

        def next_dep():
            count["slot"] += 1
            vals = []
            while count["unit"] < n_units and count["unit"] * n_slots < count["slot"] * n_units:
                vals = next(units)
                count["unit"] += 1
            return _zero_after(vals, slack) if vals and anchor2 else None

        kr = lax.broadcasted_iota(i32, (64, 128), 0)
        kc = lax.broadcasted_iota(i32, (64, 128), 1)
        same = (kr >> 5) == (kc & 1)

        def k_feats(i, g, pv):
            res = []
            for a in range(2):
                pr = 2 * g + a
                ep, en = _dual_softmax(pv[a * 64:(a + 1) * 64])
                phi = jnp.concatenate([ep.reshape(64, T), en.reshape(64, T)], axis=0)
                zs = phi[:, 0:128]
                for l in range(1, TL):
                    zs = zs + phi[:, l * 128:(l + 1) * 128]
                if i > 0:
                    zs = zs + z_v[pr]
                if i < NT - 1:
                    z_v[pr] = zs
                else:
                    zb_v[pr] = jnp.broadcast_to(jnp.sum(zs, axis=1, keepdims=True), (128, 128))
                res.append((i, pr, pv[128 + a * 64:128 + (a + 1) * 64].astype(bf16), phi.astype(bf16)))
            return res

        def k_accum(res):
            for i, pr, vT, phi in res:
                kv = _dot_nt(vT, phi)
                if i > 0:
                    kv = kv + kv_v[pr]
                if i < NT - 1:
                    kv_v[pr] = kv
                else:
                    kvT_v[pr] = _pack(jnp.where(same, kv, 0.0).astype(bf16))

        pend = []

        def flush(keep):
            while len(pend) > keep:
                fn, args = pend.pop(0)
                fn(*args)

        ahead = {0: [1], 1: [2, 3], 2: [4, 5], 4: [6, 7]}
        prepare_kv(0)
        for i in range(NT):
            for g in range(NG):
                deps = {}
                if i + 1 < NT:
                    g0 = ln0 if i == 0 else 0
                    if g == g0:
                        with scope("w_x"):
                            x_copies[i + 1].wait()
                    n16 = T // 16
                    pieces = range((g - g0) * n16 // (NG - g0), (g + 1 - g0) * n16 // (NG - g0)) if g >= g0 else []
                    for j, p in enumerate(pieces):
                        r = layernorm((i + 1) * T + p * 16, 16)
                        slot = j * 2 * TL // len(pieces)
                        if anchor1:
                            deps[((slot // 2) * 64, (slot % 2) * (D // 2))] = _zero_after([r[0:8], r[8:16]], slack)
                elif ffn_early:
                    if g == 0:
                        route()
                    if g > 0:
                        deps = {((j // 2) * 64, (j % 2) * (D // 2)): next_dep() for j in range(2 * TL)}
                    else:
                        count["slot"] += 2 * TL
                xw = _after(xn_v[i * T // 2:(i + 1) * T // 2, :], deps)
                pv = _dot_nt(_unpack(wkvT_v[g * 128:(g + 1) * 128, :]), _unpack(xw))
                pend.append((k_accum, (k_feats(i, g, pv),)))
                if i == 0:
                    for gg in ahead.get(g, []):
                        prepare_kv(gg)
                if i == NT - 1 and qfold_early:
                    if g == 0:
                        with scope("w_q"):
                            wq_copy.wait()
                    wqT_v[g * 64:(g + 1) * 64, :] = fold(g, 0)
                flush(lag)

        if not ffn_early:
            route()
        if not qfold_early:
            wq_copy.wait()
            for g in range(NG):
                wqT_v[g * 64:(g + 1) * 64, :] = fold(g, 0)
        idx = sel["idx"]
        t_sel = idx // T
        with scope("w_o"):
            wo_copy.wait()

        tiles = [lax.rem(t_sel + 1 + i, NT) for i in range(NT - 1)] + [t_sel]

        def q_feats(g, pq):
            res = []
            for a in range(2):
                pr = 2 * g + a
                ep, en = _dual_softmax(pq[a * 64:(a + 1) * 64])
                zb = jnp.tile(zb_v[pr], (1, TL))
                den = jnp.sum(ep * zb[0:64].reshape(8, 8, T) + en * zb[64:128].reshape(8, 8, T), axis=0)
                inv = _recip(_head_reduce(den, jnp.add) + 1e-6)
                phi = jnp.concatenate([ep.reshape(64, T), en.reshape(64, T)], axis=0).astype(bf16)
                res.append((pr, phi, inv))
            return res

        def q_out(i, g, res):
            parts = []
            for pr, phi, inv in res:
                num = _dot(_unpack(kvT_v[pr]), phi)
                sc = jnp.concatenate([jnp.broadcast_to(inv[0:1], (32, T)), jnp.broadcast_to(inv[1:2], (32, T))], axis=0)
                parts.append((num * sc).astype(bf16))
            o_v[i % 2, :, g * 128:(g + 1) * 128] = _pack(jnp.concatenate(parts, axis=0).T)

        def out_chunk(i, n0, n1):
            t = tiles[i]
            last = i == NT - 1
            deps = {}
            if not last:
                deps = {((j % 2) * (T // 4), (j // 2) * (D // 2)): next_dep() for j in range(4)}
            s = _dot(_unpack(_after(o_v[i % 2], deps)), wo_v[:, n0:n1])
            gin = _unpack(xn_v[pl.ds(pl.multiple_of(t * (T // 2), T // 2), T // 2), n0:n1]).astype(f32)
            if last:
                upd = _rb(_rb(jnp.sum(sel["y"][:, n0:n1], axis=0, keepdims=True)) * sel["gate"])
                hit = lax.broadcasted_iota(i32, (T, n1 - n0), 0) == idx - t_sel * T
                gin = jnp.where(hit, gin + upd, gin)
            row = pl.multiple_of(t * T, T)
            out_v[pl.ds(row, T), n0:n1] = (x_v[pl.ds(row, T), n0:n1].astype(f32) + s * _silu(gin)).astype(bf16)
            if last or n1 == D:
                c0 = n0 if last else 0
                out_copies.append(dma(out_v.at[pl.ds(row, T), pl.ds(c0, n1 - c0)],
                                      out_hbm.at[pl.ds(row, T), pl.ds(c0, n1 - c0)]))
                out_copies[-1].start()

        per = NG // NO
        outs = [(i, n * NC, (n + 1) * NC) for i in range(NT - 1) for n in range(NO)]
        outs += [(NT - 1, n, n + NCL) for n in range(0, D, NCL)]
        oi = 0
        for i in range(NT):
            for g in range(NG):
                b = i * NG + g
                row = pl.multiple_of(tiles[i] * (T // 2), T // 2)
                deps = {(n * 64, 0): next_dep() for n in range(TL)}
                xw = _after(xn_v[pl.ds(row, T // 2), :], deps)
                pq = _dot_nt(_unpack(wqT_v[g * 64:(g + 1) * 64, :]), _unpack(xw))
                pend.append((q_out, (i, g, q_feats(g, pq))))
                if (b + 1) % per == 0 and (b + 1) // per > NO + olag - 1:
                    out_chunk(*outs[oi])
                    oi += 1
                flush(lag)
        flush(0)
        while oi < len(outs):
            out_chunk(*outs[oi])
            oi += 1
        assert count["unit"] == n_units and next(units, None) is None, count
        assert len(used) <= n_dma
        with scope("w_out"):
            for c in out_copies:
                c.wait()

    scratch = [
        pltpu.VMEM((S, D), bf16),
        pltpu.VMEM((D, 3 * D), bf16),
        pltpu.VMEM((D, Dh), bf16),
        pltpu.VMEM((D, D), bf16),
        pltpu.VMEM((D,), bf16),
        pltpu.VMEM((D, F), bf16),
        pltpu.VMEM((D, F), bf16),
        pltpu.VMEM((F, D), bf16),
        pltpu.VMEM((S, D), bf16),
        pltpu.VMEM((S // 2, D), u32),
        pltpu.VMEM((D + 16, D), u32),
        pltpu.VMEM((D // 2, D), u32),
        pltpu.VMEM((64, D), u32),
        pltpu.VMEM((NP, 64, 128), f32),
        pltpu.VMEM((NP, 128, 128), f32),
        pltpu.VMEM((NP, 32, 128), u32),
        pltpu.VMEM((NP, 128, 128), f32),
        pltpu.VMEM((S, 128), f32),
        pltpu.VMEM((2, T // 2, D), u32),
        pltpu.VMEM((D, 128), f32),
        pltpu.SemaphoreType.DMA((n_dma,)),
    ]
    return kernel, scratch


@jax.jit
def pallas_recurrent_scan__linear_kernel_hedgehog__moe_arch_mod__prompt_kernel(
    A_x: jax.Array,
    A_wqkv: jax.Array,
    A_w_phi: jax.Array,
    A_wo: jax.Array,
    B_x: jax.Array,
    B_w_r: jax.Array,
    B_w_gate: jax.Array,
    B_w_up: jax.Array,
    B_w_down: jax.Array,
):
    del B_x
    B, S, D = A_x.shape
    H, Dh, _ = A_w_phi.shape
    F = B_w_gate.shape[1]
    assert B == 1
    kernel, scratch = make_kernel(S=S, D=D, H=H, F=F)
    out = pl.pallas_call(
        kernel,
        out_shape=jax.ShapeDtypeStruct((S, D), A_x.dtype),
        in_specs=[pl.BlockSpec(memory_space=pl.ANY)] * 8,
        out_specs=pl.BlockSpec(memory_space=pl.ANY),
        scratch_shapes=scratch,
        compiler_params=pltpu.CompilerParams(
            vmem_limit_bytes=100 * 1024 * 1024,
            flags={"XLA_TPU_EVENLY_DISTRIBUTE_CRITICAL_NODES": True}),
        name="hedgehog_mod",
    )(A_x.reshape(S, D), A_wqkv, A_w_phi.reshape(H * Dh, Dh), A_wo, B_w_r, B_w_gate, B_w_up, B_w_down)
    return out.reshape(B, S, D)
```

```python
import contextlib

import jax
import jax.numpy as jnp
import numpy as np
from jax import lax
import jax.experimental.pallas as pl
import jax.experimental.pallas.tpu as pltpu

bf16, f32, u32, i32 = jnp.bfloat16, jnp.float32, jnp.uint32, jnp.int32
LOG2E = 1.4426950408889634
LN_EPS = float(np.asarray(1e-5, dtype=bf16))
NT_DIMS = (((1,), (1,)), ((), ()))


def _dot(a, b):
    return jnp.dot(a, b, preferred_element_type=f32)


def _dot_nt(a, b):
    return lax.dot_general(a, b, NT_DIMS, preferred_element_type=f32)


def _pack(x):
    return pltpu.bitcast(x.astype(bf16), u32)


def _unpack(x):
    return pltpu.bitcast(x, bf16)


def _rb(x):
    return x.astype(bf16).astype(f32)


def _recip(x):
    return pltpu.reciprocal(x, approx=False, full_range=False)


def _silu(x):
    h = 0.5 * x
    return h * jnp.tanh(h) + h


def _left_terms(a11, a12, a21, a22):
    return [a11 + a22, a21 + a22, a11, a22, a11 + a12, a21 - a11, a12 - a22]


def _right_terms(b11, b12, b21, b22):
    return [b11 + b22, b11, b12 - b22, b21 - b11, b22, b11 + b12, b21 + b22]


def _zero_after(vals):
    z = None
    for v in vals:
        b = pltpu.bitcast(v, u32)
        z = b if z is None else z | b
    return (z >> 16) >> 16


def _after(op, zeros, at):
    n = op.shape[0] // len(zeros)
    parts, done = [], 0
    for k, zero in enumerate(zeros):
        r = k * n + at * 8
        if zero is not None:
            parts += [op[done:r]] if r > done else []
            parts.append(op[r:r + 8] | jnp.tile(zero, (1, op.shape[1] // 128)))
            done = r + 8
    parts += [op[done:]] if done < op.shape[0] else []
    return parts[0] if len(parts) == 1 else jnp.concatenate(parts, axis=0)


class _Interleaver:
    def __init__(self, at):
        self.slot, self.at, self.budget, self.credit = 0, at, 0, 0
        self.work, self.matmuls, self.filler = [], [], None

    def add(self, cost, fn, *args, delay=0):
        self.work.append((self.slot + delay, cost, fn, args))

    def fill(self, gen):
        self.finish_filler()
        self.filler = gen

    def finish_filler(self):
        for _ in self.filler or ():
            pass
        self.filler = None

    def tick(self):
        self.slot += 1
        self.credit = min(self.credit, 0) + self.budget
        vals = []
        while self.credit > 0 and self.work and self.work[0][0] < self.slot:
            _, cost, fn, args = self.work.pop(0)
            vals += fn(*args)
            self.credit -= cost
        while self.credit > 0 and self.filler:
            unit = next(self.filler, None)
            if unit is None:
                self.filler = None
            else:
                self.credit -= unit[0]
                vals += unit[1]
        return _zero_after(vals) if vals else None

    def operand(self, op):
        return _unpack(_after(op, [self.tick() for _ in range(op.shape[0] // 64)], self.at))

    def issue(self):
        if self.matmuls:
            fn, args = self.matmuls.pop(0)
            fn(*args)

    def need(self, ref, row):
        last = [k for k, w in enumerate(self.work) if len(w[3]) > 2 and w[3][1] is ref and row <= w[3][2] < row + 64]
        for _ in range(last[-1] + 1 if last else 0):
            _, _, fn, args = self.work.pop(0)
            fn(*args)

    def force(self):
        if self.matmuls:
            self.issue()
        else:
            _, _, fn, args = self.work.pop(0)
            fn(*args)

    def drain(self):
        while self.work or self.matmuls:
            while self.work:
                _, _, fn, args = self.work.pop(0)
                fn(*args)
            while self.matmuls:
                self.issue()


def _head_reduce(v, op):
    v = op(v, pltpu.roll(v, 4, 0))
    return op(v, pltpu.roll(v, 2, 0))


def _dual_softmax(p):
    t = p.shape[1]
    p3 = p.reshape(8, 8, t)
    mx = _head_reduce(jnp.max(p3, axis=0), jnp.maximum)
    mn = _head_reduce(jnp.min(p3, axis=0), jnp.minimum)
    ep = jnp.exp2(p3 - mx[None])
    en = jnp.exp2(mn[None] - p3)
    sp = _head_reduce(jnp.sum(ep, axis=0), jnp.add)
    sn = _head_reduce(jnp.sum(en, axis=0), jnp.add)
    return ep * _recip(sp)[None], en * _recip(sn)[None]


def make_kernel(S=2048, D=1024, H=32, F=3584, T=512, olag=2, delay=3, WR=16, at=6, RR=128, UK=32, UD=16,
                b_first=600, b_tile0=230, b_ln=130, b_ffn=160, b_alone=190, b_both=215, late_at=3, strict=False, verbose=False,
                o_groups=((0, 1), (2, 3, 4), (5, 6)), scopes=False):
    Dh = D // H
    NT = S // T
    NG = D // 128
    NP = D // 64
    NB = NG // 2
    TH, DH = T // 2, D // 2
    FP = 256
    NF = F // FP
    n_dma = 64
    F1 = 5 * FP
    ahead = {0: (2, [1]), 1: (3, [2, 3]), 3: (4, [4, 5]), 5: (5, [6, 7])}

    def kernel(x_hbm, wqkv_hbm, wphi_hbm, wo_hbm, wr_hbm, wg_hbm, wu_hbm, wd_hbm, out_hbm,
               x_v, wqkv_v, wphi_v, wo_v, wr_v, wg_v, wu_v, wd_v, out_v,
               xn_v, xs_v, wkv_v, wq_v, wos_v, pT_v, kv_v, z_v, kvT_v, zb_v, r_v, o_v, xb_v, sem):

        def scope(name):
            return jax.named_scope(name) if scopes else contextlib.nullcontext()

        used = []

        def dma(src, dst):
            used.append(None)
            return pltpu.make_async_copy(src, dst, sem.at[len(used) - 1])

        def cols(ref, c, n):
            return ref.at[:, pl.ds(c, n)]

        def rows(ref, r, n):
            return ref.at[pl.ds(r, n), :]

        def x_copy(r, n):
            return dma(rows(x_hbm, r, n), rows(x_v, r, n))

        def kv_copies(gs):
            return [dma(cols(wqkv_hbm, j * D + g * 128, 128), cols(wqkv_v, j * D + g * 128, 128))
                    for g in gs for j in (1, 2)]

        def ffn_copies(f, n):
            return [dma(cols(wg_hbm, f, n), cols(wg_v, f, n)), dma(cols(wu_hbm, f, n), cols(wu_v, f, n)),
                    dma(rows(wd_hbm, f, n), rows(wd_v, f, n))]

        stages = [[dma(wr_hbm, wr_v), dma(wphi_hbm, wphi_v)] + kv_copies([0]) + [x_copy(0, 128), x_copy(TH, 128)],
                  [x_copy(128, TH - 128), x_copy(TH + 128, TH - 128)],
                  kv_copies([1]) + [x_copy(T, T)],
                  kv_copies([2, 3]),
                  kv_copies([4]) + [x_copy(2 * T, T)] + kv_copies([5]),
                  kv_copies([6, 7]) + [x_copy(3 * T, S - 3 * T)],
                  [dma(cols(wqkv_hbm, 0, D), cols(wqkv_v, 0, D)), dma(wo_hbm, wo_v)] + ffn_copies(0, F1),
                  ffn_copies(F1, F - F1)]
        for stage in stages:
            for c in stage:
                c.start()

        def wait_stage(j):
            with scope(f"w_{j}"):
                for c in stages[j]:
                    c.wait()

        summed = (0, 2, 3, 5, 6)

        def layernorm(i, pieces):
            for p in pieces:
                starts = (i * T + p * 16, i * T + TH + p * 16)
                x = jnp.concatenate([x_v[r:r + 16, :] for r in starts], axis=0).astype(f32)
                m32 = jnp.sum(x, axis=1, keepdims=True) * (1.0 / D)
                yield 70, [jnp.broadcast_to(m32[24:], (8, 128))]
                c = x - m32
                v32 = jnp.sum(c * c, axis=1, keepdims=True) * (1.0 / D)
                inv = 1.0 / _rb(jnp.sqrt(_rb(_rb(v32) + LN_EPS)))
                yield 170, [jnp.broadcast_to(inv[24:], (8, 128))]
                halves = []
                for k, r in enumerate(starts):
                    q = slice(16 * k, 16 * (k + 1))
                    xn = (_rb(x[q] - _rb(m32[q])) * inv[q]).astype(bf16)
                    xn_v[r // 2:r // 2 + 8, :] = _pack(xn)
                    xn = xn.astype(f32)
                    score = jnp.sum(xn * wr_v[...].astype(f32).reshape(1, D), axis=1, keepdims=True)
                    r_v[r:r + 16, :] = jnp.broadcast_to(_rb(score), (16, 128))
                    halves.append(xn)
                    if k == 0:
                        yield 130, [xn[8:, D - 128:]]
                a, b = halves
                terms = _right_terms(a[:, :DH], b[:, :DH], a[:, DH:], b[:, DH:])
                row = (i * TH + p * 16) // 2
                for n, j in enumerate(summed):
                    packed = _pack(terms[j])
                    xs_v[n, row:row + 8, :] = packed
                yield 190, [packed[:, DH - 128:]]

        def token_term(t, j, l):
            def rows_at(start, stride):
                r = t * stride + start + l // 2
                return pl.ds(r if isinstance(r, int) else pl.multiple_of(r, 64), 64)
            if j == 1:
                return xn_v[rows_at(0, T // 2), :DH]
            if j == 4:
                return xn_v[rows_at(TH // 2, T // 2), DH:]
            return xs_v[summed.index(j), rows_at(0, TH // 2), :]

        wait_stage(0)

        er = lax.broadcasted_iota(i32, (128, Dh), 0)
        ec = lax.broadcasted_iota(i32, (128, Dh), 1)
        eT = jnp.where(((er & 63) >> 1) == ec, 1.0, 0.0).astype(bf16)
        pT = _dot_nt(eT, wphi_v[...])
        rr = lax.broadcasted_iota(i32, (128, 128), 0)
        cc = lax.broadcasted_iota(i32, (128, 128), 1)
        same_head = (rr >> 6) * 2 + (rr & 1) == (cc >> 5)
        for g in range(NG):
            pT_v[:, g * 128:(g + 1) * 128] = _pack(jnp.where(same_head, pT[:, g * 128:(g + 1) * 128], 0.0))

        bg = _Interleaver(at)

        def fold(g, j):
            w = wqkv_v[:, j * D + g * 128: j * D + (g + 1) * 128]
            return _dot_nt(bg.operand(pT_v[:, g * 128:(g + 1) * 128]), w)

        def weight_terms(make, ref, row, top, bot, scale=None):
            top, bot = top.astype(f32), bot.astype(f32)
            if scale is not None:
                top, bot = top * scale, bot * scale
            for j, term in enumerate(make(top[:, :DH], top[:, DH:], bot[:, :DH], bot[:, DH:])):
                packed = _pack(term)
                ref[j, row:row + packed.shape[0], :] = packed
            return [packed[-8:, DH - 128:]]

        def prepare_kv(g):
            wk = fold(g, 1)
            wv = wqkv_v[:, 2 * D + g * 128: 2 * D + (g + 1) * 128].T
            for r in range(0, 64, WR):
                bg.add(7 * WR, weight_terms, _left_terms, wkv_v, g * 64 + 32 + r // 2, wv[r:r + WR], wv[64 + r:64 + r + WR])
            for r in range(0, 64, WR):
                bg.add(7 * WR, weight_terms, _left_terms, wkv_v, g * 64 + r // 2, wk[r:r + WR], wk[64 + r:64 + r + WR], LOG2E,
                       delay=delay)

        folded = []

        def prepare_q(g):
            folded.append(fold(g, 0))
            if g % 2 == 1:
                top, bot = folded[-2:]
                for r in range(0, 128, WR):
                    bg.add(7 * WR, weight_terms, _left_terms, wq_v, g * 32 - 32 + r // 2, top[r:r + WR], bot[r:r + WR],
                           LOG2E, delay=delay)

        def prepare_o():
            for b in range(NB):
                for r in range(0, 128, WR):
                    lo, hi = 2 * b * 128 + r, (2 * b + 1) * 128 + r
                    yield 7 * WR, weight_terms(_right_terms, wos_v, b * 64 + r // 2, wo_v[lo:lo + WR, :], wo_v[hi:hi + WR, :])

        sel = {}

        def route():
            r = r_v[...]
            r = jnp.where(r != r, -jnp.inf, r)
            r = r.reshape(S // 64, 64, 128)
            io = lax.broadcasted_iota(i32, r.shape, 0) * 64 + lax.broadcasted_iota(i32, r.shape, 1)
            rmax = jnp.max(jnp.max(r, axis=0), axis=0, keepdims=True)
            first = jnp.min(jnp.min(jnp.where(r == rmax[None], io, S - 1), axis=0))
            idx = jnp.clip(first, 0, S - 1)
            wrd = jnp.broadcast_to(xn_v[pl.ds(idx // 2, 1), :], (128, D))
            bits = jnp.where(idx % 2 == 1, wrd & jnp.uint32(0xFFFF0000), wrd << 16)
            xb_v[0:D, :] = pltpu.bitcast(bits, f32).T
            r_sel = r_v[pl.ds(idx, 1), :][:, 0:1]
            spare = pl.multiple_of(D + (first >> 31) * D, 8)
            sel.update(idx=idx, gate=_rb(1.0 / (1.0 + jnp.exp(-r_sel))), y=None, hrow=spare, late_weights=False)

        def ffn_units():
            yield from prepare_o()
            sel["wo_ready"] = True
            for c in range(NF):
                col = c * FP
                assert col < F1 or sel["late_weights"]
                ag = au = None
                for k in range(0, D, 8):
                    xb = jnp.tile(xb_v[k:k + 8, :], (1, FP // 128))
                    pg = wg_v[k:k + 8, col:col + FP].astype(f32) * xb
                    pu = wu_v[k:k + 8, col:col + FP].astype(f32) * xb
                    ag = pg if ag is None else ag + pg
                    au = pu if au is None else au + pu
                    if (k + 8) % UK == 0:
                        yield 3 * UK // 2, [ag[:, 0:128], ag[:, 128:256], au[:, 0:128], au[:, 128:256]]
                gt = _rb(jnp.sum(ag, axis=0, keepdims=True))
                up = _rb(jnp.sum(au, axis=0, keepdims=True))
                h = jnp.broadcast_to(_rb(_rb(_silu(gt)) * up), (128, FP)).T
                xb_v[pl.ds(sel["hrow"], FP), :] = h
                yield 100, [h[-8:]]
                for k in range(0, FP, 8):
                    hk = xb_v[pl.ds(sel["hrow"] + k, 8), :]
                    pd = wd_v[col + k:col + k + 8, :].astype(f32) * jnp.tile(hk, (1, D // 128))
                    sel["y"] = pd if sel["y"] is None else sel["y"] + pd
                    if (k + 8) % UD == 0:
                        yield 3 * UD, [sel["y"][:, l * 128:(l + 1) * 128] for l in range(D // 128)]

        kr = lax.broadcasted_iota(i32, (64, 128), 0)
        kc = lax.broadcasted_iota(i32, (64, 128), 1)
        same = (kr >> 5) == (kc & 1)

        def strassen(product, done):
            def mul(j):
                m = product(j)
                bg.issue()
                return m
            m1 = mul(1)
            m3 = mul(3)
            done(1, 0, m1 + m3)
            m2 = mul(2)
            c22 = m2 - m1
            m4 = mul(4)
            done(0, 1, m2 + m4)
            c11 = m3 - m4
            m0 = mul(0)
            c22 = c22 + m0
            c11 = c11 + m0
            done(1, 1, c22 + mul(5))
            done(0, 0, c11 + mul(6))

        def project(w_ref, row, t, l):
            return lambda j: _dot_nt(bg.operand(w_ref[j, row:row + 64, :]), _unpack(token_term(t, j, l)))

        def k_feature(i, pr, pv, state):
            ep, en = _dual_softmax(pv[:64])
            phi = jnp.concatenate([ep.reshape(64, 128), en.reshape(64, 128)], axis=0)
            if not state and i > 0:
                state["z"] = z_v[pr]
            state["z"] = phi + state["z"] if state else phi
            state.setdefault("parts", []).append((pv[64:].astype(bf16), phi.astype(bf16)))
            if len(state["parts"]) == T // 128:
                if i < NT - 1:
                    z_v[pr] = state["z"]
                else:
                    zb_v[pr] = jnp.broadcast_to(jnp.sum(state["z"], axis=1, keepdims=True), (128, 128))
                bg.matmuls.append((k_accum, (i, pr, state["parts"])))
            return [state["parts"][-1][1][112:]]

        kv_done = set()

        def k_accum(i, pr, parts):
            kv = _dot_nt(jnp.concatenate([p[0] for p in parts], axis=1), jnp.concatenate([p[1] for p in parts], axis=1))
            if i > 0:
                kv = kv + kv_v[pr]
            if i < NT - 1:
                kv_v[pr] = kv
            else:
                kvT_v[pr] = _pack(jnp.where(same, kv, 0.0))
                kv_done.add(pr)

        prepare_kv(0)
        bg.drain()
        bg.fill(layernorm(0, range(128 // 16)))
        bg.finish_filler()
        wait_stage(1)
        bg.fill(layernorm(0, range(128 // 16, TH // 16)))
        for i in range(NT):
            for g in range(NG):
                if i + 1 < NT and g == (1 if i == 0 else 0):
                    bg.fill(layernorm(i + 1, range(TH // 16)))
                if verbose:
                    print("block", i, g, "backlog", len(bg.work), len(bg.matmuls), "filler", bg.filler is not None)
                bg.need(wkv_v, g * 64)
                states = ({}, {})
                for l in range(0, TH, 128):
                    bg.budget = b_first if (i, g, l) == (0, 0, 0) else b_tile0 if i == 0 else b_ln if i < NT - 1 else b_ffn
                    strassen(project(wkv_v, g * 64, i, l),
                             lambda rh, ch, c: bg.add(115, k_feature, i, 2 * g + rh, c, states[rh], delay=delay))
                    if (i, g, l) == (0, 0, 0):
                        bg.finish_filler()
                    if (i, g, l) == (NT - 1, 0, 0):
                        wait_stage(6)
                        route()
                        bg.fill(ffn_units())
                    if i == NT - 1 and l == 0:
                        prepare_q(g)
                if i == 0 and g in ahead:
                    wait_stage(ahead[g][0])
                    for gg in ahead[g][1]:
                        prepare_kv(gg)
            if i < NT - 1:
                bg.finish_filler()

        idx = sel["idx"]
        t_sel = idx // T

        tiles = [lax.rem(t_sel + 1 + i, NT) for i in range(NT - 1)] + [t_sel]
        o_written = set()

        def q_feature(i, b, a, l, pq, state):
            pr = 4 * b + a
            ep, en = _dual_softmax(pq)
            zb = zb_v[pr]
            den = jnp.sum(ep * zb[0:64].reshape(8, 8, 128) + en * zb[64:128].reshape(8, 8, 128), axis=0)
            inv = _recip(_head_reduce(den, jnp.add) + 1e-6)
            phi = jnp.concatenate([ep.reshape(64, 128), en.reshape(64, 128)], axis=0).astype(bf16)
            state.setdefault(a, {})[l] = (phi, inv)
            if len(state[a]) == T // 128:
                bg.matmuls.append((q_attend, (i, b, a, state)))
            return [phi[112:]]

        def q_attend(i, b, a, state):
            phi, inv = (jnp.concatenate([state[a][l][k] for l in sorted(state[a])], axis=1) for k in range(2))
            num = _dot(_unpack(kvT_v[4 * b + a]), phi)
            sc = jnp.concatenate([jnp.broadcast_to(inv[0:1], (32, T)), jnp.broadcast_to(inv[1:2], (32, T))], axis=0)
            state.setdefault("o", {})[a] = num * sc
            if len(state["o"]) == 4:
                lo, hi = (jnp.concatenate([state["o"][k], state["o"][k + 1]], axis=0) for k in (0, 2))
                for js in o_groups:
                    bg.add(50 * len(js), o_terms, i, b, js, lo, hi, delay=delay)

        def o_terms(i, b, js, lo, hi):
            terms = _left_terms(lo[:, :TH], hi[:, :TH], lo[:, TH:], hi[:, TH:])
            vals = []
            for j in js:
                packed = _pack(terms[j].astype(bf16).T)
                o_v[i % 2, j, :, b * 128:(b + 1) * 128] = packed
                o_written.add((i, b, j))
                vals.append(packed[-8:])
            return vals

        out_ready, out_copies = [], []

        def residual(i, s, r0, c0):
            t = tiles[i]
            last = i == NT - 1
            n = s.shape[0]
            gin = _unpack(xn_v[pl.ds(pl.multiple_of(t * (T // 2) + r0 // 2, n // 2), n // 2), c0:c0 + 128]).astype(f32)
            if last:
                upd = _rb(_rb(jnp.sum(sel["y"][:, c0:c0 + 128], axis=0, keepdims=True)) * sel["gate"])
                hit = lax.broadcasted_iota(i32, (n, 128), 0) == idx - t_sel * T - r0
                gin = jnp.where(hit, gin + upd, gin)
            row = pl.ds(pl.multiple_of(t * T + r0, n), n)
            res = (x_v[row, c0:c0 + 128].astype(f32) + s * _silu(gin)).astype(bf16)
            out_v[row, c0:c0 + 128] = res
            if last and (r0 + n) % TH == 0:
                row = pl.ds(pl.multiple_of(t * T + r0 + n - TH, TH), TH)
                out_ready.append(dma(out_v.at[row, pl.ds(c0, 128)], out_hbm.at[row, pl.ds(c0, 128)]))
            elif not last and r0 + n == TH and c0 == DH - 128:
                row = pl.ds(pl.multiple_of(t * T, T), T)
                out_ready.append(dma(out_v.at[row, :], out_hbm.at[row, :]))
            return [res[-16:]]

        def send_ready():
            while out_ready:
                out_copies.append(out_ready.pop(0))
                out_copies[-1].start()

        def out_chunk(i, n):
            assert sel["wo_ready"]
            while not all((i, b, j) in o_written for b in range(NB) for j in range(7)):
                if verbose:
                    print("forced", i, n, len(bg.work), len(bg.matmuls))
                bg.force()
            if i == NT - 1:
                assert bg.filler is None or not strict
                bg.finish_filler()

            def product(j):
                m = _dot(bg.operand(o_v[i % 2, j]), _unpack(wos_v[j, :, n * 128:(n + 1) * 128]))
                send_ready()
                return m

            def done(rh, ch, c):
                for r in range(0, TH, RR):
                    bg.add(9 * RR // 8, residual, i, c[r:r + RR], rh * TH + r, ch * DH + n * 128, delay=delay)

            strassen(product, done)

        outs = [(i, n) for i in range(NT) for n in range(NB)]
        for i in range(NT):
            for b in range(NB):
                step = i * NB + b
                state = {}

                with_out = step >= NB + olag
                if verbose:
                    print("step", step, "backlog", len(bg.work), len(bg.matmuls), "filler", bg.filler is not None)
                bg.need(wq_v, b * 64)
                while not all(pr in kv_done for pr in range(4 * b, 4 * b + 4)):
                    bg.force()
                bg.budget = b_both if with_out else b_alone
                for l in range(0, TH, 128):
                    def done(rh, ch, c):
                        for a in range(2):
                            bg.add(140, q_feature, i, b, 2 * rh + a, ch * TH + l, c[a * 64:(a + 1) * 64], state, delay=delay)

                    strassen(project(wq_v, b * 64, tiles[i], l), done)
                if step == late_at:
                    wait_stage(7)
                    sel["late_weights"] = True
                if with_out:
                    out_chunk(*outs.pop(0))
        while outs:
            out_chunk(*outs.pop(0))
        bg.drain()
        send_ready()
        assert len(used) <= n_dma
        with scope("w_out"):
            for c in out_copies:
                c.wait()

    scratch = [
        pltpu.VMEM((S, D), bf16),
        pltpu.VMEM((D, 3 * D), bf16),
        pltpu.VMEM((D, Dh), bf16),
        pltpu.VMEM((D, D), bf16),
        pltpu.VMEM((D,), bf16),
        pltpu.VMEM((D, F), bf16),
        pltpu.VMEM((D, F), bf16),
        pltpu.VMEM((F, D), bf16),
        pltpu.VMEM((S, D), bf16),
        pltpu.VMEM((S // 2, D), u32),
        pltpu.VMEM((5, S // 4, DH), u32),
        pltpu.VMEM((7, D // 2, DH), u32),
        pltpu.VMEM((7, D // 4, DH), u32),
        pltpu.VMEM((7, D // 4, DH), u32),
        pltpu.VMEM((64, D), u32),
        pltpu.VMEM((NP, 64, 128), f32),
        pltpu.VMEM((NP, 128, 128), f32),
        pltpu.VMEM((NP, 32, 128), u32),
        pltpu.VMEM((NP, 128, 128), f32),
        pltpu.VMEM((S, 128), f32),
        pltpu.VMEM((2, 7, TH // 2, DH), u32),
        pltpu.VMEM((D + FP + 8, 128), f32),
        pltpu.SemaphoreType.DMA((n_dma,)),
    ]
    return kernel, scratch


@jax.jit
def pallas_recurrent_scan__linear_kernel_hedgehog__moe_arch_mod__prompt_kernel(
    A_x: jax.Array,
    A_wqkv: jax.Array,
    A_w_phi: jax.Array,
    A_wo: jax.Array,
    B_x: jax.Array,
    B_w_r: jax.Array,
    B_w_gate: jax.Array,
    B_w_up: jax.Array,
    B_w_down: jax.Array,
):
    del B_x
    B, S, D = A_x.shape
    H, Dh, _ = A_w_phi.shape
    F = B_w_gate.shape[1]
    assert B == 1
    kernel, scratch = make_kernel(S=S, D=D, H=H, F=F, b_both=235, b_ln=155, UK=64, UD=32)
    out = pl.pallas_call(
        kernel,
        out_shape=jax.ShapeDtypeStruct((S, D), A_x.dtype),
        in_specs=[pl.BlockSpec(memory_space=pl.ANY)] * 8,
        out_specs=pl.BlockSpec(memory_space=pl.ANY),
        scratch_shapes=scratch,
        compiler_params=pltpu.CompilerParams(
            vmem_limit_bytes=110 * 1024 * 1024),
        name="hedgehog_mod",
    )(A_x.reshape(S, D), A_wqkv, A_w_phi.reshape(H * Dh, Dh), A_wo, B_w_r, B_w_gate, B_w_up, B_w_down)
    return out.reshape(B, S, D)
```

```python
import contextlib

import jax
import jax.numpy as jnp
import numpy as np
from jax import lax
import jax.experimental.pallas as pl
import jax.experimental.pallas.tpu as pltpu

bf16, f32, u32, i32 = jnp.bfloat16, jnp.float32, jnp.uint32, jnp.int32
LOG2E = 1.4426950408889634
LN_EPS = float(np.asarray(1e-5, dtype=bf16))
NT_DIMS = (((1,), (1,)), ((), ()))


def _dot(a, b):
    return jnp.dot(a, b, preferred_element_type=f32)


def _dot_nt(a, b):
    return lax.dot_general(a, b, NT_DIMS, preferred_element_type=f32)


def _pack(x):
    return pltpu.bitcast(x.astype(bf16), u32)


def _unpack(x):
    return pltpu.bitcast(x, bf16)


def _rb(x):
    return x.astype(bf16).astype(f32)


def _recip(x):
    return pltpu.reciprocal(x, approx=False, full_range=False)


def _silu(x):
    h = 0.5 * x
    return h * jnp.tanh(h) + h


def _left_terms(a11, a12, a21, a22):
    return [a11 + a22, a21 + a22, a11, a22, a11 + a12, a21 - a11, a12 - a22]


def _right_terms(b11, b12, b21, b22):
    return [b11 + b22, b11, b12 - b22, b21 - b11, b22, b11 + b12, b21 + b22]


def _zero_after(vals):
    parts = []
    for v in vals:
        b = pltpu.bitcast(v, u32)
        parts += [b[r:r + 8, c:c + 128] for r in range(0, b.shape[0], 8) for c in range(0, b.shape[1], 128)]
    while len(parts) > 1:
        parts = [parts[k] | parts[k + 1] if k + 1 < len(parts) else parts[k] for k in range(0, len(parts), 2)]
    return (parts[0] >> 16) >> 16


def _after(op, zeros, at):
    n = op.shape[0] // len(zeros)
    parts, done = [], 0
    for k, zero in enumerate(zeros):
        r = k * n + at * 8
        if zero is not None:
            parts += [op[done:r]] if r > done else []
            parts.append(op[r:r + 8] | jnp.tile(zero, (1, op.shape[1] // 128)))
            done = r + 8
    parts += [op[done:]] if done < op.shape[0] else []
    return parts[0] if len(parts) == 1 else jnp.concatenate(parts, axis=0)


class _Interleaver:
    def __init__(self, at):
        self.slot, self.at, self.budget, self.credit = 0, at, 0, 0
        self.work, self.matmuls, self.filler = [], [], None

    def add(self, cost, fn, *args, delay=0):
        self.work.append((self.slot + delay, cost, fn, args))

    def fill(self, gen):
        self.finish_filler()
        self.filler = gen

    def finish_filler(self):
        for _ in self.filler or ():
            pass
        self.filler = None

    def tick(self):
        self.slot += 1
        self.credit = min(self.credit, 0) + self.budget
        vals = []
        while self.credit > 0 and self.work and self.work[0][0] < self.slot:
            _, cost, fn, args = self.work.pop(0)
            vals += fn(*args)
            self.credit -= cost
        while self.credit > 0 and self.filler:
            unit = next(self.filler, None)
            if unit is None:
                self.filler = None
            else:
                self.credit -= unit[0]
                vals += unit[1]
        return _zero_after(vals) if vals else None

    def operand(self, op):
        return _unpack(_after(op, [self.tick() for _ in range(op.shape[0] // 64)], self.at))

    def issue(self):
        if self.matmuls:
            fn, args = self.matmuls.pop(0)
            fn(*args)

    def need(self, ref, row):
        last = [k for k, w in enumerate(self.work) if len(w[3]) > 2 and w[3][1] is ref and row <= w[3][2] < row + 64]
        for _ in range(last[-1] + 1 if last else 0):
            _, _, fn, args = self.work.pop(0)
            fn(*args)

    def force(self):
        if self.matmuls:
            self.issue()
        else:
            _, _, fn, args = self.work.pop(0)
            fn(*args)

    def drain(self):
        while self.work or self.matmuls:
            while self.work:
                _, _, fn, args = self.work.pop(0)
                fn(*args)
            while self.matmuls:
                self.issue()


def _head_reduce(v, op):
    v = op(v, pltpu.roll(v, 4, 0))
    return op(v, pltpu.roll(v, 2, 0))


def _dual_softmax(p):
    t = p.shape[1]
    p3 = p.reshape(8, 8, t)
    mx = _head_reduce(jnp.max(p3, axis=0), jnp.maximum)
    mn = _head_reduce(jnp.min(p3, axis=0), jnp.minimum)
    ep = jnp.exp2(p3 - mx[None])
    en = jnp.exp2(mn[None] - p3)
    sp = _head_reduce(jnp.sum(ep, axis=0), jnp.add)
    sn = _head_reduce(jnp.sum(en, axis=0), jnp.add)
    return ep * _recip(sp)[None], en * _recip(sn)[None]


def make_kernel(S=2048, D=1024, H=32, F=3584, T=512, olag=2, delay=4, WR=16, at=6, quiet=1, RR=128, UK=128, UD=32,
                b_tile0=190, b_ln=170, b_ffn=175, b_alone=215, b_both=240, late_folds=1, compact=False, pinned=('kv', 'q', 'o', 'ot'), full='w', cw=11, co=70, cq=150, cf=105, strict=False, verbose=False,
                o_groups=((0, 1, 2), (3, 4), (5, 6)), scopes=False):
    Dh = D // H
    NT = S // T
    NG = D // 128
    NP = D // 64
    NB = NG // 2
    TH, DH = T // 2, D // 2
    FP = 256
    NF = F // FP
    n_dma = 64
    F1 = 5 * FP
    ahead = {0: (2, [1]), 1: (3, [2, 3]), 3: (4, [4, 5]), 5: (5, [6, 7])}

    def kernel(x_hbm, wqkv_hbm, wphi_hbm, wo_hbm, wr_hbm, wg_hbm, wu_hbm, wd_hbm, out_hbm,
               x_v, wqkv_v, wphi_v, wo_v, wr_v, wg_v, wu_v, wd_v, out_v,
               xn_v, xs_v, wkv_v, wq_v, wos_v, pT_v, kv_v, z_v, kvT_v, zb_v, r_v, o_v, xb_v, wrb_v, sem):

        def scope(name):
            return jax.named_scope(name) if scopes else contextlib.nullcontext()

        used = []

        def dma(src, dst):
            used.append(None)
            return pltpu.make_async_copy(src, dst, sem.at[len(used) - 1])

        def cols(ref, c, n):
            return ref.at[:, pl.ds(c, n)]

        def rows(ref, r, n):
            return ref.at[pl.ds(r, n), :]

        def x_copy(r, n):
            return dma(rows(x_hbm, r, n), rows(x_v, r, n))

        def kv_copies(gs):
            return [dma(cols(wqkv_hbm, j * D + g * 128, 128), cols(wqkv_v, j * D + g * 128, 128))
                    for g in gs for j in (1, 2)]

        def ffn_copies(f, n):
            return [dma(cols(wg_hbm, f, n), cols(wg_v, f, n)), dma(cols(wu_hbm, f, n), cols(wu_v, f, n)),
                    dma(rows(wd_hbm, f, n), rows(wd_v, f, n))]

        early = [dma(wr_hbm, wr_v), x_copy(0, 128), x_copy(TH, 128)]
        stages = [[x_copy(128, TH - 128), x_copy(TH + 128, TH - 128), dma(wphi_hbm, wphi_v)],
                  kv_copies([0]),
                  kv_copies([1]) + [x_copy(T, T)],
                  kv_copies([2, 3]),
                  kv_copies([4]) + [x_copy(2 * T, T)] + kv_copies([5]),
                  kv_copies([6, 7]) + [x_copy(3 * T, S - 3 * T)],
                  [dma(cols(wqkv_hbm, 0, D), cols(wqkv_v, 0, D)), dma(wo_hbm, wo_v)] + ffn_copies(0, F1),
                  ffn_copies(F1, F - F1)]
        for stage in [early] + stages:
            for c in stage:
                c.start()

        def wait_stage(j):
            with scope(f"w_{j}"):
                for c in stages[j]:
                    c.wait()
            if j > 1:
                bg.credit = -quiet * bg.budget

        summed = (0, 2, 3, 5, 6)

        lane = lax.broadcasted_iota(i32, (8, 128), 1)

        def layernorm(i, pieces):
            scores = r_v[i] if pieces[0] else jnp.zeros((8, 128), f32)
            for p in pieces:
                starts = (i * T + p * 16, i * T + TH + p * 16)
                x = jnp.concatenate([x_v[r:r + 16, :] for r in starts], axis=0).astype(f32)
                m32 = jnp.sum(x, axis=1, keepdims=True) * (1.0 / D)
                yield 75, [jnp.broadcast_to(m32[24:], (8, 128))]
                m = _rb(m32)
                d = x - m
                v32 = jnp.sum(d * d, axis=1, keepdims=True) * (1.0 / D) - (m32 - m) * (m32 - m)
                if compact:
                    vb = jnp.broadcast_to(v32, (32, 128))
                    vc = vb[0:8]
                    for q in range(1, 4):
                        vc = jnp.where(lane >= 32 * q, vb[8 * q:8 * q + 8], vc)
                    ic = _recip(jnp.minimum(_rb(jnp.sqrt(_rb(_rb(vc) + LN_EPS))), 1e38))
                    inv = jnp.concatenate([ic[:, 32 * q:32 * q + 1] for q in range(4)], axis=0)
                else:
                    inv = _recip(jnp.minimum(_rb(jnp.sqrt(_rb(_rb(v32) + LN_EPS))), 1e38))
                yield 190, [jnp.broadcast_to(inv[24:], (8, 128))]
                xn = d * inv
                a, b = xn[:16], xn[16:]
                for r, half in zip(starts, (a, b)):
                    packed = _pack(half)
                    xn_v[r // 2:r // 2 + 8, :] = packed
                score = jnp.sum(xn * jnp.tile(wrb_v[...], (4, 1)), axis=1, keepdims=True)
                for q in range(4):
                    scores = jnp.where((lane >> 1) == 4 * p + q, score[8 * q:8 * q + 8], scores)
                yield 140, [packed[:, D - 128:], scores]
                terms = _right_terms(a[:, :DH], b[:, :DH], a[:, DH:], b[:, DH:])
                row = (i * TH + p * 16) // 2
                vals = []
                for n, j in enumerate(summed):
                    packed = _pack(terms[j])
                    xs_v[n, row:row + 8, :] = packed
                    vals.append(packed)
                if p == pieces[-1]:
                    r_v[i] = scores
                yield 75, vals if "l" in full else [packed[:, DH - 128:]]

        def token_term(t, j, l):
            def rows_at(start, stride):
                r = t * stride + start + l // 2
                return pl.ds(r if isinstance(r, int) else pl.multiple_of(r, 64), 64)
            if j == 1:
                return xn_v[rows_at(0, T // 2), :DH]
            if j == 4:
                return xn_v[rows_at(TH // 2, T // 2), DH:]
            return xs_v[summed.index(j), rows_at(0, TH // 2), :]

        with scope('w_early'):
            for c in early:
                c.wait()

        wr = jnp.broadcast_to(wr_v[...].astype(f32).reshape(1, D), (8, D))
        wrb_v[...] = wr
        nought = pl.ds(pl.multiple_of((jnp.max(pltpu.bitcast(wr[:, 0:128], i32) & 0xFFFF) >> 31) * 8, 8), 8)
        for name, ref in dict(kv=wkv_v.at[0], q=wq_v.at[0], o=wos_v.at[0], acc=kv_v.at[0], z=z_v.at[0], kvT=kvT_v.at[0],
                              zb=zb_v.at[0], ot=o_v.at[0, 0]).items():
            if name in pinned:
                ref[nought, 0:128] = jnp.zeros((8, 128), ref.dtype)
        for _ in layernorm(0, range(128 // 16)):
            pass
        wait_stage(0)

        er = lax.broadcasted_iota(i32, (128, Dh), 0)
        ec = lax.broadcasted_iota(i32, (128, Dh), 1)
        eT = jnp.where(((er & 63) >> 1) == ec, 1.0, 0.0).astype(bf16)
        pT = _dot_nt(eT, wphi_v[...])
        rr = lax.broadcasted_iota(i32, (128, 128), 0)
        cc = lax.broadcasted_iota(i32, (128, 128), 1)
        same_head = (rr >> 6) * 2 + (rr & 1) == (cc >> 5)
        for g in range(NG):
            pT_v[:, g * 128:(g + 1) * 128] = _pack(jnp.where(same_head, pT[:, g * 128:(g + 1) * 128], 0.0))

        bg = _Interleaver(at)

        def fold(g, j):
            w = wqkv_v[:, j * D + g * 128: j * D + (g + 1) * 128]
            return _dot_nt(bg.operand(pT_v[:, g * 128:(g + 1) * 128]), w)

        def weight_terms(make, ref, row, top, bot, scale=None):
            top, bot = top.astype(f32), bot.astype(f32)
            if scale is not None:
                top, bot = top * scale, bot * scale
            vals = []
            for j, term in enumerate(make(top[:, :DH], top[:, DH:], bot[:, :DH], bot[:, DH:])):
                packed = _pack(term)
                ref[j, row:row + packed.shape[0], :] = packed
                vals.append(packed)
            return vals if "w" in full else [packed[-8:, DH - 128:]]

        def prepare_kv(g):
            wk = fold(g, 1)
            wv = _pack(wqkv_v[:, 2 * D + g * 128: 2 * D + (g + 1) * 128].T)
            for r in range(0, 64, WR):
                bg.add(cw * WR, weight_terms, _left_terms, wkv_v, g * 64 + 32 + r // 2, _unpack(wv[r // 2:(r + WR) // 2]), _unpack(wv[32 + r // 2:32 + (r + WR) // 2]))
            for r in range(0, 64, WR):
                bg.add(cw * WR, weight_terms, _left_terms, wkv_v, g * 64 + r // 2, wk[r:r + WR], wk[64 + r:64 + r + WR], LOG2E,
                       delay=delay)

        folded = []

        def prepare_q(g):
            folded.append(fold(g, 0))
            if g % 2 == 1:
                top, bot = folded[-2:]
                for r in range(0, 128, WR):
                    bg.add(cw * WR, weight_terms, _left_terms, wq_v, g * 32 - 32 + r // 2, top[r:r + WR], bot[r:r + WR],
                           LOG2E, delay=delay)

        def prepare_o():
            for b in range(NB):
                for r in range(0, 128, WR):
                    lo, hi = 2 * b * 128 + r, (2 * b + 1) * 128 + r
                    yield cw * WR, weight_terms(_right_terms, wos_v, b * 64 + r // 2, wo_v[lo:lo + WR, :], wo_v[hi:hi + WR, :])

        sel = {}

        def route():
            r = _rb(r_v[...])
            key = jnp.where(r != r, -jnp.inf, r)
            best = jnp.max(jnp.max(jnp.max(key, axis=0), axis=0, keepdims=True), axis=1, keepdims=True)
            tile, sub = (lax.broadcasted_iota(i32, r.shape, k) for k in range(2))
            row = tile * T + ((lane >> 2) & 1) * TH + (lane >> 3) * 16 + ((lane >> 1) & 1) * 8 + sub
            first = jnp.min(jnp.min(jnp.where(key == best, row, S - 1), axis=0))
            idx = jnp.clip(first, 0, S - 1)
            hit = (row == idx) & ((lane & 1) == 0)
            r_sel = jnp.sum(jnp.sum(jnp.sum(jnp.where(hit, r, 0.0), axis=0), axis=0, keepdims=True), axis=1, keepdims=True)
            wrd = jnp.broadcast_to(xn_v[pl.ds(idx // 2, 1), :], (128, D))
            bits = jnp.where(idx % 2 == 1, wrd & jnp.uint32(0xFFFF0000), wrd << 16)
            xb = pltpu.bitcast(bits, f32).T
            xb_v[0:D, :] = xb
            sel.update(idx=idx, gate=_rb(1.0 / (1.0 + jnp.exp(-r_sel))), y=None,
                       hrow=pl.multiple_of(D + (first >> 31) * D, 8))
            yield 100, [xb[-8:]]

        def ffn_units():
            for c in range(NF):
                col = c * FP
                assert col < F1 or "late" in sel
                ag = au = None
                for k in range(0, D, 8):
                    xb = jnp.tile(xb_v[k:k + 8, :], (1, FP // 128))
                    pg = wg_v[k:k + 8, col:col + FP].astype(f32) * xb
                    pu = wu_v[k:k + 8, col:col + FP].astype(f32) * xb
                    ag = pg if ag is None else ag + pg
                    au = pu if au is None else au + pu
                    if (k + 8) % UK == 0:
                        yield cf * UK // 64, [ag[:, 0:128], ag[:, 128:256], au[:, 0:128], au[:, 128:256]]
                gt = _rb(jnp.sum(ag, axis=0, keepdims=True))
                up = _rb(jnp.sum(au, axis=0, keepdims=True))
                h = jnp.broadcast_to(_rb(_rb(_silu(gt)) * up), (128, FP)).T
                xb_v[pl.ds(sel["hrow"], FP), :] = h
                yield 100, [h[-8:]]
                for k in range(0, FP, 8):
                    hk = xb_v[pl.ds(sel["hrow"] + k, 8), :]
                    pd = wd_v[col + k:col + k + 8, :].astype(f32) * jnp.tile(hk, (1, D // 128))
                    sel["y"] = pd if sel["y"] is None else sel["y"] + pd
                    if (k + 8) % UD == 0:
                        yield cf * UD // 32, [sel["y"][:, l * 128:(l + 1) * 128] for l in range(D // 128)]

        kr = lax.broadcasted_iota(i32, (64, 128), 0)
        kc = lax.broadcasted_iota(i32, (64, 128), 1)
        same = (kr >> 5) == (kc & 1)

        def strassen(product, done):
            def mul(j):
                m = product(j)
                bg.issue()
                return m
            m1 = mul(1)
            m3 = mul(3)
            done(1, 0, m1 + m3)
            m2 = mul(2)
            c22 = m2 - m1
            m4 = mul(4)
            done(0, 1, m2 + m4)
            c11 = m3 - m4
            m0 = mul(0)
            c22 = c22 + m0
            c11 = c11 + m0
            done(1, 1, c22 + mul(5))
            done(0, 0, c11 + mul(6))

        def project(w_ref, row, t, l):
            return lambda j: _dot_nt(bg.operand(w_ref[j, row:row + 64, :]), _unpack(token_term(t, j, l)))

        def k_feature(i, pr, pv, state):
            ep, en = _dual_softmax(pv[:64])
            phi = jnp.concatenate([ep.reshape(64, 128), en.reshape(64, 128)], axis=0)
            if not state and i > 0:
                state["z"] = z_v[pr]
            state["z"] = phi + state["z"] if state else phi
            state.setdefault("parts", []).append((pv[64:].astype(bf16), phi.astype(bf16)))
            if len(state["parts"]) == T // 128:
                if i < NT - 1:
                    z_v[pr] = state["z"]
                else:
                    zb_v[pr] = jnp.broadcast_to(jnp.sum(state["z"], axis=1, keepdims=True), (128, 128))
                bg.matmuls.append((k_accum, (i, pr, state["parts"])))
            return [state["parts"][-1][1][112:]]

        kv_done = set()

        def k_accum(i, pr, parts):
            kv = _dot_nt(jnp.concatenate([p[0] for p in parts], axis=1), jnp.concatenate([p[1] for p in parts], axis=1))
            if i > 0:
                kv = kv + kv_v[pr]
            if i < NT - 1:
                kv_v[pr] = kv
            else:
                kvT_v[pr] = _pack(jnp.where(same, kv, 0.0))
                kv_done.add(pr)

        for _ in layernorm(0, range(128 // 16, TH // 16)):
            pass
        wait_stage(1)
        prepare_kv(0)
        bg.drain()
        for i in range(NT):
            for g in range(NG):
                if i + 1 < NT and g == (1 if i == 0 else 0):
                    bg.fill(layernorm(i + 1, range(TH // 16)))
                if verbose:
                    print("block", i, g, "backlog", len(bg.work), len(bg.matmuls), "filler", bg.filler is not None)
                bg.need(wkv_v, g * 64)
                states = ({}, {})
                for l in range(0, TH, 128):
                    bg.budget = b_tile0 if i == 0 else b_ln if i < NT - 1 else b_ffn
                    strassen(project(wkv_v, g * 64, i, l),
                             lambda rh, ch, c: bg.add(125, k_feature, i, 2 * g + rh, c, states[rh], delay=delay))
                    if (i, g, l) == (NT - 1, 0, 0):
                        wait_stage(6)
                        bg.fill(u for gen in (prepare_o(), route(), ffn_units()) for u in gen)
                    if i == NT - 1 and l == 0 and g < NG - late_folds:
                        prepare_q(g)
                if i == 0 and g in ahead:
                    wait_stage(ahead[g][0])
                    for gg in ahead[g][1]:
                        prepare_kv(gg)
            if i < NT - 1:
                bg.finish_filler()

        wait_stage(7)
        sel["late"] = True
        idx = sel["idx"]
        for g in range(NG - late_folds, NG):
            prepare_q(g)
        t_sel = idx // T

        tiles = [lax.rem(t_sel + 1 + i, NT) for i in range(NT - 1)] + [t_sel]
        o_written = set()

        def q_feature(i, b, a, l, pq, state):
            pr = 4 * b + a
            ep, en = _dual_softmax(pq)
            zb = zb_v[pr]
            den = jnp.sum(ep * zb[0:64].reshape(8, 8, 128) + en * zb[64:128].reshape(8, 8, 128), axis=0)
            inv = _recip(_head_reduce(den, jnp.add) + 1e-6)
            phi = jnp.concatenate([ep.reshape(64, 128), en.reshape(64, 128)], axis=0).astype(bf16)
            state.setdefault(a, {})[l] = (phi, inv)
            if len(state[a]) == T // 128:
                bg.matmuls.append((q_attend, (i, b, a, state)))
            return [phi[112:]]

        def q_attend(i, b, a, state):
            phi, inv = (jnp.concatenate([state[a][l][k] for l in sorted(state[a])], axis=1) for k in range(2))
            num = _dot(_unpack(kvT_v[4 * b + a]), phi)
            sc = jnp.concatenate([jnp.broadcast_to(inv[0:1], (32, T)), jnp.broadcast_to(inv[1:2], (32, T))], axis=0)
            state.setdefault("o", {})[a] = num * sc
            if len(state["o"]) == 4:
                lo, hi = (jnp.concatenate([state["o"][k], state["o"][k + 1]], axis=0) for k in (0, 2))
                for js in o_groups:
                    bg.add(co * len(js), o_terms, i, b, js, lo, hi, delay=delay)

        def o_terms(i, b, js, lo, hi):
            terms = _left_terms(lo[:, :TH], hi[:, :TH], lo[:, TH:], hi[:, TH:])
            vals = []
            for j in js:
                packed = _pack(terms[j].astype(bf16).T)
                o_v[i, j, :, b * 128:(b + 1) * 128] = packed
                o_written.add((i, b, j))
                vals.append(packed if "o" in full else packed[-8:])
            return vals

        out_ready, out_copies = [], []

        def residual(i, s, r0, c0):
            t = tiles[i]
            last = i == NT - 1
            n = s.shape[0]
            gin = _unpack(xn_v[pl.ds(pl.multiple_of(t * (T // 2) + r0 // 2, n // 2), n // 2), c0:c0 + 128]).astype(f32)
            if last:
                upd = _rb(_rb(jnp.sum(sel["y"][:, c0:c0 + 128], axis=0, keepdims=True)) * sel["gate"])
                hit = lax.broadcasted_iota(i32, (n, 128), 0) == idx - t_sel * T - r0
                gin = jnp.where(hit, gin + upd, gin)
            row = pl.ds(pl.multiple_of(t * T + r0, n), n)
            out32 = x_v[row, c0:c0 + 128].astype(f32) + s * _silu(gin)
            res = out32.astype(bf16)
            out_v[row, c0:c0 + 128] = res
            if last and (r0 + n) % TH == 0:
                row = pl.ds(pl.multiple_of(t * T + r0 + n - TH, TH), TH)
                out_ready.append(dma(out_v.at[row, pl.ds(c0, 128)], out_hbm.at[row, pl.ds(c0, 128)]))
            elif not last and r0 + n == TH and c0 == DH - 128:
                row = pl.ds(pl.multiple_of(t * T, T), T)
                out_ready.append(dma(out_v.at[row, :], out_hbm.at[row, :]))
            return [_pack(out32)] if "r" in full else [res[-16:]]

        def send_ready():
            while out_ready:
                out_copies.append(out_ready.pop(0))
                out_copies[-1].start()

        def out_chunk(i, n):
            while not all((i, b, j) in o_written for b in range(NB) for j in range(7)):
                if verbose:
                    print("forced", i, n, len(bg.work), len(bg.matmuls))
                bg.force()
            if i == NT - 1:
                assert bg.filler is None or not strict
                bg.finish_filler()

            def product(j):
                m = _dot(bg.operand(o_v[i, j]), _unpack(wos_v[j, :, n * 128:(n + 1) * 128]))
                send_ready()
                return m

            def done(rh, ch, c):
                for r in range(0, TH, RR):
                    bg.add(9 * RR // 8, residual, i, c[r:r + RR], rh * TH + r, ch * DH + n * 128, delay=delay)

            strassen(product, done)

        outs = [(i, n) for i in range(NT) for n in range(NB)]
        for i in range(NT):
            for b in range(NB):
                step = i * NB + b
                state = {}

                with_out = step >= NB + olag
                if verbose:
                    print("step", step, "backlog", len(bg.work), len(bg.matmuls), "filler", bg.filler is not None)
                bg.need(wq_v, b * 64)
                while not all(pr in kv_done for pr in range(4 * b, 4 * b + 4)):
                    bg.force()
                bg.budget = b_both if with_out else b_alone
                for l in range(0, TH, 128):
                    def done(rh, ch, c):
                        for a in range(2):
                            bg.add(cq, q_feature, i, b, 2 * rh + a, ch * TH + l, c[a * 64:(a + 1) * 64], state, delay=delay)

                    strassen(project(wq_v, b * 64, tiles[i], l), done)
                if with_out:
                    out_chunk(*outs.pop(0))
        while outs:
            out_chunk(*outs.pop(0))
        bg.drain()
        send_ready()
        assert len(used) <= n_dma
        with scope("w_out"):
            for c in out_copies:
                c.wait()

    scratch = [
        pltpu.VMEM((S, D), bf16),
        pltpu.VMEM((D, 3 * D), bf16),
        pltpu.VMEM((D, Dh), bf16),
        pltpu.VMEM((D, D), bf16),
        pltpu.VMEM((D,), bf16),
        pltpu.VMEM((D, F), bf16),
        pltpu.VMEM((D, F), bf16),
        pltpu.VMEM((F, D), bf16),
        pltpu.VMEM((S, D), bf16),
        pltpu.VMEM((S // 2, D), u32),
        pltpu.VMEM((5, S // 4, DH), u32),
        pltpu.VMEM((7, D // 2, DH), u32),
        pltpu.VMEM((7, D // 4, DH), u32),
        pltpu.VMEM((7, D // 4, DH), u32),
        pltpu.VMEM((64, D), u32),
        pltpu.VMEM((NP, 64, 128), f32),
        pltpu.VMEM((NP, 128, 128), f32),
        pltpu.VMEM((NP, 32, 128), u32),
        pltpu.VMEM((NP, 128, 128), f32),
        pltpu.VMEM((NT, 8, 128), f32),
        pltpu.VMEM((NT, 7, TH // 2, DH), u32),
        pltpu.VMEM((D + FP + 8, 128), f32),
        pltpu.VMEM((8, D), f32),
        pltpu.SemaphoreType.DMA((n_dma,)),
    ]
    return kernel, scratch


@jax.jit
def pallas_recurrent_scan__linear_kernel_hedgehog__moe_arch_mod__prompt_kernel(
    A_x: jax.Array,
    A_wqkv: jax.Array,
    A_w_phi: jax.Array,
    A_wo: jax.Array,
    B_x: jax.Array,
    B_w_r: jax.Array,
    B_w_gate: jax.Array,
    B_w_up: jax.Array,
    B_w_down: jax.Array,
):
    del B_x
    B, S, D = A_x.shape
    H, Dh, _ = A_w_phi.shape
    F = B_w_gate.shape[1]
    assert B == 1
    kernel, scratch = make_kernel(S=S, D=D, H=H, F=F)
    out = pl.pallas_call(
        kernel,
        out_shape=jax.ShapeDtypeStruct((S, D), A_x.dtype),
        in_specs=[pl.BlockSpec(memory_space=pl.ANY)] * 8,
        out_specs=pl.BlockSpec(memory_space=pl.ANY),
        scratch_shapes=scratch,
        compiler_params=pltpu.CompilerParams(
            vmem_limit_bytes=110 * 1024 * 1024,
            flags={"XLA_TPU_EVENLY_DISTRIBUTE_CRITICAL_NODES": True}),
        name="hedgehog_mod",
    )(A_x.reshape(S, D), A_wqkv, A_w_phi.reshape(H * Dh, Dh), A_wo, B_w_r, B_w_gate, B_w_up, B_w_down)
    return out.reshape(B, S, D)
```

```python
import contextlib

import jax
import jax.numpy as jnp
import numpy as np
from jax import lax
import jax.experimental.pallas as pl
import jax.experimental.pallas.tpu as pltpu

bf16, f32, u32, i32 = jnp.bfloat16, jnp.float32, jnp.uint32, jnp.int32
LOG2E = 1.4426950408889634
LN_EPS = float(np.asarray(1e-5, dtype=bf16))
NT_DIMS = (((1,), (1,)), ((), ()))


def _dot(a, b):
    return jnp.dot(a, b, preferred_element_type=f32)


def _dot_nt(a, b):
    return lax.dot_general(a, b, NT_DIMS, preferred_element_type=f32)


def _pack(x):
    return pltpu.bitcast(x.astype(bf16), u32)


def _unpack(x):
    return pltpu.bitcast(x, bf16)


def _rb(x):
    return x.astype(bf16).astype(f32)


def _recip(x):
    return pltpu.reciprocal(x, approx=False, full_range=False)


def _silu(x):
    h = 0.5 * x
    return h * jnp.tanh(h) + h


def _left_terms(a11, a12, a21, a22):
    return [a11 + a22, a21 + a22, a11, a22, a11 + a12, a21 - a11, a12 - a22]


def _right_terms(b11, b12, b21, b22):
    return [b11 + b22, b11, b12 - b22, b21 - b11, b22, b11 + b12, b21 + b22]


def _zero_after(vals):
    parts = []
    for v in vals:
        b = pltpu.bitcast(v, u32)
        parts += [b[r:r + 8, c:c + 128] for r in range(0, b.shape[0], 8) for c in range(0, b.shape[1], 128)]
    while len(parts) > 1:
        parts = [parts[k] | parts[k + 1] if k + 1 < len(parts) else parts[k] for k in range(0, len(parts), 2)]
    return (parts[0] >> 16) >> 16


def _after(op, zeros, at):
    n = op.shape[0] // len(zeros)
    parts, done = [], 0
    for k, zero in enumerate(zeros):
        r = k * n + at * 8
        if zero is not None:
            parts += [op[done:r]] if r > done else []
            parts.append(op[r:r + 8] | jnp.tile(zero, (1, op.shape[1] // 128)))
            done = r + 8
    parts += [op[done:]] if done < op.shape[0] else []
    return parts[0] if len(parts) == 1 else jnp.concatenate(parts, axis=0)


class _Interleaver:
    def __init__(self, at):
        self.slot, self.at, self.budget, self.credit = 0, at, 0, 0
        self.work, self.matmuls, self.filler = [], [], None

    def add(self, cost, fn, *args, delay=0):
        self.work.append((self.slot + delay, cost, fn, args))

    def fill(self, gen):
        self.finish_filler()
        self.filler = gen

    def finish_filler(self):
        for _ in self.filler or ():
            pass
        self.filler = None

    def tick(self):
        self.slot += 1
        self.credit = min(self.credit, 0) + self.budget
        vals = []
        while self.credit > 0 and self.work and self.work[0][0] < self.slot:
            _, cost, fn, args = self.work.pop(0)
            vals += fn(*args)
            self.credit -= cost
        while self.credit > 0 and self.filler:
            unit = next(self.filler, None)
            if unit is None:
                self.filler = None
            else:
                self.credit -= unit[0]
                vals += unit[1]
        return _zero_after(vals) if vals else None

    def operand(self, op):
        return _unpack(_after(op, [self.tick() for _ in range(op.shape[0] // 64)], self.at))

    def issue(self):
        if self.matmuls:
            fn, args = self.matmuls.pop(0)
            fn(*args)

    def need(self, ref, row):
        last = [k for k, w in enumerate(self.work) if len(w[3]) > 2 and w[3][1] is ref and row <= w[3][2] < row + 64]
        for _ in range(last[-1] + 1 if last else 0):
            _, _, fn, args = self.work.pop(0)
            fn(*args)

    def force(self):
        if self.matmuls:
            self.issue()
        else:
            _, _, fn, args = self.work.pop(0)
            fn(*args)

    def drain(self):
        while self.work or self.matmuls:
            while self.work:
                _, _, fn, args = self.work.pop(0)
                fn(*args)
            while self.matmuls:
                self.issue()


def _head_reduce(v, op):
    v = op(v, pltpu.roll(v, 4, 0))
    return op(v, pltpu.roll(v, 2, 0))


def _dual_softmax(p):
    t = p.shape[1]
    p3 = p.reshape(8, 8, t)
    mx = _head_reduce(jnp.max(p3, axis=0), jnp.maximum)
    mn = _head_reduce(jnp.min(p3, axis=0), jnp.minimum)
    ep = jnp.exp2(p3 - mx[None])
    en = jnp.exp2(mn[None] - p3)
    sp = _head_reduce(jnp.sum(ep, axis=0), jnp.add)
    sn = _head_reduce(jnp.sum(en, axis=0), jnp.add)
    return ep * _recip(sp)[None], en * _recip(sn)[None]


def make_kernel(S=2048, D=1024, H=32, F=3584, T=512, olag=2, delay=4, WR=16, at=7, quiet=1, RR=128, UK=128, UD=64,
                b_early=200, phi_early=True, b_tile0=260, b_ln=145, b_ln2=170, b_ffn=150, b_alone=215, b_both=250, late_folds=0, route_at=(3, 2, 0), dynx=False, qpar=0, tail_delay=2, compact=False, pinned=('kv', 'q', 'o', 'ot'), full='2o', cw=11, co=70, cq=150, cf=105, strict=False, verbose=False,
                o_groups=((0, 1), (2, 3, 4), (5, 6)), scopes=False):
    Dh = D // H
    NT = S // T
    NG = D // 128
    NP = D // 64
    NB = NG // 2
    TH, DH = T // 2, D // 2
    FP = 256
    NF = F // FP
    n_dma = 64
    awaited = {(0, 0): 2, (1, 0): 3, (3, 0): 4, (5, 0): 5}
    prepared = {(0, 0): 1, (1, 0): 2, (1, 128): 3, (3, 0): 4, (3, 128): 5, (5, 0): 6, (5, 128): 7}

    def kernel(x_hbm, wqkv_hbm, wphi_hbm, wo_hbm, wr_hbm, wg_hbm, wu_hbm, wd_hbm, out_hbm,
               x_v, wqkv_v, wphi_v, wo_v, wr_v, wg_v, wu_v, wd_v, out_v,
               xn_v, xs_v, wkv_v, wq_v, wos_v, pT_v, kv_v, z_v, kvT_v, zb_v, r_v, o_v, xb_v, wrb_v, sem):

        def scope(name):
            return jax.named_scope(name) if scopes else contextlib.nullcontext()

        used = []

        def dma(src, dst):
            used.append(None)
            return pltpu.make_async_copy(src, dst, sem.at[len(used) - 1])

        def cols(ref, c, n):
            return ref.at[:, pl.ds(c, n)]

        def rows(ref, r, n):
            return ref.at[pl.ds(r, n), :]

        def x_copy(r, n):
            return dma(rows(x_hbm, r, n), rows(x_v, r, n))

        def kv_copies(gs):
            return [dma(cols(wqkv_hbm, j * D + g * 128, 128), cols(wqkv_v, j * D + g * 128, 128))
                    for g in gs for j in (1, 2)]

        early = [dma(wr_hbm, wr_v), x_copy(0, 128), x_copy(TH, 128)]
        phi_copy = dma(wphi_hbm, wphi_v)
        if phi_early:
            early.insert(1, phi_copy)
        stages = [([] if phi_early else [phi_copy]) + kv_copies([0]),
                  [x_copy(128, TH - 128), x_copy(TH + 128, TH - 128)],
                  kv_copies([1]),
                  kv_copies([2, 3]),
                  [x_copy(T, T)] + kv_copies([4, 5]),
                  kv_copies([6, 7]) + [x_copy(2 * T, T)],
                  [x_copy(3 * T, T), dma(cols(wqkv_hbm, 0, D), cols(wqkv_v, 0, D)), dma(wo_hbm, wo_v)],
                  [dma(wg_hbm, wg_v)], [dma(wu_hbm, wu_v), dma(wd_hbm, wd_v)]]
        for stage in [early] + stages:
            for c in stage:
                c.start()

        def wait_stage(j):
            with scope(f"w_{j}"):
                for c in stages[j]:
                    c.wait()
            if j > 1:
                bg.credit = -quiet * bg.budget

        summed = (0, 2, 3, 5, 6)

        lane = lax.broadcasted_iota(i32, (8, 128), 1)

        def layernorm(i, pieces):
            scores = r_v[i] if pieces[0] else jnp.zeros((8, 128), f32)
            for p in pieces:
                starts = (i * T + p * 16, i * T + TH + p * 16)
                x = jnp.concatenate([x_v[r:r + 16, :] for r in starts], axis=0).astype(f32)
                m32 = jnp.sum(x, axis=1, keepdims=True) * (1.0 / D)
                yield 75, [jnp.broadcast_to(m32[24:], (8, 128))]
                m = _rb(m32)
                d = x - m
                v32 = jnp.sum(d * d, axis=1, keepdims=True) * (1.0 / D) - (m32 - m) * (m32 - m)
                if compact:
                    vb = jnp.broadcast_to(v32, (32, 128))
                    vc = vb[0:8]
                    for q in range(1, 4):
                        vc = jnp.where(lane >= 32 * q, vb[8 * q:8 * q + 8], vc)
                    ic = _recip(jnp.minimum(_rb(jnp.sqrt(_rb(_rb(vc) + LN_EPS))), 1e38))
                    inv = jnp.concatenate([ic[:, 32 * q:32 * q + 1] for q in range(4)], axis=0)
                else:
                    inv = _recip(jnp.minimum(_rb(jnp.sqrt(_rb(_rb(v32) + LN_EPS))), 1e38))
                yield 190, [jnp.broadcast_to(inv[24:], (8, 128))]
                xn = d * inv
                a, b = xn[:16], xn[16:]
                vals = []
                for r, half in zip(starts, (a, b)):
                    packed = _pack(half)
                    xn_v[r // 2:r // 2 + 8, :] = packed
                    vals.append(packed)
                score = jnp.sum(xn * jnp.tile(wrb_v[...], (4, 1)), axis=1, keepdims=True)
                for q in range(4):
                    scores = jnp.where((lane >> 1) == 4 * p + q, score[8 * q:8 * q + 8], scores)
                yield 140, (vals if str(i) in full else [packed[:, D - 128:]]) + [scores]
                terms = _right_terms(a[:, :DH], b[:, :DH], a[:, DH:], b[:, DH:])
                row = (i * TH + p * 16) // 2
                vals = []
                for n, j in enumerate(summed):
                    packed = _pack(terms[j])
                    xs_v[n, row:row + 8, :] = packed
                    vals.append(packed)
                if p == pieces[-1]:
                    r_v[i] = scores
                yield 75, vals if str(i) in full else [packed[:, DH - 128:]]

        def token_term(t, j, l):
            def rows_at(start, stride):
                r = t * stride + start + l // 2
                return pl.ds(r if isinstance(r, int) else pl.multiple_of(r, 64), 64)
            if j == 1:
                return xn_v[rows_at(0, T // 2), :DH]
            if j == 4:
                return xn_v[rows_at(TH // 2, T // 2), DH:]
            return xs_v[summed.index(j), rows_at(0, TH // 2), :]

        with scope('w_early'):
            for c in early:
                c.wait()

        wr = jnp.broadcast_to(wr_v[...].astype(f32).reshape(1, D), (8, D))
        wrb_v[...] = wr
        nought = jnp.max(pltpu.bitcast(wr[:, 0:128], i32) & 0xFFFF) >> 31
        for name, ref in dict(kv=wkv_v.at[0], q=wq_v.at[0], o=wos_v.at[0], acc=kv_v.at[0], z=z_v.at[0], kvT=kvT_v.at[0],
                              zb=zb_v.at[0], ot=o_v.at[0, 0]).items():
            if name in pinned:
                ref[pl.ds(pl.multiple_of(nought * 8, 8), 8), 0:128] = jnp.zeros((8, 128), ref.dtype)
        for _ in layernorm(0, range(128 // 16)):
            pass
        if not phi_early:
            wait_stage(0)

        er = lax.broadcasted_iota(i32, (128, Dh), 0)
        ec = lax.broadcasted_iota(i32, (128, Dh), 1)
        eT = jnp.where(((er & 63) >> 1) == ec, 1.0, 0.0).astype(bf16)
        pT = _dot_nt(eT, wphi_v[...])
        rr = lax.broadcasted_iota(i32, (128, 128), 0)
        cc = lax.broadcasted_iota(i32, (128, 128), 1)
        same_head = (rr >> 6) * 2 + (rr & 1) == (cc >> 5)
        for g in range(NG):
            pT_v[:, g * 128:(g + 1) * 128] = _pack(jnp.where(same_head, pT[:, g * 128:(g + 1) * 128], 0.0))

        bg = _Interleaver(at)

        def fold(g, j):
            w = wqkv_v[:, j * D + g * 128: j * D + (g + 1) * 128]
            return _dot_nt(bg.operand(pT_v[:, g * 128:(g + 1) * 128]), w)

        def weight_terms(make, ref, row, top, bot, scale=None):
            top, bot = top.astype(f32), bot.astype(f32)
            if scale is not None:
                top, bot = top * scale, bot * scale
            vals = []
            for j, term in enumerate(make(top[:, :DH], top[:, DH:], bot[:, :DH], bot[:, DH:])):
                packed = _pack(term)
                ref[j, row:row + packed.shape[0], :] = packed
                vals.append(packed)
            return vals if ("k" if ref is wkv_v else "q" if ref is wq_v else "o") in full else [packed[-8:, DH - 128:]]

        def prepare_kv(g):
            wk = fold(g, 1)
            wv = _pack(wqkv_v[:, 2 * D + g * 128: 2 * D + (g + 1) * 128].T)
            for r in range(0, 64, WR):
                bg.add(cw * WR, weight_terms, _left_terms, wkv_v, g * 64 + 32 + r // 2, _unpack(wv[r // 2:(r + WR) // 2]), _unpack(wv[32 + r // 2:32 + (r + WR) // 2]))
            for r in range(0, 64, WR):
                bg.add(cw * WR, weight_terms, _left_terms, wkv_v, g * 64 + r // 2, wk[r:r + WR], wk[64 + r:64 + r + WR], LOG2E,
                       delay=delay)

        folded = []

        def prepare_q(g):
            folded.append(fold(g, 0))
            if g % 2 == 1:
                top, bot = folded[-2:]
                for r in range(0, 128, WR):
                    bg.add(cw * WR, weight_terms, _left_terms, wq_v, g * 32 - 32 + r // 2, top[r:r + WR], bot[r:r + WR],
                           LOG2E, delay=delay)

        def prepare_o():
            for b in range(NB):
                for r in range(0, 128, WR):
                    lo, hi = 2 * b * 128 + r, (2 * b + 1) * 128 + r
                    yield cw * WR, weight_terms(_right_terms, wos_v, b * 64 + r // 2, wo_v[lo:lo + WR, :], wo_v[hi:hi + WR, :])

        sel = {}

        def route():
            r = _rb(r_v[...])
            key = jnp.where(r != r, -jnp.inf, r)
            best = jnp.max(jnp.max(jnp.max(key, axis=0), axis=0, keepdims=True), axis=1, keepdims=True)
            tile, sub = (lax.broadcasted_iota(i32, r.shape, k) for k in range(2))
            row = tile * T + ((lane >> 2) & 1) * TH + (lane >> 3) * 16 + ((lane >> 1) & 1) * 8 + sub
            first = jnp.min(jnp.min(jnp.where(key == best, row, S - 1), axis=0))
            idx = jnp.clip(first, 0, S - 1)
            hit = (row == idx) & ((lane & 1) == 0)
            r_sel = jnp.sum(jnp.sum(jnp.sum(jnp.where(hit, r, 0.0), axis=0), axis=0, keepdims=True), axis=1, keepdims=True)
            wrd = jnp.broadcast_to(xn_v[pl.ds(idx // 2, 1), :], (128, D))
            bits = jnp.where(idx % 2 == 1, wrd & jnp.uint32(0xFFFF0000), wrd << 16)
            xb = pltpu.bitcast(bits, f32).T
            xb_v[0:D, :] = xb
            sel.update(idx=idx, gate=_rb(1.0 / (1.0 + jnp.exp(-r_sel))), y=None,
                       hrow=pl.multiple_of(D + nought * D, 8))
            yield 100, [xb[-8:]]

        def ffn_units():
            for c in range(NF):
                col = c * FP
                ag = au = None
                for k in range(0, D, 8):
                    xb = jnp.tile(xb_v[pl.ds(sel["hrow"] + (k - D), 8), :] if dynx else xb_v[k:k + 8, :], (1, FP // 128))
                    pg = wg_v[k:k + 8, col:col + FP].astype(f32) * xb
                    pu = wu_v[k:k + 8, col:col + FP].astype(f32) * xb
                    ag = pg if ag is None else ag + pg
                    au = pu if au is None else au + pu
                    if (k + 8) % UK == 0:
                        yield cf * UK // 64, [ag[:, 0:128], ag[:, 128:256], au[:, 0:128], au[:, 128:256]]
                gt = _rb(jnp.sum(ag, axis=0, keepdims=True))
                up = _rb(jnp.sum(au, axis=0, keepdims=True))
                h = jnp.broadcast_to(_rb(_rb(_silu(gt)) * up), (128, FP)).T
                xb_v[pl.ds(sel["hrow"], FP), :] = h
                yield 100, [h[-8:]]
                for k in range(0, FP, 8):
                    hk = xb_v[pl.ds(sel["hrow"] + k, 8), :]
                    pd = wd_v[col + k:col + k + 8, :].astype(f32) * jnp.tile(hk, (1, D // 128))
                    sel["y"] = pd if sel["y"] is None else sel["y"] + pd
                    if (k + 8) % UD == 0:
                        yield cf * UD // 32, [sel["y"][:, l * 128:(l + 1) * 128] for l in range(D // 128)]

        kr = lax.broadcasted_iota(i32, (64, 128), 0)
        kc = lax.broadcasted_iota(i32, (64, 128), 1)
        same = (kr >> 5) == (kc & 1)

        def strassen(product, done):
            def mul(j):
                m = product(j)
                bg.issue()
                return m
            m1 = mul(1)
            m3 = mul(3)
            done(1, 0, m1 + m3)
            m2 = mul(2)
            c22 = m2 - m1
            m4 = mul(4)
            done(0, 1, m2 + m4)
            c11 = m3 - m4
            m0 = mul(0)
            c22 = c22 + m0
            c11 = c11 + m0
            done(1, 1, c22 + mul(5))
            done(0, 0, c11 + mul(6))

        def project(w_ref, row, t, l):
            return lambda j: _dot_nt(bg.operand(w_ref[j, row:row + 64, :]), _unpack(token_term(t, j, l)))

        def k_feature(i, pr, pv, state):
            ep, en = _dual_softmax(pv[:64])
            phi = jnp.concatenate([ep.reshape(64, 128), en.reshape(64, 128)], axis=0)
            if not state and i > 0:
                state["z"] = z_v[pr]
            state["z"] = phi + state["z"] if state else phi
            state.setdefault("parts", []).append((pv[64:].astype(bf16), phi.astype(bf16)))
            if len(state["parts"]) == T // 128:
                if i < NT - 1:
                    z_v[pr] = state["z"]
                else:
                    zb_v[pr] = jnp.broadcast_to(jnp.sum(state["z"], axis=1, keepdims=True), (128, 128))
                bg.matmuls.append((k_accum, (i, pr, state["parts"])))
            return [state["parts"][-1][1][112:]]

        kv_done = set()

        def k_accum(i, pr, parts):
            kv = _dot_nt(jnp.concatenate([p[0] for p in parts], axis=1), jnp.concatenate([p[1] for p in parts], axis=1))
            if i > 0:
                kv = kv + kv_v[pr]
            if i < NT - 1:
                kv_v[pr] = kv
            else:
                kvT_v[pr] = _pack(jnp.where(same, kv, 0.0))
                kv_done.add(pr)

        if phi_early:
            wait_stage(0)
        prepare_kv(0)
        bg.drain()
        for i in range(NT):
            for g in range(NG):
                if 0 < i < NT - 1 and g == 0:
                    bg.fill(layernorm(i + 1, range(TH // 16)))
                if verbose:
                    print("block", i, g, "backlog", len(bg.work), len(bg.matmuls), "filler", bg.filler is not None)
                bg.need(wkv_v, g * 64)
                states = ({}, {})
                for l in range(0, TH, 128):
                    bg.budget = (b_early if g < 3 else b_tile0) if i == 0 else b_ln if i == 1 else b_ln2 if i == 2 else b_ffn
                    strassen(project(wkv_v, g * 64, i, l),
                             lambda rh, ch, c: bg.add(125, k_feature, i, 2 * g + rh, c, states[rh], delay=delay))
                    if (i, g, l) == (0, 0, 0):
                        wait_stage(1)
                        for _ in layernorm(0, range(128 // 16, TH // 16)):
                            pass
                        bg.drain()
                    if i == 0 and (g, l) in awaited:
                        wait_stage(awaited[g, l])
                    if (i, g, l) == (0, 3, 0):
                        bg.fill(layernorm(1, range(TH // 16)))
                    if i == 0 and (g, l) in prepared:
                        prepare_kv(prepared[g, l])
                    if (i, g, l) == route_at:
                        wait_stage(7)
                        bg.add(100, lambda: next(route())[1], delay=delay)
                    block = (i - 2) * NG + g
                    if block >= 0 and l == 0 and block % 2 == qpar and block // 2 < NG - late_folds:
                        prepare_q(block // 2)
            if i < NT - 1:
                bg.finish_filler()
            if i == 1:
                wait_stage(6)
            if i == 2:
                bg.fill(prepare_o())

        bg.finish_filler()
        wait_stage(8)
        bg.fill(ffn_units())
        for g in range(NG - late_folds, NG):
            prepare_q(g)
            bg.issue()
        idx = sel["idx"]
        for g in range(NG - late_folds, NG):
            prepare_q(g)
        t_sel = idx // T

        tiles = [lax.rem(t_sel + 1 + i, NT) for i in range(NT - 1)] + [t_sel]
        o_written = set()

        def q_feature(i, b, a, l, pq, state):
            pr = 4 * b + a
            ep, en = _dual_softmax(pq)
            zb = zb_v[pr]
            den = jnp.sum(ep * zb[0:64].reshape(8, 8, 128) + en * zb[64:128].reshape(8, 8, 128), axis=0)
            inv = _recip(_head_reduce(den, jnp.add) + 1e-6)
            phi = jnp.concatenate([ep.reshape(64, 128), en.reshape(64, 128)], axis=0).astype(bf16)
            state.setdefault(a, {})[l] = (phi, inv)
            if len(state[a]) == T // 128:
                bg.matmuls.append((q_attend, (i, b, a, state)))
            return [phi[112:]]

        def q_attend(i, b, a, state):
            phi, inv = (jnp.concatenate([state[a][l][k] for l in sorted(state[a])], axis=1) for k in range(2))
            num = _dot(_unpack(kvT_v[4 * b + a]), phi)
            sc = jnp.concatenate([jnp.broadcast_to(inv[0:1], (32, T)), jnp.broadcast_to(inv[1:2], (32, T))], axis=0)
            state.setdefault("o", {})[a] = num * sc
            if len(state["o"]) == 4:
                lo, hi = (jnp.concatenate([state["o"][k], state["o"][k + 1]], axis=0) for k in (0, 2))
                for js in o_groups:
                    bg.add(co * len(js), o_terms, i, b, js, lo, hi, delay=delay)

        def o_terms(i, b, js, lo, hi):
            terms = _left_terms(lo[:, :TH], hi[:, :TH], lo[:, TH:], hi[:, TH:])
            vals = []
            for j in js:
                packed = _pack(terms[j].astype(bf16).T)
                o_v[i, j, :, b * 128:(b + 1) * 128] = packed
                o_written.add((i, b, j))
                vals.append(packed if "t" in full else packed[-8:])
            return vals

        out_ready, out_copies = [], []

        def residual(i, s, r0, c0):
            t = tiles[i]
            last = i == NT - 1
            n = s.shape[0]
            gin = _unpack(xn_v[pl.ds(pl.multiple_of(t * (T // 2) + r0 // 2, n // 2), n // 2), c0:c0 + 128]).astype(f32)
            if last:
                upd = _rb(_rb(jnp.sum(sel["y"][:, c0:c0 + 128], axis=0, keepdims=True)) * sel["gate"])
                hit = lax.broadcasted_iota(i32, (n, 128), 0) == idx - t_sel * T - r0
                gin = jnp.where(hit, gin + upd, gin)
            row = pl.ds(pl.multiple_of(t * T + r0, n), n)
            out32 = x_v[row, c0:c0 + 128].astype(f32) + s * _silu(gin)
            res = out32.astype(bf16)
            out_v[row, c0:c0 + 128] = res
            if last and (r0 + n) % TH == 0:
                row = pl.ds(pl.multiple_of(t * T + r0 + n - TH, TH), TH)
                out_ready.append(dma(out_v.at[row, pl.ds(c0, 128)], out_hbm.at[row, pl.ds(c0, 128)]))
            elif not last and r0 + n == TH and c0 == DH - 128:
                row = pl.ds(pl.multiple_of(t * T, T), T)
                out_ready.append(dma(out_v.at[row, :], out_hbm.at[row, :]))
            return [_pack(out32)] if "r" in full else [res[-16:]]

        def send_ready():
            while out_ready:
                out_copies.append(out_ready.pop(0))
                out_copies[-1].start()

        def out_chunk(i, n):
            while not all((i, b, j) in o_written for b in range(NB) for j in range(7)):
                if verbose:
                    print("forced", i, n, len(bg.work), len(bg.matmuls))
                bg.force()
            if i == NT - 1:
                assert bg.filler is None or not strict
                bg.finish_filler()

            def product(j):
                m = _dot(bg.operand(o_v[i, j]), _unpack(wos_v[j, :, n * 128:(n + 1) * 128]))
                send_ready()
                return m

            def done(rh, ch, c):
                for r in range(0, TH, RR):
                    bg.add(9 * RR // 8, residual, i, c[r:r + RR], rh * TH + r, ch * DH + n * 128,
                           delay=tail_delay if (i, n) == (NT - 1, NB - 1) else delay)

            strassen(product, done)

        outs = [(i, n) for i in range(NT) for n in range(NB)]
        for i in range(NT):
            for b in range(NB):
                step = i * NB + b
                state = {}

                with_out = step >= NB + olag
                if verbose:
                    print("step", step, "backlog", len(bg.work), len(bg.matmuls), "filler", bg.filler is not None)
                bg.need(wq_v, b * 64)
                while not all(pr in kv_done for pr in range(4 * b, 4 * b + 4)):
                    bg.force()
                bg.budget = b_both if with_out else b_alone
                for l in range(0, TH, 128):
                    def done(rh, ch, c):
                        for a in range(2):
                            bg.add(cq, q_feature, i, b, 2 * rh + a, ch * TH + l, c[a * 64:(a + 1) * 64], state, delay=delay)

                    strassen(project(wq_v, b * 64, tiles[i], l), done)
                if with_out:
                    out_chunk(*outs.pop(0))
        while outs:
            out_chunk(*outs.pop(0))
        bg.drain()
        send_ready()
        assert len(used) <= n_dma
        with scope("w_out"):
            for c in out_copies:
                c.wait()

    scratch = [
        pltpu.VMEM((S, D), bf16),
        pltpu.VMEM((D, 3 * D), bf16),
        pltpu.VMEM((D, Dh), bf16),
        pltpu.VMEM((D, D), bf16),
        pltpu.VMEM((D,), bf16),
        pltpu.VMEM((D, F), bf16),
        pltpu.VMEM((D, F), bf16),
        pltpu.VMEM((F, D), bf16),
        pltpu.VMEM((S, D), bf16),
        pltpu.VMEM((S // 2, D), u32),
        pltpu.VMEM((5, S // 4, DH), u32),
        pltpu.VMEM((7, D // 2, DH), u32),
        pltpu.VMEM((7, D // 4, DH), u32),
        pltpu.VMEM((7, D // 4, DH), u32),
        pltpu.VMEM((64, D), u32),
        pltpu.VMEM((NP, 64, 128), f32),
        pltpu.VMEM((NP, 128, 128), f32),
        pltpu.VMEM((NP, 32, 128), u32),
        pltpu.VMEM((NP, 128, 128), f32),
        pltpu.VMEM((NT, 8, 128), f32),
        pltpu.VMEM((NT, 7, TH // 2, DH), u32),
        pltpu.VMEM((D + FP + 8, 128), f32),
        pltpu.VMEM((8, D), f32),
        pltpu.SemaphoreType.DMA((n_dma,)),
    ]
    return kernel, scratch


@jax.jit
def pallas_recurrent_scan__linear_kernel_hedgehog__moe_arch_mod__prompt_kernel(
    A_x: jax.Array,
    A_wqkv: jax.Array,
    A_w_phi: jax.Array,
    A_wo: jax.Array,
    B_x: jax.Array,
    B_w_r: jax.Array,
    B_w_gate: jax.Array,
    B_w_up: jax.Array,
    B_w_down: jax.Array,
):
    del B_x
    B, S, D = A_x.shape
    H, Dh, _ = A_w_phi.shape
    F = B_w_gate.shape[1]
    assert B == 1
    kernel, scratch = make_kernel(S=S, D=D, H=H, F=F)
    out = pl.pallas_call(
        kernel,
        out_shape=jax.ShapeDtypeStruct((S, D), A_x.dtype),
        in_specs=[pl.BlockSpec(memory_space=pl.ANY)] * 8,
        out_specs=pl.BlockSpec(memory_space=pl.ANY),
        scratch_shapes=scratch,
        compiler_params=pltpu.CompilerParams(
            vmem_limit_bytes=110 * 1024 * 1024),
        name="hedgehog_mod",
    )(A_x.reshape(S, D), A_wqkv, A_w_phi.reshape(H * Dh, Dh), A_wo, B_w_r, B_w_gate, B_w_up, B_w_down)
    return out.reshape(B, S, D)
```

```python
import contextlib

import jax
import jax.numpy as jnp
import numpy as np
from jax import lax
import jax.experimental.pallas as pl
import jax.experimental.pallas.tpu as pltpu

bf16, f32, u32, i32 = jnp.bfloat16, jnp.float32, jnp.uint32, jnp.int32
LOG2E = 1.4426950408889634
LN_EPS = float(np.asarray(1e-5, dtype=bf16))
NT_DIMS = (((1,), (1,)), ((), ()))


def _dot(a, b):
    return jnp.dot(a, b, preferred_element_type=f32)


def _dot_nt(a, b):
    return lax.dot_general(a, b, NT_DIMS, preferred_element_type=f32)


def _pack(x):
    return pltpu.bitcast(x.astype(bf16), u32)


def _unpack(x):
    return pltpu.bitcast(x, bf16)


def _zip(even, odd):
    return pltpu.bitcast(pltpu.pack_elementwise([even, odd], packed_dtype=bf16), u32)


def _unzip(x):
    return [pltpu.unpack_elementwise(x, index=k, packed_dtype=bf16, unpacked_dtype=f32) for k in range(2)]


def _shuffle_pack(x):
    return jnp.concatenate([_zip(x[r:r + 8], x[r + 8:r + 16]) for r in range(0, x.shape[0], 16)], axis=0)


def _rb(x):
    return x.astype(bf16).astype(f32)


def _recip(x):
    return pltpu.reciprocal(x, approx=False, full_range=False)


def _silu(x):
    h = 0.5 * x
    return h * jnp.tanh(h) + h


def _left_terms(a11, a12, a21, a22):
    return [a11 + a22, a21 + a22, a11, a22, a11 + a12, a21 - a11, a12 - a22]


def _right_terms(b11, b12, b21, b22):
    return [b11 + b22, b11, b12 - b22, b21 - b11, b22, b11 + b12, b21 + b22]


def _zero_after(vals):
    parts = []
    for v in vals:
        b = pltpu.bitcast(v, u32)
        parts += [b[r:r + 8, c:c + 128] for r in range(0, b.shape[0], 8) for c in range(0, b.shape[1], 128)]
    while len(parts) > 1:
        parts = [parts[k] | parts[k + 1] if k + 1 < len(parts) else parts[k] for k in range(0, len(parts), 2)]
    return (parts[0] >> 16) >> 16


def _after(op, zeros, at):
    n = op.shape[0] // len(zeros)
    parts, done = [], 0
    for k, zero in enumerate(zeros):
        r = k * n + at * 8
        if zero is not None:
            parts += [op[done:r]] if r > done else []
            parts.append(op[r:r + 8] | jnp.tile(zero, (1, op.shape[1] // 128)))
            done = r + 8
    parts += [op[done:]] if done < op.shape[0] else []
    return parts[0] if len(parts) == 1 else jnp.concatenate(parts, axis=0)


class _Interleaver:
    def __init__(self, at):
        self.slot, self.at, self.budget, self.credit = 0, at, 0, 0
        self.work, self.matmuls, self.filler = [], [], None

    def add(self, cost, fn, *args, delay=0):
        self.work.append((self.slot + delay, cost, fn, args))

    def fill(self, gen):
        self.finish_filler()
        self.filler = gen

    def finish_filler(self):
        for _ in self.filler or ():
            pass
        self.filler = None

    def tick(self):
        self.slot += 1
        self.credit = min(self.credit, 0) + self.budget
        vals = []
        while self.credit > 0 and self.work and self.work[0][0] < self.slot:
            _, cost, fn, args = self.work.pop(0)
            vals += fn(*args)
            self.credit -= cost
        while self.credit > 0 and self.filler:
            unit = next(self.filler, None)
            if unit is None:
                self.filler = None
            else:
                self.credit -= unit[0]
                vals += unit[1]
        return _zero_after(vals) if vals else None

    def operand(self, op):
        return _unpack(_after(op, [self.tick() for _ in range(op.shape[0] // 64)], self.at))

    def issue(self):
        if self.matmuls:
            fn, args = self.matmuls.pop(0)
            fn(*args)

    def need(self, ref, row):
        last = [k for k, w in enumerate(self.work) if len(w[3]) > 2 and w[3][1] is ref and row <= w[3][2] < row + 64]
        for _ in range(last[-1] + 1 if last else 0):
            _, _, fn, args = self.work.pop(0)
            fn(*args)

    def force(self):
        if self.matmuls:
            self.issue()
        else:
            _, _, fn, args = self.work.pop(0)
            fn(*args)

    def drain(self):
        while self.work or self.matmuls:
            while self.work:
                _, _, fn, args = self.work.pop(0)
                fn(*args)
            while self.matmuls:
                self.issue()


def _head_reduce(v, op):
    v = op(v, pltpu.roll(v, 4, 0))
    return op(v, pltpu.roll(v, 2, 0))


def _dual_softmax(p):
    t = p.shape[1]
    p3 = p.reshape(8, 8, t)
    mx = _head_reduce(jnp.max(p3, axis=0), jnp.maximum)
    mn = _head_reduce(jnp.min(p3, axis=0), jnp.minimum)
    ep = jnp.exp2(p3 - mx[None])
    en = jnp.exp2(mn[None] - p3)
    sp = _head_reduce(jnp.sum(ep, axis=0), jnp.add)
    sn = _head_reduce(jnp.sum(en, axis=0), jnp.add)
    return ep * _recip(sp)[None], en * _recip(sn)[None]


def make_kernel(S=2048, D=1024, H=32, F=3584, T=512, olag=2, delay=4, WR=16, at=7, quiet=1, RR=128, UK=128, UD=64,
                b_early=170, phi_early=True, b_tile0=220, b_ln=136, b_ln2=152, b_ffn=130, b_alone=200, b_both=240, late_folds=0, route_at=(3, 2, 0), dynx=False, qpar=0, tail_delay=2, compact=False, pinned=('kv', 'q', 'o', 'ot'), full='2o', cw=8, co=70, cq=150, ck=125, cl=(70, 170, 110, 65), cf=105, strict=False, verbose=False,
                o_groups=((0, 1), (2, 3, 4), (5, 6)), scopes=False):
    Dh = D // H
    NT = S // T
    NG = D // 128
    NP = D // 64
    NB = NG // 2
    TH, DH = T // 2, D // 2
    FP = 256
    NF = F // FP
    n_dma = 64
    n_ring = 12
    awaited = {(0, 0): 2, (1, 0): 3, (3, 0): 4, (5, 0): 5}
    prepared = {(0, 0): 1, (1, 0): 2, (1, 128): 3, (3, 0): 4, (3, 128): 5, (5, 0): 6, (5, 128): 7}

    def kernel(x_hbm, wqkv_hbm, wphi_hbm, wo_hbm, wr_hbm, wg_hbm, wu_hbm, wd_hbm, out_hbm,
               x_v, wqkv_v, wphi_v, wo_v, wr_v, wg_v, wu_v, wd_v, out_v,
               xn_v, xs_v, wkv_v, wq_v, wos_v, pT_v, kv_v, z_v, kvT_v, zb_v, r_v, o_v, xb_v, wrb_v, phi_v, sem):

        def scope(name):
            return jax.named_scope(name) if scopes else contextlib.nullcontext()

        used = []

        def dma(src, dst):
            used.append(None)
            return pltpu.make_async_copy(src, dst, sem.at[len(used) - 1])

        def cols(ref, c, n):
            return ref.at[:, pl.ds(c, n)]

        def rows(ref, r, n):
            return ref.at[pl.ds(r, n), :]

        def x_copy(r, n):
            return dma(rows(x_hbm, r, n), rows(x_v, r, n))

        def kv_copies(gs):
            return [dma(cols(wqkv_hbm, j * D + g * 128, 128), cols(wqkv_v, j * D + g * 128, 128))
                    for g in gs for j in (1, 2)]

        early = [dma(wr_hbm, wr_v), x_copy(0, 128), x_copy(TH, 128)]
        phi_copy = dma(wphi_hbm, wphi_v)
        if phi_early:
            early.insert(1, phi_copy)
        stages = [([] if phi_early else [phi_copy]) + kv_copies([0]),
                  [x_copy(128, TH - 128), x_copy(TH + 128, TH - 128)],
                  kv_copies([1]),
                  kv_copies([2, 3]),
                  [x_copy(T, T)] + kv_copies([4, 5]),
                  kv_copies([6, 7]) + [x_copy(2 * T, T)],
                  [x_copy(3 * T, T), dma(cols(wqkv_hbm, 0, D), cols(wqkv_v, 0, D)), dma(wo_hbm, wo_v)],
                  [dma(wg_hbm, wg_v)], [dma(wu_hbm, wu_v), dma(wd_hbm, wd_v)]]
        for stage in [early] + stages:
            for c in stage:
                c.start()

        def wait_stage(j):
            with scope(f"w_{j}"):
                for c in stages[j]:
                    c.wait()
            if j > 1:
                bg.credit = -quiet * bg.budget

        summed = (0, 2, 3, 5, 6)

        lane = lax.broadcasted_iota(i32, (8, 128), 1)

        def layernorm(i, pieces):
            scores = r_v[i] if pieces[0] else jnp.zeros((8, 128), f32)
            for p in pieces:
                starts = (i * T + p * 16, i * T + TH + p * 16)
                x = jnp.concatenate([h for r in starts for h in _unzip(pltpu.bitcast(x_v[r:r + 16, :], u32))], axis=0)
                m32 = jnp.sum(x, axis=1, keepdims=True) * (1.0 / D)
                yield cl[0], [jnp.broadcast_to(m32[24:], (8, 128))]
                m = _rb(m32)
                d = x - m
                v32 = jnp.sum(d * d, axis=1, keepdims=True) * (1.0 / D) - (m32 - m) * (m32 - m)
                if compact:
                    vb = jnp.broadcast_to(v32, (32, 128))
                    vc = vb[0:8]
                    for q in range(1, 4):
                        vc = jnp.where(lane >= 32 * q, vb[8 * q:8 * q + 8], vc)
                    ic = _recip(jnp.minimum(_rb(jnp.sqrt(_rb(_rb(vc) + LN_EPS))), 1e38))
                    inv = jnp.concatenate([ic[:, 32 * q:32 * q + 1] for q in range(4)], axis=0)
                else:
                    inv = _recip(jnp.minimum(_rb(jnp.sqrt(_rb(_rb(v32) + LN_EPS))), 1e38))
                yield cl[1], [jnp.broadcast_to(inv[24:], (8, 128))]
                xn = d * inv
                a, b = xn[:16], xn[16:]
                for r, half in zip(starts, (a, b)):
                    xn_v[r // 2:r // 2 + 8, :] = _zip(half[:8], half[8:])
                score = jnp.sum(xn * jnp.tile(wrb_v[...], (4, 1)), axis=1, keepdims=True)
                for q in range(4):
                    scores = jnp.where((lane >> 1) == 4 * p + q, score[8 * q:8 * q + 8], scores)
                yield cl[2], [scores]
                terms = _right_terms(a[:, :DH], b[:, :DH], a[:, DH:], b[:, DH:])
                row = (i * TH + p * 16) // 2
                for n, j in enumerate(summed):
                    xs_v[n, row:row + 8, :] = _zip(terms[j][:8], terms[j][8:])
                if p == pieces[-1]:
                    r_v[i] = scores
                yield cl[3], [terms[j][8:] for j in summed] if str(i) in full else [terms[-1][8:, DH - 128:]]

        def token_term(t, j, l):
            def rows_at(start, stride):
                r = t * stride + start + l // 2
                return pl.ds(r if isinstance(r, int) else pl.multiple_of(r, 64), 64)
            if j == 1:
                return xn_v[rows_at(0, T // 2), :DH]
            if j == 4:
                return xn_v[rows_at(TH // 2, T // 2), DH:]
            return xs_v[summed.index(j), rows_at(0, TH // 2), :]

        with scope('w_early'):
            for c in early:
                c.wait()

        wr = jnp.broadcast_to(wr_v[...].astype(f32).reshape(1, D), (8, D))
        wrb_v[...] = wr
        nought = jnp.max(pltpu.bitcast(wr[:, 0:128], i32) & 0xFFFF) >> 31
        for name, ref in dict(kv=wkv_v.at[0], q=wq_v.at[0], o=wos_v.at[0], acc=kv_v.at[0], z=z_v.at[0], kvT=kvT_v.at[0],
                              zb=zb_v.at[0], ot=o_v.at[0, 0], phi=phi_v.at[0]).items():
            if name in pinned:
                ref[pl.ds(pl.multiple_of(nought * 8, 8), 8), 0:128] = jnp.zeros((8, 128), ref.dtype)
        for _ in layernorm(0, range(128 // 16)):
            pass
        if not phi_early:
            wait_stage(0)

        er = lax.broadcasted_iota(i32, (128, Dh), 0)
        ec = lax.broadcasted_iota(i32, (128, Dh), 1)
        eT = jnp.where(((er & 63) >> 4) * 8 + (er & 7) == ec, 1.0, 0.0).astype(bf16)
        pT = _dot_nt(eT, wphi_v[...])
        rr = lax.broadcasted_iota(i32, (128, 128), 0)
        cc = lax.broadcasted_iota(i32, (128, 128), 1)
        same_head = (rr >> 6) * 2 + ((rr >> 3) & 1) == (cc >> 5)
        for g in range(NG):
            pT_v[:, g * 128:(g + 1) * 128] = _pack(jnp.where(same_head, pT[:, g * 128:(g + 1) * 128], 0.0))

        bg = _Interleaver(at)

        def fold(g, j):
            w = wqkv_v[:, j * D + g * 128: j * D + (g + 1) * 128]
            return _dot_nt(bg.operand(pT_v[:, g * 128:(g + 1) * 128]), w)

        def weight_terms(make, ref, row, top, bot, scale=None):
            top, bot = top.astype(f32), bot.astype(f32)
            if scale is not None:
                top, bot = top * scale, bot * scale
            terms = make(top[:, :DH], top[:, DH:], bot[:, :DH], bot[:, DH:])
            for j, term in enumerate(terms):
                ref[j, row:row + term.shape[0] // 2, :] = _shuffle_pack(term)
            if ("k" if ref is wkv_v else "q" if ref is wq_v else "o") in full:
                return [term[-8:] for term in terms]
            return [terms[-1][-8:, DH - 128:]]

        def value_terms(make, ref, row, top, bot):
            return weight_terms(make, ref, row, *(jnp.concatenate(_unzip(w), axis=0) for w in (top, bot)))

        def prepare_kv(g):
            wk = fold(g, 1)
            wv = pltpu.bitcast(wqkv_v[:, 2 * D + g * 128: 2 * D + (g + 1) * 128].T, u32)
            for r in range(0, 32, 8):
                bg.add(cw * 16, value_terms, _left_terms, wkv_v, g * 64 + 32 + r, wv[r:r + 8], wv[32 + r:40 + r])
            for r in range(0, 64, WR):
                bg.add(cw * WR, weight_terms, _left_terms, wkv_v, g * 64 + r // 2, wk[r:r + WR], wk[64 + r:64 + r + WR], LOG2E,
                       delay=delay)

        folded = []

        def prepare_q(g):
            folded.append(fold(g, 0))
            if g % 2 == 1:
                top, bot = folded[-2:]
                for r in range(0, 128, WR):
                    bg.add(cw * WR, weight_terms, _left_terms, wq_v, g * 32 - 32 + r // 2, top[r:r + WR], bot[r:r + WR],
                           LOG2E, delay=delay)

        def prepare_o():
            for b in range(NB):
                for r in range(0, 128, WR):
                    lo, hi = 2 * b * 128 + r, (2 * b + 1) * 128 + r
                    yield cw * WR, weight_terms(_right_terms, wos_v, b * 64 + r // 2, wo_v[lo:lo + WR, :], wo_v[hi:hi + WR, :])

        sel = {}

        def route():
            r = _rb(r_v[...])
            key = jnp.where(r != r, -jnp.inf, r)
            best = jnp.max(jnp.max(jnp.max(key, axis=0), axis=0, keepdims=True), axis=1, keepdims=True)
            tile, sub = (lax.broadcasted_iota(i32, r.shape, k) for k in range(2))
            row = tile * T + ((lane >> 2) & 1) * TH + (lane >> 3) * 16 + ((lane >> 1) & 1) + 2 * sub
            first = jnp.min(jnp.min(jnp.where(key == best, row, S - 1), axis=0))
            idx = jnp.clip(first, 0, S - 1)
            hit = (row == idx) & ((lane & 1) == 0)
            r_sel = jnp.sum(jnp.sum(jnp.sum(jnp.where(hit, r, 0.0), axis=0), axis=0, keepdims=True), axis=1, keepdims=True)
            wrd = jnp.broadcast_to(xn_v[pl.ds(idx // 2, 1), :], (128, D))
            bits = jnp.where(idx % 2 == 1, wrd & jnp.uint32(0xFFFF0000), wrd << 16)
            xb = pltpu.bitcast(bits, f32).T
            xb_v[0:D, :] = xb
            sel.update(idx=idx, gate=_rb(1.0 / (1.0 + jnp.exp(-r_sel))), y=None,
                       hrow=pl.multiple_of(D + nought * D, 8))
            yield 100, [xb[-8:]]

        def ffn_units():
            for c in range(NF):
                col = c * FP
                ag = au = None
                for k in range(0, D, 8):
                    xb = jnp.tile(xb_v[pl.ds(sel["hrow"] + (k - D), 8), :] if dynx else xb_v[k:k + 8, :], (1, FP // 128))
                    pg = wg_v[k:k + 8, col:col + FP].astype(f32) * xb
                    pu = wu_v[k:k + 8, col:col + FP].astype(f32) * xb
                    ag = pg if ag is None else ag + pg
                    au = pu if au is None else au + pu
                    if (k + 8) % UK == 0:
                        yield cf * UK // 64, [ag[:, 0:128], ag[:, 128:256], au[:, 0:128], au[:, 128:256]]
                gt = _rb(jnp.sum(ag, axis=0, keepdims=True))
                up = _rb(jnp.sum(au, axis=0, keepdims=True))
                h = jnp.broadcast_to(_rb(_rb(_silu(gt)) * up), (128, FP)).T
                xb_v[pl.ds(sel["hrow"], FP), :] = h
                yield 100, [h[-8:]]
                for k in range(0, FP, 8):
                    hk = xb_v[pl.ds(sel["hrow"] + k, 8), :]
                    pd = wd_v[col + k:col + k + 8, :].astype(f32) * jnp.tile(hk, (1, D // 128))
                    sel["y"] = pd if sel["y"] is None else sel["y"] + pd
                    if (k + 8) % UD == 0:
                        yield cf * UD // 32, [sel["y"][:, l * 128:(l + 1) * 128] for l in range(D // 128)]

        kr = lax.broadcasted_iota(i32, (64, 128), 0)
        kc = lax.broadcasted_iota(i32, (64, 128), 1)
        same = (kr >> 5) == ((kc >> 1) & 1)

        def strassen(product, done):
            def mul(j):
                m = product(j)
                bg.issue()
                return m
            m1 = mul(1)
            m3 = mul(3)
            done(1, 0, m1 + m3)
            m2 = mul(2)
            c22 = m2 - m1
            m4 = mul(4)
            done(0, 1, m2 + m4)
            c11 = m3 - m4
            m0 = mul(0)
            c22 = c22 + m0
            c11 = c11 + m0
            done(1, 1, c22 + mul(5))
            done(0, 0, c11 + mul(6))

        def project(w_ref, row, t, l):
            return lambda j: _dot_nt(bg.operand(w_ref[j, row:row + 64, :]), _unpack(token_term(t, j, l)))

        ring = {"next": 0, "busy": set()}

        def take_slot():
            slot = ring["next"] % n_ring
            assert slot not in ring["busy"]
            ring["busy"].add(slot)
            ring["next"] += 1
            return slot

        def k_feature(i, pr, pv, state):
            ep, en = _dual_softmax(pv[:64])
            phi = jnp.concatenate([ep.reshape(64, 128), en.reshape(64, 128)], axis=0)
            if not state:
                state.update(slot=take_slot(), n=0, z=phi + z_v[pr] if i > 0 else phi)
            else:
                state["z"] = state["z"] + phi
            col = state["n"] * 128
            phi_v[state["slot"], 0:64, col:col + 128] = _shuffle_pack(phi)
            phi_v[state["slot"], 64:96, col:col + 128] = _shuffle_pack(pv[64:])
            state["n"] += 1
            if state["n"] == T // 128:
                if i < NT - 1:
                    z_v[pr] = state["z"]
                else:
                    zb_v[pr] = jnp.broadcast_to(jnp.sum(state["z"], axis=1, keepdims=True), (128, 128))
                bg.matmuls.append((k_accum, (i, pr, state["slot"])))
            return [phi[120:]]

        kv_done = set()

        def k_accum(i, pr, slot):
            kv = _dot_nt(_unpack(phi_v[slot, 64:96, :]), _unpack(phi_v[slot, 0:64, :]))
            ring["busy"].remove(slot)
            if i > 0:
                kv = kv + kv_v[pr]
            if i < NT - 1:
                kv_v[pr] = kv
            else:
                kvT_v[pr] = _pack(jnp.where(same, kv, 0.0))
                kv_done.add(pr)

        if phi_early:
            wait_stage(0)
        prepare_kv(0)
        bg.drain()
        for i in range(NT):
            for g in range(NG):
                if 0 < i < NT - 1 and g == 0:
                    bg.fill(layernorm(i + 1, range(TH // 16)))
                if verbose:
                    print("block", i, g, "backlog", len(bg.work), len(bg.matmuls), "filler", bg.filler is not None)
                bg.need(wkv_v, g * 64)
                states = ({}, {})
                for l in range(0, TH, 128):
                    bg.budget = (b_early if g < 3 else b_tile0) if i == 0 else b_ln if i == 1 else b_ln2 if i == 2 else b_ffn
                    strassen(project(wkv_v, g * 64, i, l),
                             lambda rh, ch, c: bg.add(ck, k_feature, i, 2 * g + rh, c, states[rh], delay=delay))
                    if (i, g, l) == (0, 0, 0):
                        wait_stage(1)
                        for _ in layernorm(0, range(128 // 16, TH // 16)):
                            pass
                        bg.drain()
                    if i == 0 and (g, l) in awaited:
                        wait_stage(awaited[g, l])
                    if (i, g, l) == (0, 3, 0):
                        bg.fill(layernorm(1, range(TH // 16)))
                    if i == 0 and (g, l) in prepared:
                        prepare_kv(prepared[g, l])
                    if (i, g, l) == route_at:
                        wait_stage(7)
                        bg.add(100, lambda: next(route())[1], delay=delay)
                    block = (i - 2) * NG + g
                    if block >= 0 and l == 0 and block % 2 == qpar and block // 2 < NG - late_folds:
                        prepare_q(block // 2)
            if i < NT - 1:
                bg.finish_filler()
            if i == 1:
                wait_stage(6)
            if i == 2:
                bg.fill(prepare_o())

        bg.finish_filler()
        wait_stage(8)
        bg.fill(ffn_units())
        for g in range(NG - late_folds, NG):
            prepare_q(g)
            bg.issue()
        idx = sel["idx"]
        for g in range(NG - late_folds, NG):
            prepare_q(g)
        t_sel = idx // T

        tiles = [lax.rem(t_sel + 1 + i, NT) for i in range(NT - 1)] + [t_sel]
        o_written = set()

        def q_feature(i, b, a, l, pq, state):
            pr = 4 * b + a
            ep, en = _dual_softmax(pq)
            zb = zb_v[pr]
            den = jnp.sum(ep * zb[0:64].reshape(8, 8, 128) + en * zb[64:128].reshape(8, 8, 128), axis=0)
            inv = _recip(_head_reduce(den, jnp.add) + 1e-6)
            phi = jnp.concatenate([ep.reshape(64, 128), en.reshape(64, 128)], axis=0)
            if a not in state:
                state[a] = (take_slot(), {})
            slot, invs = state[a]
            phi_v[slot, 0:64, l:l + 128] = _shuffle_pack(phi)
            invs[l] = inv
            if len(invs) == T // 128:
                bg.matmuls.append((q_attend, (i, b, a, state)))
            return [phi[120:]]

        def q_attend(i, b, a, state):
            slot, invs = state[a]
            inv = jnp.concatenate([invs[l] for l in sorted(invs)], axis=1)
            num = _dot(_unpack(kvT_v[4 * b + a]), _unpack(phi_v[slot, 0:64, :]))
            ring["busy"].remove(slot)
            sc = jnp.concatenate([jnp.broadcast_to(inv[0:1], (32, T)), jnp.broadcast_to(inv[1:2], (32, T))], axis=0)
            state.setdefault("o", {})[a] = num * sc
            if len(state["o"]) == 4:
                lo, hi = (jnp.concatenate([state["o"][k], state["o"][k + 1]], axis=0) for k in (0, 2))
                for js in o_groups:
                    bg.add(co * len(js), o_terms, i, b, js, lo, hi, delay=delay)

        def o_terms(i, b, js, lo, hi):
            terms = _left_terms(lo[:, :TH], hi[:, :TH], lo[:, TH:], hi[:, TH:])
            vals = []
            for j in js:
                packed = _pack(terms[j].astype(bf16).T)
                o_v[i, j, :, b * 128:(b + 1) * 128] = packed
                o_written.add((i, b, j))
                vals.append(packed if "t" in full else packed[-8:])
            return vals

        out_ready, out_copies = [], []

        def residual(i, s, r0, c0):
            t = tiles[i]
            last = i == NT - 1
            n = s.shape[0]
            gin = _unpack(xn_v[pl.ds(pl.multiple_of(t * (T // 2) + r0 // 2, n // 2), n // 2), c0:c0 + 128]).astype(f32)
            if last:
                upd = _rb(_rb(jnp.sum(sel["y"][:, c0:c0 + 128], axis=0, keepdims=True)) * sel["gate"])
                hit = lax.broadcasted_iota(i32, (n, 128), 0) == idx - t_sel * T - r0
                gin = jnp.where(hit, gin + upd, gin)
            row = pl.ds(pl.multiple_of(t * T + r0, n), n)
            out32 = x_v[row, c0:c0 + 128].astype(f32) + s * _silu(gin)
            res = out32.astype(bf16)
            out_v[row, c0:c0 + 128] = res
            if last and (r0 + n) % TH == 0:
                row = pl.ds(pl.multiple_of(t * T + r0 + n - TH, TH), TH)
                out_ready.append(dma(out_v.at[row, pl.ds(c0, 128)], out_hbm.at[row, pl.ds(c0, 128)]))
            elif not last and r0 + n == TH and c0 == DH - 128:
                row = pl.ds(pl.multiple_of(t * T, T), T)
                out_ready.append(dma(out_v.at[row, :], out_hbm.at[row, :]))
            return [out32] if "r" in full else [out32[-8:]]

        def send_ready():
            while out_ready:
                out_copies.append(out_ready.pop(0))
                out_copies[-1].start()

        def out_chunk(i, n):
            while not all((i, b, j) in o_written for b in range(NB) for j in range(7)):
                if verbose:
                    print("forced", i, n, len(bg.work), len(bg.matmuls))
                bg.force()
            if i == NT - 1:
                assert bg.filler is None or not strict
                bg.finish_filler()

            def product(j):
                m = _dot(bg.operand(o_v[i, j]), _unpack(wos_v[j, :, n * 128:(n + 1) * 128]))
                send_ready()
                return m

            def done(rh, ch, c):
                for r in range(0, TH, RR):
                    bg.add(9 * RR // 8, residual, i, c[r:r + RR], rh * TH + r, ch * DH + n * 128,
                           delay=tail_delay if (i, n) == (NT - 1, NB - 1) else delay)

            strassen(product, done)

        outs = [(i, n) for i in range(NT) for n in range(NB)]
        for i in range(NT):
            for b in range(NB):
                step = i * NB + b
                state = {}

                with_out = step >= NB + olag
                if verbose:
                    print("step", step, "backlog", len(bg.work), len(bg.matmuls), "filler", bg.filler is not None)
                bg.need(wq_v, b * 64)
                while not all(pr in kv_done for pr in range(4 * b, 4 * b + 4)):
                    bg.force()
                bg.budget = b_both if with_out else b_alone
                for l in range(0, TH, 128):
                    def done(rh, ch, c):
                        for a in range(2):
                            bg.add(cq, q_feature, i, b, 2 * rh + a, ch * TH + l, c[a * 64:(a + 1) * 64], state, delay=delay)

                    strassen(project(wq_v, b * 64, tiles[i], l), done)
                if with_out:
                    out_chunk(*outs.pop(0))
        while outs:
            out_chunk(*outs.pop(0))
        bg.drain()
        send_ready()
        assert len(used) <= n_dma
        with scope("w_out"):
            for c in out_copies:
                c.wait()

    scratch = [
        pltpu.VMEM((S, D), bf16),
        pltpu.VMEM((D, 3 * D), bf16),
        pltpu.VMEM((D, Dh), bf16),
        pltpu.VMEM((D, D), bf16),
        pltpu.VMEM((D,), bf16),
        pltpu.VMEM((D, F), bf16),
        pltpu.VMEM((D, F), bf16),
        pltpu.VMEM((F, D), bf16),
        pltpu.VMEM((S, D), bf16),
        pltpu.VMEM((S // 2, D), u32),
        pltpu.VMEM((5, S // 4, DH), u32),
        pltpu.VMEM((7, D // 2, DH), u32),
        pltpu.VMEM((7, D // 4, DH), u32),
        pltpu.VMEM((7, D // 4, DH), u32),
        pltpu.VMEM((64, D), u32),
        pltpu.VMEM((NP, 64, 128), f32),
        pltpu.VMEM((NP, 128, 128), f32),
        pltpu.VMEM((NP, 32, 128), u32),
        pltpu.VMEM((NP, 128, 128), f32),
        pltpu.VMEM((NT, 8, 128), f32),
        pltpu.VMEM((NT, 7, TH // 2, DH), u32),
        pltpu.VMEM((D + FP + 8, 128), f32),
        pltpu.VMEM((8, D), f32),
        pltpu.VMEM((n_ring, 96, T), u32),
        pltpu.SemaphoreType.DMA((n_dma,)),
    ]
    return kernel, scratch


@jax.jit
def pallas_recurrent_scan__linear_kernel_hedgehog__moe_arch_mod__prompt_kernel(
    A_x: jax.Array,
    A_wqkv: jax.Array,
    A_w_phi: jax.Array,
    A_wo: jax.Array,
    B_x: jax.Array,
    B_w_r: jax.Array,
    B_w_gate: jax.Array,
    B_w_up: jax.Array,
    B_w_down: jax.Array,
):
    del B_x
    B, S, D = A_x.shape
    H, Dh, _ = A_w_phi.shape
    F = B_w_gate.shape[1]
    assert B == 1
    kernel, scratch = make_kernel(S=S, D=D, H=H, F=F)
    out = pl.pallas_call(
        kernel,
        out_shape=jax.ShapeDtypeStruct((S, D), A_x.dtype),
        in_specs=[pl.BlockSpec(memory_space=pl.ANY)] * 8,
        out_specs=pl.BlockSpec(memory_space=pl.ANY),
        scratch_shapes=scratch,
        compiler_params=pltpu.CompilerParams(
            vmem_limit_bytes=110 * 1024 * 1024,
            flags={"XLA_TPU_EVENLY_DISTRIBUTE_CRITICAL_NODES": True}),
        name="hedgehog_mod",
    )(A_x.reshape(S, D), A_wqkv, A_w_phi.reshape(H * Dh, Dh), A_wo, B_w_r, B_w_gate, B_w_up, B_w_down)
    return out.reshape(B, S, D)
```

```python
import contextlib

import jax
import jax.numpy as jnp
import numpy as np
from jax import lax
import jax.experimental.pallas as pl
import jax.experimental.pallas.tpu as pltpu

bf16, f32, u32, i32 = jnp.bfloat16, jnp.float32, jnp.uint32, jnp.int32
LOG2E = 1.4426950408889634
LN_EPS = float(np.asarray(1e-5, dtype=bf16))
NT_DIMS = (((1,), (1,)), ((), ()))


def _dot(a, b):
    return jnp.dot(a, b, preferred_element_type=f32)


def _dot_nt(a, b):
    return lax.dot_general(a, b, NT_DIMS, preferred_element_type=f32)


def _pack(x):
    return pltpu.bitcast(x.astype(bf16), u32)


def _unpack(x):
    return pltpu.bitcast(x, bf16)


def _rb(x):
    return x.astype(bf16).astype(f32)


def _recip(x):
    return pltpu.reciprocal(x, approx=False, full_range=False)


def _silu(x):
    h = 0.5 * x
    return h * jnp.tanh(h) + h


def _left_terms(a11, a12, a21, a22):
    return [a11 + a22, a21 + a22, a11, a22, a11 + a12, a21 - a11, a12 - a22]


def _right_terms(b11, b12, b21, b22):
    return [b11 + b22, b11, b12 - b22, b21 - b11, b22, b11 + b12, b21 + b22]


def _zero_after(vals):
    parts = []
    for v in vals:
        b = pltpu.bitcast(v, u32)
        parts += [b[r:r + 8, c:c + 128] for r in range(0, b.shape[0], 8) for c in range(0, b.shape[1], 128)]
    while len(parts) > 1:
        parts = [parts[k] | parts[k + 1] if k + 1 < len(parts) else parts[k] for k in range(0, len(parts), 2)]
    return (parts[0] >> 16) >> 16


def _after(op, zeros, at):
    n = op.shape[0] // len(zeros)
    parts, done = [], 0
    for k, zero in enumerate(zeros):
        r = k * n + at * 8
        if zero is not None:
            parts += [op[done:r]] if r > done else []
            parts.append(op[r:r + 8] | jnp.tile(zero, (1, op.shape[1] // 128)))
            done = r + 8
    parts += [op[done:]] if done < op.shape[0] else []
    return parts[0] if len(parts) == 1 else jnp.concatenate(parts, axis=0)


class _Interleaver:
    def __init__(self, at):
        self.slot, self.at, self.budget, self.credit = 0, at, 0, 0
        self.work, self.matmuls, self.filler = [], [], None

    def add(self, cost, fn, *args, delay=0):
        self.work.append((self.slot + delay, cost, fn, args))

    def fill(self, gen):
        self.finish_filler()
        self.filler = gen

    def finish_filler(self):
        for _ in self.filler or ():
            pass
        self.filler = None

    def tick(self):
        self.slot += 1
        self.credit = min(self.credit, 0) + self.budget
        vals = []
        while self.credit > 0 and self.work and self.work[0][0] < self.slot:
            _, cost, fn, args = self.work.pop(0)
            vals += fn(*args)
            self.credit -= cost
        while self.credit > 0 and self.filler:
            unit = next(self.filler, None)
            if unit is None:
                self.filler = None
            else:
                self.credit -= unit[0]
                vals += unit[1]
        return _zero_after(vals) if vals else None

    def operand(self, op):
        return _unpack(_after(op, [self.tick() for _ in range(op.shape[0] // 64)], self.at))

    def issue(self):
        if self.matmuls:
            fn, args = self.matmuls.pop(0)
            fn(*args)

    def need(self, ref, row):
        last = [k for k, w in enumerate(self.work) if len(w[3]) > 2 and w[3][1] is ref and row <= w[3][2] < row + 64]
        for _ in range(last[-1] + 1 if last else 0):
            _, _, fn, args = self.work.pop(0)
            fn(*args)

    def force(self):
        if self.matmuls:
            self.issue()
        else:
            _, _, fn, args = self.work.pop(0)
            fn(*args)

    def drain(self):
        while self.work or self.matmuls:
            while self.work:
                _, _, fn, args = self.work.pop(0)
                fn(*args)
            while self.matmuls:
                self.issue()


def _head_reduce(v, op):
    v = op(v, pltpu.roll(v, 4, 0))
    return op(v, pltpu.roll(v, 2, 0))


def _dual_softmax(p):
    t = p.shape[1]
    p3 = p.reshape(8, 8, t)
    mx = _head_reduce(jnp.max(p3, axis=0), jnp.maximum)
    mn = _head_reduce(jnp.min(p3, axis=0), jnp.minimum)
    ep = jnp.exp2(p3 - mx[None])
    en = jnp.exp2(mn[None] - p3)
    sp = _head_reduce(jnp.sum(ep, axis=0), jnp.add)
    sn = _head_reduce(jnp.sum(en, axis=0), jnp.add)
    return ep * _recip(sp)[None], en * _recip(sn)[None]


def make_kernel(S=2048, D=1024, H=32, F=3584, T=512, olag=2, delay=4, WR=16, at=7, quiet=1, RR=128, UK=128, UD=64,
                b_early=170, phi_early=True, b_tile0=220, b_ln=136, b_ln2=152, b_ffn=130, b_alone=200, b_both=240, late_folds=0, route_at=(3, 4, 0), dynx=False, qpar=0, tree=False, tail_delay=2, compact=False, pinned=('kv', 'q', 'o', 'ot'), full='2o', cw=8, co=70, cq=150, ck=125, cl=(70, 170, 110, 65), cf=105, strict=False, verbose=False,
                o_groups=((0, 1), (2, 3, 4), (5, 6)), scopes=False):
    Dh = D // H
    NT = S // T
    NG = D // 128
    NP = D // 64
    NB = NG // 2
    TH, DH = T // 2, D // 2
    FP = 256
    NF = F // FP
    n_dma = 64
    awaited = {(0, 0): 2, (1, 0): 3, (3, 0): 4, (5, 0): 5}
    prepared = {(0, 0): 1, (1, 0): 2, (1, 128): 3, (3, 0): 4, (3, 128): 5, (5, 0): 6, (5, 128): 7}

    def kernel(x_hbm, wqkv_hbm, wphi_hbm, wo_hbm, wr_hbm, wg_hbm, wu_hbm, wd_hbm, out_hbm,
               x_v, wqkv_v, wphi_v, wo_v, wr_v, wg_v, wu_v, wd_v, out_v,
               xn_v, xs_v, wkv_v, wq_v, wos_v, pT_v, kv_v, z_v, kvT_v, zb_v, r_v, o_v, xb_v, wrb_v, sem):

        def scope(name):
            return jax.named_scope(name) if scopes else contextlib.nullcontext()

        used = []

        def dma(src, dst):
            used.append(None)
            return pltpu.make_async_copy(src, dst, sem.at[len(used) - 1])

        def cols(ref, c, n):
            return ref.at[:, pl.ds(c, n)]

        def rows(ref, r, n):
            return ref.at[pl.ds(r, n), :]

        def x_copy(r, n):
            return dma(rows(x_hbm, r, n), rows(x_v, r, n))

        def kv_copies(gs):
            return [dma(cols(wqkv_hbm, j * D + g * 128, 128), cols(wqkv_v, j * D + g * 128, 128))
                    for g in gs for j in (1, 2)]

        early = [dma(wr_hbm, wr_v), x_copy(0, 128), x_copy(TH, 128)]
        phi_copy = dma(wphi_hbm, wphi_v)
        if phi_early:
            early.insert(1, phi_copy)
        stages = [([] if phi_early else [phi_copy]) + kv_copies([0]),
                  [x_copy(128, TH - 128), x_copy(TH + 128, TH - 128)],
                  kv_copies([1]),
                  kv_copies([2, 3]),
                  [x_copy(T, T)] + kv_copies([4, 5]),
                  kv_copies([6, 7]) + [x_copy(2 * T, T)],
                  [x_copy(3 * T, T), dma(cols(wqkv_hbm, 0, D), cols(wqkv_v, 0, D)), dma(wo_hbm, wo_v)],
                  [dma(wg_hbm, wg_v)], [dma(wu_hbm, wu_v), dma(wd_hbm, wd_v)]]
        for stage in [early] + stages:
            for c in stage:
                c.start()

        def wait_stage(j):
            with scope(f"w_{j}"):
                for c in stages[j]:
                    c.wait()
            if j > 1:
                bg.credit = -quiet * bg.budget

        summed = (0, 2, 3, 5, 6)

        lane = lax.broadcasted_iota(i32, (8, 128), 1)

        def layernorm(i, pieces):
            scores = r_v[i] if pieces[0] else jnp.zeros((8, 128), f32)
            for p in pieces:
                starts = (i * T + p * 16, i * T + TH + p * 16)
                x = jnp.concatenate([x_v[r:r + 16, :] for r in starts], axis=0).astype(f32)
                m32 = jnp.sum(x, axis=1, keepdims=True) * (1.0 / D)
                yield cl[0], [jnp.broadcast_to(m32[24:], (8, 128))]
                m = _rb(m32)
                d = x - m
                v32 = jnp.sum(d * d, axis=1, keepdims=True) * (1.0 / D) - (m32 - m) * (m32 - m)
                if compact:
                    vb = jnp.broadcast_to(v32, (32, 128))
                    vc = vb[0:8]
                    for q in range(1, 4):
                        vc = jnp.where(lane >= 32 * q, vb[8 * q:8 * q + 8], vc)
                    ic = _recip(jnp.minimum(_rb(jnp.sqrt(_rb(_rb(vc) + LN_EPS))), 1e38))
                    inv = jnp.concatenate([ic[:, 32 * q:32 * q + 1] for q in range(4)], axis=0)
                else:
                    inv = _recip(jnp.minimum(_rb(jnp.sqrt(_rb(_rb(v32) + LN_EPS))), 1e38))
                yield cl[1], [jnp.broadcast_to(inv[24:], (8, 128))]
                xn = d * inv
                a, b = xn[:16], xn[16:]
                for r, half in zip(starts, (a, b)):
                    xn_v[r // 2:r // 2 + 8, :] = _pack(half)
                score = jnp.sum(xn * jnp.tile(wrb_v[...], (4, 1)), axis=1, keepdims=True)
                for q in range(4):
                    scores = jnp.where((lane >> 1) == 4 * p + q, score[8 * q:8 * q + 8], scores)
                yield cl[2], [scores]
                terms = _right_terms(a[:, :DH], b[:, :DH], a[:, DH:], b[:, DH:])
                row = (i * TH + p * 16) // 2
                for n, j in enumerate(summed):
                    xs_v[n][row:row + 8, :] = _pack(terms[j])
                if p == pieces[-1]:
                    r_v[i] = scores
                yield cl[3], [terms[j][8:] for j in summed] if str(i) in full else [terms[-1][8:, DH - 128:]]

        def token_term(t, j, l):
            def rows_at(start, stride):
                r = t * stride + start + l // 2
                return pl.ds(r if isinstance(r, int) else pl.multiple_of(r, 64), 64)
            if j == 1:
                return xn_v[rows_at(0, T // 2), :DH]
            if j == 4:
                return xn_v[rows_at(TH // 2, T // 2), DH:]
            return xs_v[summed.index(j)][rows_at(0, TH // 2), :]

        with scope('w_early'):
            for c in early:
                c.wait()

        wr = jnp.broadcast_to(wr_v[...].astype(f32).reshape(1, D), (8, D))
        wrb_v[...] = wr
        nought = jnp.max(pltpu.bitcast(wr[:, 0:128], i32) & 0xFFFF) >> 31
        for ref in (*wkv_v, *wq_v, *wos_v, o_v.at[0, 0]):
            ref[pl.ds(pl.multiple_of(nought * 8, 8), 8), 0:128] = jnp.zeros((8, 128), u32)
        for _ in layernorm(0, range(128 // 16)):
            pass
        if not phi_early:
            wait_stage(0)

        er = lax.broadcasted_iota(i32, (128, Dh), 0)
        ec = lax.broadcasted_iota(i32, (128, Dh), 1)
        eT = jnp.where(((er & 63) >> 1) == ec, 1.0, 0.0).astype(bf16)
        pT = _dot_nt(eT, wphi_v[...])
        rr = lax.broadcasted_iota(i32, (128, 128), 0)
        cc = lax.broadcasted_iota(i32, (128, 128), 1)
        same_head = (rr >> 6) * 2 + (rr & 1) == (cc >> 5)
        for g in range(NG):
            pT_v[:, g * 128:(g + 1) * 128] = _pack(jnp.where(same_head, pT[:, g * 128:(g + 1) * 128], 0.0))

        bg = _Interleaver(at)

        def fold(g, j):
            w = wqkv_v[:, j * D + g * 128: j * D + (g + 1) * 128]
            return _dot_nt(bg.operand(pT_v[:, g * 128:(g + 1) * 128]), w)

        def weight_terms(make, ref, row, top, bot, scale=None):
            top, bot = top.astype(f32), bot.astype(f32)
            if scale is not None:
                top, bot = top * scale, bot * scale
            terms = make(top[:, :DH], top[:, DH:], bot[:, :DH], bot[:, DH:])
            for j, term in enumerate(terms):
                ref[j][row:row + term.shape[0] // 2, :] = _pack(term)
            if ("k" if ref is wkv_v else "q" if ref is wq_v else "o") in full:
                return [term[-8:] for term in terms]
            return [terms[-1][-8:, DH - 128:]]

        def prepare_kv(g):
            wk = fold(g, 1)
            wv = _pack(wqkv_v[:, 2 * D + g * 128: 2 * D + (g + 1) * 128].T)
            for r in range(0, 64, WR):
                bg.add(cw * WR, weight_terms, _left_terms, wkv_v, g * 64 + 32 + r // 2, _unpack(wv[r // 2:(r + WR) // 2]), _unpack(wv[32 + r // 2:32 + (r + WR) // 2]))
            for r in range(0, 64, WR):
                bg.add(cw * WR, weight_terms, _left_terms, wkv_v, g * 64 + r // 2, wk[r:r + WR], wk[64 + r:64 + r + WR], LOG2E,
                       delay=delay)

        folded = []

        def prepare_q(g):
            folded.append(fold(g, 0))
            if g % 2 == 1:
                top, bot = folded[-2:]
                for r in range(0, 128, WR):
                    bg.add(cw * WR, weight_terms, _left_terms, wq_v, g * 32 - 32 + r // 2, top[r:r + WR], bot[r:r + WR],
                           LOG2E, delay=delay)

        def prepare_o():
            for b in range(NB):
                for r in range(0, 128, WR):
                    lo, hi = 2 * b * 128 + r, (2 * b + 1) * 128 + r
                    yield cw * WR, weight_terms(_right_terms, wos_v, b * 64 + r // 2, wo_v[lo:lo + WR, :], wo_v[hi:hi + WR, :])

        sel = {}

        def route():
            r = _rb(r_v[...])
            key = jnp.where(r != r, -jnp.inf, r)
            best = jnp.max(jnp.max(jnp.max(key, axis=0), axis=0, keepdims=True), axis=1, keepdims=True)
            tile, sub = (lax.broadcasted_iota(i32, r.shape, k) for k in range(2))
            row = tile * T + ((lane >> 2) & 1) * TH + (lane >> 3) * 16 + ((lane >> 1) & 1) * 8 + sub
            first = jnp.min(jnp.min(jnp.where(key == best, row, S - 1), axis=0))
            idx = jnp.clip(first, 0, S - 1)
            hit = (row == idx) & ((lane & 1) == 0)
            r_sel = jnp.sum(jnp.sum(jnp.sum(jnp.where(hit, r, 0.0), axis=0), axis=0, keepdims=True), axis=1, keepdims=True)
            wrd = jnp.broadcast_to(xn_v[pl.ds(idx // 2, 1), :], (128, D))
            bits = jnp.where(idx % 2 == 1, wrd & jnp.uint32(0xFFFF0000), wrd << 16)
            xb = pltpu.bitcast(bits, f32).T
            xb_v[0:D, :] = xb
            sel.update(idx=idx, gate=_rb(1.0 / (1.0 + jnp.exp(-r_sel))), y=None,
                       hrow=pl.multiple_of(D + nought * D, 8))
            yield 100, [xb[-8:]]

        def ffn_units():
            for c in range(NF):
                col = c * FP
                ag = au = None
                for k in range(0, D, 8):
                    xb = jnp.tile(xb_v[pl.ds(sel["hrow"] + (k - D), 8), :] if dynx else xb_v[k:k + 8, :], (1, FP // 128))
                    pg = wg_v[k:k + 8, col:col + FP].astype(f32) * xb
                    pu = wu_v[k:k + 8, col:col + FP].astype(f32) * xb
                    ag = pg if ag is None else ag + pg
                    au = pu if au is None else au + pu
                    if (k + 8) % UK == 0:
                        yield cf * UK // 64, [ag[:, 0:128], ag[:, 128:256], au[:, 0:128], au[:, 128:256]]
                gt = _rb(jnp.sum(ag, axis=0, keepdims=True))
                up = _rb(jnp.sum(au, axis=0, keepdims=True))
                h = jnp.broadcast_to(_rb(_rb(_silu(gt)) * up), (128, FP)).T
                xb_v[pl.ds(sel["hrow"], FP), :] = h
                yield 100, [h[-8:]]
                for k in range(0, FP, 8):
                    hk = xb_v[pl.ds(sel["hrow"] + k, 8), :]
                    pd = wd_v[col + k:col + k + 8, :].astype(f32) * jnp.tile(hk, (1, D // 128))
                    sel["y"] = pd if sel["y"] is None else sel["y"] + pd
                    if (k + 8) % UD == 0:
                        yield cf * UD // 32, [sel["y"][:, l * 128:(l + 1) * 128] for l in range(D // 128)]

        kr = lax.broadcasted_iota(i32, (64, 128), 0)
        kc = lax.broadcasted_iota(i32, (64, 128), 1)
        same = (kr >> 5) == (kc & 1)

        def strassen(product, done):
            def mul(j):
                m = product(j)
                bg.issue()
                return m
            m1 = mul(1)
            m3 = mul(3)
            done(1, 0, m1 + m3)
            m2 = mul(2)
            c22 = m2 - m1
            m4 = mul(4)
            done(0, 1, m2 + m4)
            c11 = m3 - m4
            m0 = mul(0)
            c22 = c22 + m0
            c11 = c11 + m0
            done(1, 1, c22 + mul(5))
            done(0, 0, c11 + mul(6))

        def project(w_ref, row, t, l):
            return lambda j: _dot_nt(bg.operand(w_ref[j][row:row + 64, :]), _unpack(token_term(t, j, l)))

        def k_feature(i, pr, pv, state):
            ep, en = _dual_softmax(pv[:64])
            phi = jnp.concatenate([ep.reshape(64, 128), en.reshape(64, 128)], axis=0)
            if not state:
                state.update(parts=[], z=phi + z_v[pr] if i > 0 else phi)
            else:
                state["z"] = state["z"] + phi
            state["parts"].append((pv[64:].astype(bf16), phi.astype(bf16)))
            if len(state["parts"]) == T // 128:
                if i < NT - 1:
                    z_v[pr] = state["z"]
                else:
                    zb_v[pr] = jnp.broadcast_to(jnp.sum(state["z"], axis=1, keepdims=True), (128, 128))
                bg.matmuls.append((k_accum, (i, pr, state["parts"])))
            return [phi[120:]]

        kv_done = set()

        def k_accum(i, pr, parts):
            kvs = [_dot_nt(vT, phi) for vT, phi in parts]
            kv = (kvs[0] + kvs[1]) + (kvs[2] + kvs[3]) if tree else ((kvs[0] + kvs[1]) + kvs[2]) + kvs[3]
            if i > 0:
                kv = kv + kv_v[pr]
            if i < NT - 1:
                kv_v[pr] = kv
            else:
                kvT_v[pr] = _pack(jnp.where(same, kv, 0.0))
                kv_done.add(pr)

        if phi_early:
            wait_stage(0)
        prepare_kv(0)
        bg.drain()
        for i in range(NT):
            for g in range(NG):
                if 0 < i < NT - 1 and g == 0:
                    bg.fill(layernorm(i + 1, range(TH // 16)))
                if verbose:
                    print("block", i, g, "backlog", len(bg.work), len(bg.matmuls), "filler", bg.filler is not None)
                bg.need(wkv_v, g * 64)
                states = ({}, {})
                for l in range(0, TH, 128):
                    bg.budget = (b_early if g < 3 else b_tile0) if i == 0 else b_ln if i == 1 else b_ln2 if i == 2 else b_ffn
                    strassen(project(wkv_v, g * 64, i, l),
                             lambda rh, ch, c: bg.add(ck, k_feature, i, 2 * g + rh, c, states[rh], delay=delay))
                    if (i, g, l) == (0, 0, 0):
                        wait_stage(1)
                        for _ in layernorm(0, range(128 // 16, TH // 16)):
                            pass
                        bg.drain()
                    if i == 0 and (g, l) in awaited:
                        wait_stage(awaited[g, l])
                    if (i, g, l) == (0, 3, 0):
                        bg.fill(layernorm(1, range(TH // 16)))
                    if i == 0 and (g, l) in prepared:
                        prepare_kv(prepared[g, l])
                    if (i, g, l) == route_at:
                        wait_stage(7)
                        bg.add(100, lambda: next(route())[1], delay=delay)
                    block = (i - 2) * NG + g
                    if block >= 0 and l == 0 and block % 2 == qpar and block // 2 < NG - late_folds:
                        prepare_q(block // 2)
            if i < NT - 1:
                bg.finish_filler()
            if i == 1:
                wait_stage(6)
            if i == 2:
                bg.fill(prepare_o())

        bg.finish_filler()
        wait_stage(8)
        bg.fill(ffn_units())
        for g in range(NG - late_folds, NG):
            prepare_q(g)
            bg.issue()
        idx = sel["idx"]
        for g in range(NG - late_folds, NG):
            prepare_q(g)
        t_sel = idx // T

        tiles = [lax.rem(t_sel + 1 + i, NT) for i in range(NT - 1)] + [t_sel]
        o_written = set()

        def q_feature(i, b, a, l, pq, state):
            pr = 4 * b + a
            ep, en = _dual_softmax(pq)
            zb = zb_v[pr]
            den = jnp.sum(ep * zb[0:64].reshape(8, 8, 128) + en * zb[64:128].reshape(8, 8, 128), axis=0)
            inv = _recip(_head_reduce(den, jnp.add) + 1e-6)
            phi = jnp.concatenate([ep.reshape(64, 128), en.reshape(64, 128)], axis=0)
            state.setdefault(a, {})[l] = (phi.astype(bf16), inv)
            if len(state[a]) == T // 128:
                bg.matmuls.append((q_attend, (i, b, a, state)))
            return [phi[120:]]

        def q_attend(i, b, a, state):
            parts = [state[a][l] for l in sorted(state[a])]
            kvT = _unpack(kvT_v[4 * b + a])
            num = jnp.concatenate([_dot(kvT, phi) for phi, _ in parts], axis=1)
            inv = jnp.concatenate([inv for _, inv in parts], axis=1)
            sc = jnp.concatenate([jnp.broadcast_to(inv[0:1], (32, T)), jnp.broadcast_to(inv[1:2], (32, T))], axis=0)
            state.setdefault("o", {})[a] = num * sc
            if len(state["o"]) == 4:
                lo, hi = (jnp.concatenate([state["o"][k], state["o"][k + 1]], axis=0) for k in (0, 2))
                for js in o_groups:
                    bg.add(co * len(js), o_terms, i, b, js, lo, hi, delay=delay)

        def o_terms(i, b, js, lo, hi):
            terms = _left_terms(lo[:, :TH], hi[:, :TH], lo[:, TH:], hi[:, TH:])
            vals = []
            for j in js:
                packed = _pack(terms[j].astype(bf16).T)
                o_v[i, j, :, b * 128:(b + 1) * 128] = packed
                o_written.add((i, b, j))
                vals.append(packed if "t" in full else packed[-8:])
            return vals

        out_ready, out_copies = [], []

        def residual(i, s, r0, c0):
            t = tiles[i]
            last = i == NT - 1
            n = s.shape[0]
            gin = _unpack(xn_v[pl.ds(pl.multiple_of(t * (T // 2) + r0 // 2, n // 2), n // 2), c0:c0 + 128]).astype(f32)
            if last:
                upd = _rb(_rb(jnp.sum(sel["y"][:, c0:c0 + 128], axis=0, keepdims=True)) * sel["gate"])
                hit = lax.broadcasted_iota(i32, (n, 128), 0) == idx - t_sel * T - r0
                gin = jnp.where(hit, gin + upd, gin)
            row = pl.ds(pl.multiple_of(t * T + r0, n), n)
            out32 = x_v[row, c0:c0 + 128].astype(f32) + s * _silu(gin)
            res = out32.astype(bf16)
            out_v[row, c0:c0 + 128] = res
            if last and (r0 + n) % TH == 0:
                row = pl.ds(pl.multiple_of(t * T + r0 + n - TH, TH), TH)
                out_ready.append(dma(out_v.at[row, pl.ds(c0, 128)], out_hbm.at[row, pl.ds(c0, 128)]))
            elif not last and r0 + n == TH and c0 == DH - 128:
                row = pl.ds(pl.multiple_of(t * T, T), T)
                out_ready.append(dma(out_v.at[row, :], out_hbm.at[row, :]))
            return [out32] if "r" in full else [out32[-8:]]

        def send_ready():
            while out_ready:
                out_copies.append(out_ready.pop(0))
                out_copies[-1].start()

        def out_chunk(i, n):
            while not all((i, b, j) in o_written for b in range(NB) for j in range(7)):
                if verbose:
                    print("forced", i, n, len(bg.work), len(bg.matmuls))
                bg.force()
            if i == NT - 1:
                assert bg.filler is None or not strict
                bg.finish_filler()

            def product(j):
                m = _dot(bg.operand(o_v[i, j]), _unpack(wos_v[j][:, n * 128:(n + 1) * 128]))
                send_ready()
                return m

            def done(rh, ch, c):
                for r in range(0, TH, RR):
                    bg.add(9 * RR // 8, residual, i, c[r:r + RR], rh * TH + r, ch * DH + n * 128,
                           delay=tail_delay if (i, n) == (NT - 1, NB - 1) else delay)

            strassen(product, done)

        outs = [(i, n) for i in range(NT) for n in range(NB)]
        for i in range(NT):
            for b in range(NB):
                step = i * NB + b
                state = {}

                with_out = step >= NB + olag
                if verbose:
                    print("step", step, "backlog", len(bg.work), len(bg.matmuls), "filler", bg.filler is not None)
                bg.need(wq_v, b * 64)
                while not all(pr in kv_done for pr in range(4 * b, 4 * b + 4)):
                    bg.force()
                bg.budget = b_both if with_out else b_alone
                for l in range(0, TH, 128):
                    def done(rh, ch, c):
                        for a in range(2):
                            bg.add(cq, q_feature, i, b, 2 * rh + a, ch * TH + l, c[a * 64:(a + 1) * 64], state, delay=delay)

                    strassen(project(wq_v, b * 64, tiles[i], l), done)
                if with_out:
                    out_chunk(*outs.pop(0))
        while outs:
            out_chunk(*outs.pop(0))
        bg.drain()
        send_ready()
        assert len(used) <= n_dma
        with scope("w_out"):
            for c in out_copies:
                c.wait()

    scratch = [
        pltpu.VMEM((S, D), bf16),
        pltpu.VMEM((D, 3 * D), bf16),
        pltpu.VMEM((D, Dh), bf16),
        pltpu.VMEM((D, D), bf16),
        pltpu.VMEM((D,), bf16),
        pltpu.VMEM((D, F), bf16),
        pltpu.VMEM((D, F), bf16),
        pltpu.VMEM((F, D), bf16),
        pltpu.VMEM((S, D), bf16),
        pltpu.VMEM((S // 2, D), u32),
        [pltpu.VMEM((S // 4, DH), u32)] * 5,
        [pltpu.VMEM((D // 2, DH), u32)] * 7,
        [pltpu.VMEM((D // 4, DH), u32)] * 7,
        [pltpu.VMEM((D // 4, DH), u32)] * 7,
        pltpu.VMEM((64, D), u32),
        pltpu.VMEM((NP, 64, 128), f32),
        pltpu.VMEM((NP, 128, 128), f32),
        pltpu.VMEM((NP, 32, 128), u32),
        pltpu.VMEM((NP, 128, 128), f32),
        pltpu.VMEM((NT, 8, 128), f32),
        pltpu.VMEM((NT, 7, TH // 2, DH), u32),
        pltpu.VMEM((D + FP + 8, 128), f32),
        pltpu.VMEM((8, D), f32),
        pltpu.SemaphoreType.DMA((n_dma,)),
    ]
    return kernel, scratch


@jax.jit
def pallas_recurrent_scan__linear_kernel_hedgehog__moe_arch_mod__prompt_kernel(
    A_x: jax.Array,
    A_wqkv: jax.Array,
    A_w_phi: jax.Array,
    A_wo: jax.Array,
    B_x: jax.Array,
    B_w_r: jax.Array,
    B_w_gate: jax.Array,
    B_w_up: jax.Array,
    B_w_down: jax.Array,
):
    del B_x
    B, S, D = A_x.shape
    H, Dh, _ = A_w_phi.shape
    F = B_w_gate.shape[1]
    assert B == 1
    kernel, scratch = make_kernel(S=S, D=D, H=H, F=F)
    out = pl.pallas_call(
        kernel,
        out_shape=jax.ShapeDtypeStruct((S, D), A_x.dtype),
        in_specs=[pl.BlockSpec(memory_space=pl.ANY)] * 8,
        out_specs=pl.BlockSpec(memory_space=pl.ANY),
        scratch_shapes=scratch,
        compiler_params=pltpu.CompilerParams(
            vmem_limit_bytes=110 * 1024 * 1024),
        name="hedgehog_mod",
    )(A_x.reshape(S, D), A_wqkv, A_w_phi.reshape(H * Dh, Dh), A_wo, B_w_r, B_w_gate, B_w_up, B_w_down)
    return out.reshape(B, S, D)
```

```python
import jax
import jax.numpy as jnp
import numpy as np
from jax import lax
import jax.experimental.pallas as pl
import jax.experimental.pallas.tpu as pltpu

bf16, f32, u32, i32 = jnp.bfloat16, jnp.float32, jnp.uint32, jnp.int32
LOG2E = 1.4426950408889634
LN_EPS = float(np.asarray(1e-5, dtype=bf16))


def _dot(a, b):
    return jnp.dot(a, b, preferred_element_type=f32)


def _dot_nt(a, b):
    return lax.dot_general(a, b, (((1,), (1,)), ((), ())), preferred_element_type=f32)


def _pack(x):
    return pltpu.bitcast(x.astype(bf16), u32)


def _unpack(x):
    return pltpu.bitcast(x, bf16)


def _rb(x):
    return x.astype(bf16).astype(f32)


def _recip(x):
    return pltpu.reciprocal(x, approx=False, full_range=False)


def _silu(x):
    h = 0.5 * x
    return h * jnp.tanh(h) + h


def _left_terms(a11, a12, a21, a22):
    return [a11 + a22, a21 + a22, a11, a22, a11 + a12, a21 - a11, a12 - a22]


def _right_terms(b11, b12, b21, b22):
    return [b11 + b22, b11, b12 - b22, b21 - b11, b22, b11 + b12, b21 + b22]


def _strassen(product, done):
    m1 = product(1)
    m3 = product(3)
    done(1, 0, m1 + m3)
    m2 = product(2)
    c22 = m2 - m1
    m4 = product(4)
    done(0, 1, m2 + m4)
    c11 = m3 - m4
    m0 = product(0)
    c22 = c22 + m0
    c11 = c11 + m0
    done(1, 1, c22 + product(5))
    done(0, 0, c11 + product(6))


def _head_reduce(v, op):
    v = op(v, pltpu.roll(v, 4, 0))
    return op(v, pltpu.roll(v, 2, 0))


def _dual_softmax(p):
    p3 = p.reshape(8, 8, p.shape[1])
    mx = _head_reduce(jnp.max(p3, axis=0), jnp.maximum)
    mn = _head_reduce(jnp.min(p3, axis=0), jnp.minimum)
    ep = jnp.exp2(p3 - mx[None])
    en = jnp.exp2(mn[None] - p3)
    sp = _head_reduce(jnp.sum(ep, axis=0), jnp.add)
    sn = _head_reduce(jnp.sum(en, axis=0), jnp.add)
    return ep * _recip(sp)[None], en * _recip(sn)[None]


def _zero_after(vals):
    parts = []
    for v in vals:
        b = pltpu.bitcast(v, u32)
        parts += [b[r:r + 8, c:c + 128] for r in range(0, b.shape[0], 8) for c in range(0, b.shape[1], 128)]
    while len(parts) > 1:
        parts = [parts[k] | parts[k + 1] if k + 1 < len(parts) else parts[k] for k in range(0, len(parts), 2)]
    return (parts[0] >> 16) >> 16


class _Interleaver:
    def __init__(self, at):
        self.at, self.slot, self.budget, self.credit = at, 0, 0, 0
        self.work, self.matmuls, self.filler = [], [], None

    def add(self, cost, fn, *args, delay=0):
        self.work.append((self.slot + delay, cost, fn, args))

    def fill(self, gen):
        self.finish_filler()
        self.filler = gen

    def finish_filler(self):
        for _ in self.filler or ():
            pass
        self.filler = None

    def tick(self):
        self.slot += 1
        self.credit = min(self.credit, 0) + self.budget
        vals = []
        while self.credit > 0 and self.work and self.work[0][0] < self.slot:
            _, cost, fn, args = self.work.pop(0)
            vals += fn(*args)
            self.credit -= cost
        while self.credit > 0 and self.filler:
            unit = next(self.filler, None)
            if unit is None:
                self.filler = None
            else:
                self.credit -= unit[0]
                vals += unit[1]
                if unit[0] >= 200:
                    break
        return _zero_after(vals) if vals else None

    def operand(self, op):
        parts, done = [], 0
        for r in range(self.at * 8, op.shape[0], 64):
            zero = self.tick()
            if zero is not None:
                parts += [op[done:r]] if r > done else []
                parts.append(op[r:r + 8] | jnp.tile(zero, (1, op.shape[1] // 128)))
                done = r + 8
        parts += [op[done:]] if done < op.shape[0] else []
        return _unpack(parts[0] if len(parts) == 1 else jnp.concatenate(parts, axis=0))

    def issue(self):
        if self.matmuls:
            fn, args = self.matmuls.pop(0)
            fn(*args)

    def until(self, ready):
        while not ready():
            if self.matmuls:
                self.issue()
            else:
                _, _, fn, args = self.work.pop(0)
                fn(*args)

    def drain(self):
        self.until(lambda: not self.work and not self.matmuls)


def make_kernel(S, D, H, F, olag=2, delay=4, tail_delay=2, at=7, UK=128, UD=64, route_at=(3, 4, 0),
                b_early=170, b_tile0=220, b_ln=136, b_ln2=152, b_free=130, b_alone=200, b_both=240):
    T = 512
    Dh = D // H
    NT = S // T
    NG = D // 128
    NP = D // 64
    NB = NG // 2
    TH, DH = T // 2, D // 2
    FP = 256
    WR = 16
    n_dma = 64
    assert (Dh, NT, NG) == (32, 4, 8) and F % FP == 0
    awaited = {(0, 0): 2, (1, 0): 3, (3, 0): 4, (5, 0): 5}
    prepared = {(0, 0): 1, (1, 0): 2, (1, 128): 3, (3, 0): 4, (3, 128): 5, (5, 0): 6, (5, 128): 7}

    def kernel(x_hbm, wqkv_hbm, wphi_hbm, wo_hbm, wr_hbm, wg_hbm, wu_hbm, wd_hbm, out_hbm,
               x_v, wqkv_v, wphi_v, wo_v, wr_v, wg_v, wu_v, wd_v, out_v,
               xn_v, xs_v, wkv_v, wq_v, wos_v, pT_v, kv_v, z_v, kvT_v, zb_v, r_v, o_v, xb_v, wrb_v, sem):

        used = []

        def dma(src, dst):
            used.append(None)
            return pltpu.make_async_copy(src, dst, sem.at[len(used) - 1])

        def x_copy(r, n):
            return dma(x_hbm.at[pl.ds(r, n), :], x_v.at[pl.ds(r, n), :])

        def w_copy(c, n):
            return dma(wqkv_hbm.at[:, pl.ds(c, n)], wqkv_v.at[:, pl.ds(c, n)])

        def kv_copies(groups):
            return [w_copy(j * D + g * 128, 128) for g in groups for j in (1, 2)]

        first_copies = [dma(wr_hbm, wr_v), dma(wphi_hbm, wphi_v), x_copy(0, 128), x_copy(TH, 128)]
        stages = [kv_copies([0]),
                  [x_copy(128, TH - 128), x_copy(TH + 128, TH - 128)],
                  kv_copies([1]),
                  kv_copies([2, 3]),
                  [x_copy(T, T)] + kv_copies([4, 5]),
                  kv_copies([6, 7]) + [x_copy(2 * T, T)],
                  [x_copy(3 * T, T), w_copy(0, D), dma(wo_hbm, wo_v)],
                  [dma(wg_hbm, wg_v), dma(wu_hbm, wu_v), dma(wd_hbm, wd_v)]]
        for stage in [first_copies] + stages:
            for c in stage:
                c.start()

        bg = _Interleaver(at)
        emitted = set()

        def wait_stage(j):
            for c in stages[j]:
                c.wait()
            bg.credit = -bg.budget

        summed = (0, 2, 3, 5, 6)
        lane = lax.broadcasted_iota(i32, (8, 128), 1)

        def layernorm(i, pieces):
            scores = r_v[i] if pieces[0] else jnp.zeros((8, 128), f32)
            for p in pieces:
                starts = (i * T + p * 16, i * T + TH + p * 16)
                x = jnp.concatenate([x_v[r:r + 16, :] for r in starts], axis=0).astype(f32)
                m32 = jnp.sum(x, axis=1, keepdims=True) * (1.0 / D)
                yield 70, [jnp.broadcast_to(m32[24:], (8, 128))]
                m = _rb(m32)
                d = x - m
                v32 = jnp.sum(d * d, axis=1, keepdims=True) * (1.0 / D) - (m32 - m) * (m32 - m)
                inv = _recip(jnp.minimum(_rb(jnp.sqrt(_rb(_rb(v32) + LN_EPS))), 1e38))
                yield 170, [jnp.broadcast_to(inv[24:], (8, 128))]
                xn = d * inv
                a, b = xn[:16], xn[16:]
                for r, half in zip(starts, (a, b)):
                    xn_v[r // 2:r // 2 + 8, :] = _pack(half)
                score = jnp.sum(xn * jnp.tile(wrb_v[...], (4, 1)), axis=1, keepdims=True)
                for q in range(4):
                    scores = jnp.where((lane >> 1) == 4 * p + q, score[8 * q:8 * q + 8], scores)
                yield 110, [scores]
                terms = _right_terms(a[:, :DH], b[:, :DH], a[:, DH:], b[:, DH:])
                row = (i * TH + p * 16) // 2
                for n, j in enumerate(summed):
                    xs_v[n][row:row + 8, :] = _pack(terms[j])
                if p == pieces[-1]:
                    r_v[i] = scores
                yield 65, [terms[j][8:] for j in summed] if i == 2 else [terms[-1][8:, DH - 128:]]

        def token_term(t, j, l):
            def rows(start, stride):
                r = t * stride + start + l // 2
                return pl.ds(r if isinstance(r, int) else pl.multiple_of(r, 64), 64)
            if j == 1:
                return xn_v[rows(0, T // 2), :DH]
            if j == 4:
                return xn_v[rows(TH // 2, T // 2), DH:]
            return xs_v[summed.index(j)][rows(0, TH // 2), :]

        for c in first_copies:
            c.wait()
        wr = jnp.broadcast_to(wr_v[...].astype(f32).reshape(1, D), (8, D))
        wrb_v[...] = wr
        nought = jnp.max(pltpu.bitcast(wr[:, 0:128], i32) & 0xFFFF) >> 31
        for ref in (*wkv_v, *wq_v, *wos_v, o_v.at[0, 0]):
            ref[pl.ds(pl.multiple_of(nought * 8, 8), 8), 0:128] = jnp.zeros((8, 128), u32)
        for _ in layernorm(0, range(128 // 16)):
            pass

        er = lax.broadcasted_iota(i32, (128, Dh), 0)
        ec = lax.broadcasted_iota(i32, (128, Dh), 1)
        spread = jnp.where(((er & 63) >> 1) == ec, 1.0, 0.0).astype(bf16)
        pT = _dot_nt(spread, wphi_v[...])
        rr = lax.broadcasted_iota(i32, (128, 128), 0)
        cc = lax.broadcasted_iota(i32, (128, 128), 1)
        same_head = (rr >> 6) * 2 + (rr & 1) == (cc >> 5)
        for g in range(NG):
            pT_v[:, g * 128:(g + 1) * 128] = _pack(jnp.where(same_head, pT[:, g * 128:(g + 1) * 128], 0.0))

        def fold(g, j):
            w = wqkv_v[:, j * D + g * 128: j * D + (g + 1) * 128]
            return _dot_nt(bg.operand(pT_v[:, g * 128:(g + 1) * 128]), w)

        def weight_terms(tag, make, refs, row, top, bot, scale=None):
            top, bot = top.astype(f32), bot.astype(f32)
            if scale is not None:
                top, bot = top * scale, bot * scale
            terms = make(top[:, :DH], top[:, DH:], bot[:, :DH], bot[:, DH:])
            for ref, term in zip(refs, terms):
                ref[row:row + WR // 2, :] = _pack(term)
            emitted.add((tag, row))
            return [term[-8:] for term in terms] if tag == "o" else [terms[-1][-8:, DH - 128:]]

        def terms_ready(tag, row):
            return lambda: all((tag, r) in emitted for r in range(row, row + 64, WR // 2))

        def prepare_kv(g):
            wk = fold(g, 1)
            wv = _pack(wqkv_v[:, 2 * D + g * 128: 2 * D + (g + 1) * 128].T)
            for r in range(0, 32, WR // 2):
                bg.add(8 * WR, weight_terms, "kv", _left_terms, wkv_v, g * 64 + 32 + r,
                       _unpack(wv[r:r + WR // 2]), _unpack(wv[32 + r:32 + r + WR // 2]))
            for r in range(0, 64, WR):
                bg.add(8 * WR, weight_terms, "kv", _left_terms, wkv_v, g * 64 + r // 2,
                       wk[r:r + WR], wk[64 + r:64 + r + WR], LOG2E, delay=delay)

        folded = []

        def prepare_q(g):
            folded.append(fold(g, 0))
            if g % 2 == 1:
                top, bot = folded[-2:]
                for r in range(0, 128, WR):
                    bg.add(8 * WR, weight_terms, "q", _left_terms, wq_v, (g - 1) * 32 + r // 2,
                           top[r:r + WR], bot[r:r + WR], LOG2E, delay=delay)

        def prepare_o():
            for b in range(NB):
                for r in range(0, 128, WR):
                    lo, hi = 2 * b * 128 + r, (2 * b + 1) * 128 + r
                    yield 8 * WR, weight_terms("o", _right_terms, wos_v, b * 64 + r // 2,
                                               wo_v[lo:lo + WR, :], wo_v[hi:hi + WR, :])

        sel = {"y": None}

        def route():
            r = _rb(r_v[...])
            key = jnp.where(r != r, -jnp.inf, r)
            best = jnp.max(jnp.max(jnp.max(key, axis=0), axis=0, keepdims=True), axis=1, keepdims=True)
            tile, sub = (lax.broadcasted_iota(i32, r.shape, k) for k in range(2))
            row = tile * T + ((lane >> 2) & 1) * TH + (lane >> 3) * 16 + ((lane >> 1) & 1) * 8 + sub
            idx = jnp.clip(jnp.min(jnp.min(jnp.where(key == best, row, S - 1), axis=0)), 0, S - 1)
            hit = (row == idx) & ((lane & 1) == 0)
            r_sel = jnp.sum(jnp.sum(jnp.sum(jnp.where(hit, r, 0.0), axis=0), axis=0, keepdims=True),
                            axis=1, keepdims=True)
            word = jnp.broadcast_to(xn_v[pl.ds(idx // 2, 1), :], (128, D))
            bits = jnp.where(idx % 2 == 1, word & jnp.uint32(0xFFFF0000), word << 16)
            xb = pltpu.bitcast(bits, f32).T
            xb_v[0:D, :] = xb
            sel.update(idx=idx, gate=_rb(1.0 / (1.0 + jnp.exp(-r_sel))))
            return [xb[-8:]]

        def swiglu():
            h_row = pl.multiple_of(D + nought * D, 8)
            for col in range(0, F, FP):
                ag = au = None
                for k in range(0, D, 8):
                    xb = jnp.tile(xb_v[k:k + 8, :], (1, FP // 128))
                    pg = wg_v[k:k + 8, col:col + FP].astype(f32) * xb
                    pu = wu_v[k:k + 8, col:col + FP].astype(f32) * xb
                    ag = pg if ag is None else ag + pg
                    au = pu if au is None else au + pu
                    if (k + 8) % UK == 0:
                        yield 105 * UK // 64, [ag[:, 0:128], ag[:, 128:256], au[:, 0:128], au[:, 128:256]]
                gate = _rb(jnp.sum(ag, axis=0, keepdims=True))
                up = _rb(jnp.sum(au, axis=0, keepdims=True))
                h = jnp.broadcast_to(_rb(_rb(_silu(gate)) * up), (128, FP)).T
                xb_v[pl.ds(h_row, FP), :] = h
                yield 100, [h[-8:]]
                for k in range(0, FP, 8):
                    hk = xb_v[pl.ds(h_row + k, 8), :]
                    pd = wd_v[col + k:col + k + 8, :].astype(f32) * jnp.tile(hk, (1, D // 128))
                    sel["y"] = pd if sel["y"] is None else sel["y"] + pd
                    if (k + 8) % UD == 0:
                        yield 105 * UD // 32, [sel["y"][:, c:c + 128] for c in range(0, D, 128)]

        kr = lax.broadcasted_iota(i32, (64, 128), 0)
        kc = lax.broadcasted_iota(i32, (64, 128), 1)
        same = (kr >> 5) == (kc & 1)

        def project(refs, row, t, l):
            def product(j):
                m = _dot_nt(bg.operand(refs[j][row:row + 64, :]), _unpack(token_term(t, j, l)))
                bg.issue()
                return m
            return product

        def k_feature(i, pr, pv, state):
            ep, en = _dual_softmax(pv[:64])
            phi = jnp.concatenate([ep.reshape(64, 128), en.reshape(64, 128)], axis=0)
            if not state:
                state.update(parts=[], z=phi + z_v[pr] if i > 0 else phi)
            else:
                state["z"] = state["z"] + phi
            state["parts"].append((pv[64:].astype(bf16), phi.astype(bf16)))
            if len(state["parts"]) == T // 128:
                if i < NT - 1:
                    z_v[pr] = state["z"]
                else:
                    zb_v[pr] = jnp.broadcast_to(jnp.sum(state["z"], axis=1, keepdims=True), (128, 128))
                bg.matmuls.append((k_accumulate, (i, pr, state["parts"])))
            return [phi[120:]]

        def k_accumulate(i, pr, parts):
            kv = None
            for part in [_dot_nt(vT, phi) for vT, phi in parts]:
                kv = part if kv is None else kv + part
            if i > 0:
                kv = kv + kv_v[pr]
            if i < NT - 1:
                kv_v[pr] = kv
            else:
                kvT_v[pr] = _pack(jnp.where(same, kv, 0.0))
                emitted.add(("kvT", pr))

        wait_stage(0)
        prepare_kv(0)
        bg.drain()
        for i in range(NT):
            for g in range(NG):
                if 0 < i < NT - 1 and g == 0:
                    bg.fill(layernorm(i + 1, range(TH // 16)))
                bg.until(terms_ready("kv", g * 64))
                states = ({}, {})
                for l in range(0, TH, 128):
                    bg.budget = ((b_early if g < 3 else b_tile0), b_ln, b_ln2, b_free)[i]
                    _strassen(project(wkv_v, g * 64, i, l),
                              lambda rh, ch, c: bg.add(125, k_feature, i, 2 * g + rh, c, states[rh], delay=delay))
                    if (i, g, l) == (0, 0, 0):
                        wait_stage(1)
                        for _ in layernorm(0, range(128 // 16, TH // 16)):
                            pass
                        bg.drain()
                    if i == 0 and (g, l) in awaited:
                        wait_stage(awaited[g, l])
                    if (i, g, l) == (0, 3, 0):
                        bg.fill(layernorm(1, range(TH // 16)))
                    if i == 0 and (g, l) in prepared:
                        prepare_kv(prepared[g, l])
                    if (i, g, l) == route_at:
                        bg.add(100, route, delay=delay)
                    if i >= 2 and l == 0 and g % 2 == 0:
                        prepare_q(((i - 2) * NG + g) // 2)
            bg.finish_filler()
            if i == 1:
                wait_stage(6)
            if i == 2:
                bg.fill(prepare_o())

        bg.until(lambda: "idx" in sel)
        wait_stage(7)
        bg.fill(swiglu())
        idx = sel["idx"]
        t_sel = idx // T
        tiles = [lax.rem(t_sel + 1 + i, NT) for i in range(NT - 1)] + [t_sel]

        def q_feature(i, b, a, l, pq, state):
            ep, en = _dual_softmax(pq)
            zb = zb_v[4 * b + a]
            den = jnp.sum(ep * zb[0:64].reshape(8, 8, 128) + en * zb[64:128].reshape(8, 8, 128), axis=0)
            inv = _recip(_head_reduce(den, jnp.add) + 1e-6)
            phi = jnp.concatenate([ep.reshape(64, 128), en.reshape(64, 128)], axis=0)
            state.setdefault(a, {})[l] = (phi.astype(bf16), inv)
            if len(state[a]) == T // 128:
                bg.matmuls.append((q_attend, (i, b, a, state)))
            return [phi[120:]]

        def q_attend(i, b, a, state):
            parts = [state[a][l] for l in sorted(state[a])]
            kvT = _unpack(kvT_v[4 * b + a])
            num = jnp.concatenate([_dot(kvT, phi) for phi, _ in parts], axis=1)
            inv = jnp.concatenate([inv for _, inv in parts], axis=1)
            scale = jnp.concatenate([jnp.broadcast_to(inv[h:h + 1], (32, T)) for h in range(2)], axis=0)
            state.setdefault("o", {})[a] = num * scale
            if len(state["o"]) == 4:
                lo, hi = (jnp.concatenate([state["o"][k], state["o"][k + 1]], axis=0) for k in (0, 2))
                for js in ((0, 1), (2, 3, 4), (5, 6)):
                    bg.add(70 * len(js), o_terms, i, b, js, lo, hi, delay=delay)

        def o_terms(i, b, js, lo, hi):
            terms = _left_terms(lo[:, :TH], hi[:, :TH], lo[:, TH:], hi[:, TH:])
            vals = []
            for j in js:
                packed = _pack(terms[j].astype(bf16).T)
                o_v[i, j, :, b * 128:(b + 1) * 128] = packed
                emitted.add(("ot", i, b, j))
                vals.append(packed[-8:])
            return vals

        out_ready, out_copies = [], []

        def residual(i, s, r0, c0):
            t, n, last = tiles[i], s.shape[0], i == NT - 1
            gin = _unpack(xn_v[pl.ds(pl.multiple_of(t * (T // 2) + r0 // 2, n // 2), n // 2), c0:c0 + 128]).astype(f32)
            if last:
                bg.finish_filler()
                upd = _rb(_rb(jnp.sum(sel["y"][:, c0:c0 + 128], axis=0, keepdims=True)) * sel["gate"])
                hit = lax.broadcasted_iota(i32, (n, 128), 0) == idx - t_sel * T - r0
                gin = jnp.where(hit, gin + upd, gin)
            row = pl.ds(pl.multiple_of(t * T + r0, n), n)
            res = x_v[row, c0:c0 + 128].astype(f32) + s * _silu(gin)
            out_v[row, c0:c0 + 128] = res.astype(bf16)
            if last and (r0 + n) % TH == 0:
                row = pl.ds(pl.multiple_of(t * T + r0 + n - TH, TH), TH)
                out_ready.append(dma(out_v.at[row, pl.ds(c0, 128)], out_hbm.at[row, pl.ds(c0, 128)]))
            elif not last and r0 + n == TH and c0 == DH - 128:
                row = pl.ds(pl.multiple_of(t * T, T), T)
                out_ready.append(dma(out_v.at[row, :], out_hbm.at[row, :]))
            return [res[-8:]]

        def send_ready():
            while out_ready:
                out_copies.append(out_ready.pop(0))
                out_copies[-1].start()

        def out_chunk(i, n):
            bg.until(lambda: all(("ot", i, b, j) in emitted for b in range(NB) for j in range(7)))

            def product(j):
                m = _dot(bg.operand(o_v[i, j]), _unpack(wos_v[j][:, n * 128:(n + 1) * 128]))
                send_ready()
                bg.issue()
                return m

            def done(rh, ch, c):
                for r in range(0, TH, 128):
                    bg.add(144, residual, i, c[r:r + 128], rh * TH + r, ch * DH + n * 128,
                           delay=tail_delay if (i, n) == (NT - 1, NB - 1) else delay)

            _strassen(product, done)

        chunks = [(i, n) for i in range(NT) for n in range(NB)]
        for i in range(NT):
            for b in range(NB):
                state = {}
                with_out = i * NB + b >= NB + olag
                bg.until(terms_ready("q", b * 64))
                bg.until(lambda: all(("kvT", pr) in emitted for pr in range(4 * b, 4 * b + 4)))
                bg.budget = b_both if with_out else b_alone
                for l in range(0, TH, 128):
                    def done(rh, ch, c):
                        for a in range(2):
                            bg.add(150, q_feature, i, b, 2 * rh + a, ch * TH + l, c[a * 64:(a + 1) * 64], state,
                                   delay=delay)

                    _strassen(project(wq_v, b * 64, tiles[i], l), done)
                if with_out:
                    out_chunk(*chunks.pop(0))
        while chunks:
            out_chunk(*chunks.pop(0))
        bg.drain()
        send_ready()
        assert len(used) <= n_dma
        for c in out_copies:
            c.wait()

    scratch = [
        pltpu.VMEM((S, D), bf16),
        pltpu.VMEM((D, 3 * D), bf16),
        pltpu.VMEM((D, Dh), bf16),
        pltpu.VMEM((D, D), bf16),
        pltpu.VMEM((D,), bf16),
        pltpu.VMEM((D, F), bf16),
        pltpu.VMEM((D, F), bf16),
        pltpu.VMEM((F, D), bf16),
        pltpu.VMEM((S, D), bf16),
        pltpu.VMEM((S // 2, D), u32),
        [pltpu.VMEM((S // 4, DH), u32)] * 5,
        [pltpu.VMEM((D // 2, DH), u32)] * 7,
        [pltpu.VMEM((D // 4, DH), u32)] * 7,
        [pltpu.VMEM((D // 4, DH), u32)] * 7,
        pltpu.VMEM((64, D), u32),
        pltpu.VMEM((NP, 64, 128), f32),
        pltpu.VMEM((NP, 128, 128), f32),
        pltpu.VMEM((NP, 32, 128), u32),
        pltpu.VMEM((NP, 128, 128), f32),
        pltpu.VMEM((NT, 8, 128), f32),
        pltpu.VMEM((NT, 7, TH // 2, DH), u32),
        pltpu.VMEM((D + FP, 128), f32),
        pltpu.VMEM((8, D), f32),
        pltpu.SemaphoreType.DMA((n_dma,)),
    ]
    return kernel, scratch


@jax.jit
def pallas_recurrent_scan__linear_kernel_hedgehog__moe_arch_mod__prompt_kernel(
    A_x: jax.Array,
    A_wqkv: jax.Array,
    A_w_phi: jax.Array,
    A_wo: jax.Array,
    B_x: jax.Array,
    B_w_r: jax.Array,
    B_w_gate: jax.Array,
    B_w_up: jax.Array,
    B_w_down: jax.Array,
):
    del B_x
    B, S, D = A_x.shape
    H, Dh, _ = A_w_phi.shape
    F = B_w_gate.shape[1]
    assert B == 1
    kernel, scratch = make_kernel(S=S, D=D, H=H, F=F)
    out = pl.pallas_call(
        kernel,
        out_shape=jax.ShapeDtypeStruct((S, D), A_x.dtype),
        in_specs=[pl.BlockSpec(memory_space=pl.ANY)] * 8,
        out_specs=pl.BlockSpec(memory_space=pl.ANY),
        scratch_shapes=scratch,
        compiler_params=pltpu.CompilerParams(
            vmem_limit_bytes=110 * 1024 * 1024),
        name="hedgehog_mod",
    )(A_x.reshape(S, D), A_wqkv, A_w_phi.reshape(H * Dh, Dh), A_wo, B_w_r, B_w_gate, B_w_up, B_w_down)
    return out.reshape(B, S, D)
```

```python
import jax
import jax.numpy as jnp
import numpy as np
from jax import lax
import jax.experimental.pallas as pl
import jax.experimental.pallas.tpu as pltpu

bf16, f32, u32, i32 = jnp.bfloat16, jnp.float32, jnp.uint32, jnp.int32
LOG2E = 1.4426950408889634
LN_EPS = float(np.asarray(1e-5, dtype=bf16))


def _dot(a, b):
    return jnp.dot(a, b, preferred_element_type=f32)


def _dot_nt(a, b):
    return lax.dot_general(a, b, (((1,), (1,)), ((), ())), preferred_element_type=f32)


def _pack(x):
    return pltpu.bitcast(x.astype(bf16), u32)


def _unpack(x):
    return pltpu.bitcast(x, bf16)


def _rb(x):
    return x.astype(bf16).astype(f32)


def _recip(x):
    return pltpu.reciprocal(x, approx=False, full_range=False)


def _silu(x):
    h = 0.5 * x
    return h * jnp.tanh(h) + h


def _left_terms(a11, a12, a21, a22):
    return [a11 + a22, a21 + a22, a11, a22, a11 + a12, a21 - a11, a12 - a22]


def _right_terms(b11, b12, b21, b22):
    return [b11 + b22, b11, b12 - b22, b21 - b11, b22, b11 + b12, b21 + b22]


def _strassen(product, done):
    m1 = product(1)
    m3 = product(3)
    done(1, 0, m1 + m3)
    m2 = product(2)
    c22 = m2 - m1
    m4 = product(4)
    done(0, 1, m2 + m4)
    c11 = m3 - m4
    m0 = product(0)
    c22 = c22 + m0
    c11 = c11 + m0
    done(1, 1, c22 + product(5))
    done(0, 0, c11 + product(6))


def _head_reduce(v, op):
    v = op(v, pltpu.roll(v, 4, 0))
    return op(v, pltpu.roll(v, 2, 0))


def _dual_softmax(p):
    p3 = p.reshape(8, 8, p.shape[1])
    mx = _head_reduce(jnp.max(p3, axis=0), jnp.maximum)
    mn = _head_reduce(jnp.min(p3, axis=0), jnp.minimum)
    ep = jnp.exp2(p3 - mx[None])
    en = jnp.exp2(mn[None] - p3)
    sp = _head_reduce(jnp.sum(ep, axis=0), jnp.add)
    sn = _head_reduce(jnp.sum(en, axis=0), jnp.add)
    return ep * _recip(sp)[None], en * _recip(sn)[None]


def _zero_after(vals):
    parts = []
    for v in vals:
        b = pltpu.bitcast(v, u32)
        parts += [b[r:r + 8, c:c + 128] for r in range(0, b.shape[0], 8) for c in range(0, b.shape[1], 128)]
    while len(parts) > 1:
        parts = [parts[k] | parts[k + 1] if k + 1 < len(parts) else parts[k] for k in range(0, len(parts), 2)]
    return (parts[0] >> 16) >> 16


class _Interleaver:
    def __init__(self, at):
        self.at, self.slot, self.budget, self.credit = at, 0, 0, 0
        self.work, self.matmuls, self.filler = [], [], None

    def add(self, cost, fn, *args, delay=0):
        self.work.append((self.slot + delay, cost, fn, args))

    def fill(self, gen):
        self.finish_filler()
        self.filler = gen

    def finish_filler(self):
        for _ in self.filler or ():
            pass
        self.filler = None

    def tick(self):
        self.slot += 1
        self.credit = min(self.credit, 0) + self.budget
        vals = []
        while self.credit > 0 and self.work and self.work[0][0] < self.slot:
            _, cost, fn, args = self.work.pop(0)
            vals += fn(*args)
            self.credit -= cost
        while self.credit > 0 and self.filler:
            unit = next(self.filler, None)
            if unit is None:
                self.filler = None
            else:
                self.credit -= unit[0]
                vals += unit[1]
                if unit[0] >= 200:
                    break
        return _zero_after(vals) if vals else None

    def operand(self, op, at=None):
        parts, done = [], 0
        for r in range((self.at if at is None else at) * 8, op.shape[0], 64):
            zero = self.tick()
            if zero is not None:
                parts += [op[done:r]] if r > done else []
                parts.append(op[r:r + 8] | jnp.tile(zero, (1, op.shape[1] // 128)))
                done = r + 8
        parts += [op[done:]] if done < op.shape[0] else []
        return _unpack(parts[0] if len(parts) == 1 else jnp.concatenate(parts, axis=0))

    def issue(self):
        if self.matmuls:
            fn, args = self.matmuls.pop(0)
            fn(*args)

    def until(self, ready):
        while not ready():
            if self.matmuls:
                self.issue()
            else:
                _, _, fn, args = self.work.pop(0)
                fn(*args)

    def drain(self):
        self.until(lambda: not self.work and not self.matmuls)


def make_kernel(S, D, H, F, olag=2, delay=4, tail_delay=2, at=7, UK=128, UD=64, route_at=(3, 4, 0),
                b_early=170, b_tile0=220, b_ln=136, b_ln2=152, b_free=130, b_alone=200, b_both=240):
    T = 512
    Dh = D // H
    NT = S // T
    NG = D // 128
    NP = D // 64
    NB = NG // 2
    TH, DH = T // 2, D // 2
    FP = 256
    WR = 16
    n_dma = 64
    assert (Dh, NT, NG) == (32, 4, 8) and F % FP == 0
    awaited = {(0, 0): 2, (1, 0): 3, (3, 0): 4, (5, 0): 5}
    prepared = {(0, 0): 1, (1, 0): 2, (1, 128): 3, (3, 0): 4, (3, 128): 5, (5, 0): 6, (5, 128): 7}

    def kernel(x_hbm, wqkv_hbm, wphi_hbm, wo_hbm, wr_hbm, wg_hbm, wu_hbm, wd_hbm, out_hbm,
               x_v, wqkv_v, wphi_v, wo_v, wr_v, wg_v, wu_v, wd_v, out_v,
               xn_v, xs_v, wkv_v, wq_v, wos_v, pT_v, kv_v, z_v, kvT_v, zb_v, r_v, o_v, xb_v, wrb_v, sem):

        used = []

        def dma(src, dst):
            used.append(None)
            return pltpu.make_async_copy(src, dst, sem.at[len(used) - 1])

        def x_copy(r, n):
            return dma(x_hbm.at[pl.ds(r, n), :], x_v.at[pl.ds(r, n), :])

        def w_copy(c, n):
            return dma(wqkv_hbm.at[:, pl.ds(c, n)], wqkv_v.at[:, pl.ds(c, n)])

        def kv_copies(groups):
            return [w_copy(j * D + g * 128, 128) for g in groups for j in (1, 2)]

        first_copies = [dma(wr_hbm, wr_v), dma(wphi_hbm, wphi_v), x_copy(0, 128), x_copy(TH, 128)]
        stages = [kv_copies([0]),
                  [x_copy(128, TH - 128), x_copy(TH + 128, TH - 128)],
                  kv_copies([1]),
                  kv_copies([2, 3]),
                  [x_copy(T, T)] + kv_copies([4, 5]),
                  kv_copies([6, 7]) + [x_copy(2 * T, T)],
                  [x_copy(3 * T, T), w_copy(0, D), dma(wo_hbm, wo_v)],
                  [dma(wg_hbm, wg_v), dma(wu_hbm, wu_v), dma(wd_hbm, wd_v)]]
        for stage in [first_copies] + stages:
            for c in stage:
                c.start()

        bg = _Interleaver(at)
        emitted = set()

        def wait_stage(j):
            for c in stages[j]:
                c.wait()
            bg.credit = -bg.budget

        summed = (0, 2, 3, 5, 6)
        lane = lax.broadcasted_iota(i32, (8, 128), 1)

        def layernorm(i, pieces):
            scores = r_v[i] if pieces[0] else jnp.zeros((8, 128), f32)
            for p in pieces:
                starts = (i * T + p * 16, i * T + TH + p * 16)
                x = jnp.concatenate([x_v[r:r + 16, :] for r in starts], axis=0).astype(f32)
                m32 = jnp.sum(x, axis=1, keepdims=True) * (1.0 / D)
                yield 70, [jnp.broadcast_to(m32[24:], (8, 128))]
                m = _rb(m32)
                d = x - m
                v32 = jnp.sum(d * d, axis=1, keepdims=True) * (1.0 / D) - (m32 - m) * (m32 - m)
                inv = _recip(jnp.minimum(_rb(jnp.sqrt(_rb(_rb(v32) + LN_EPS))), 1e38))
                yield 170, [jnp.broadcast_to(inv[24:], (8, 128))]
                xn = d * inv
                a, b = xn[:16], xn[16:]
                for r, half in zip(starts, (a, b)):
                    xn_v[r // 2:r // 2 + 8, :] = _pack(half)
                score = jnp.sum(xn * jnp.tile(wrb_v[...], (4, 1)), axis=1, keepdims=True)
                for q in range(4):
                    scores = jnp.where((lane >> 1) == 4 * p + q, score[8 * q:8 * q + 8], scores)
                yield 110, [scores]
                terms = _right_terms(a[:, :DH], b[:, :DH], a[:, DH:], b[:, DH:])
                row = (i * TH + p * 16) // 2
                for n, j in enumerate(summed):
                    xs_v[n][row:row + 8, :] = _pack(terms[j])
                if p == pieces[-1]:
                    r_v[i] = scores
                yield 65, [terms[j][8:] for j in summed] if i == 2 else [terms[-1][8:, DH - 128:]]

        def token_term(t, j, l):
            def rows(start, stride):
                r = t * stride + start + l // 2
                return pl.ds(r if isinstance(r, int) else pl.multiple_of(r, 64), 64)
            if j == 1:
                return xn_v[rows(0, T // 2), :DH]
            if j == 4:
                return xn_v[rows(TH // 2, T // 2), DH:]
            return xs_v[summed.index(j)][rows(0, TH // 2), :]

        for c in first_copies:
            c.wait()
        wr = jnp.broadcast_to(wr_v[...].astype(f32).reshape(1, D), (8, D))
        wrb_v[...] = wr
        nought = jnp.max(pltpu.bitcast(wr[:, 0:128], i32) & 0xFFFF) >> 31
        for ref in (*wkv_v, *wq_v, *wos_v, o_v.at[0, 0]):
            ref[pl.ds(pl.multiple_of(nought * 8, 8), 8), 0:128] = jnp.zeros((8, 128), u32)
        for _ in layernorm(0, range(128 // 16)):
            pass

        er = lax.broadcasted_iota(i32, (128, Dh), 0)
        ec = lax.broadcasted_iota(i32, (128, Dh), 1)
        spread = jnp.where(((er & 63) >> 1) == ec, 1.0, 0.0).astype(bf16)
        pT = _dot_nt(spread, wphi_v[...])
        rr = lax.broadcasted_iota(i32, (128, 128), 0)
        cc = lax.broadcasted_iota(i32, (128, 128), 1)
        same_head = (rr >> 6) * 2 + (rr & 1) == (cc >> 5)
        for g in range(NG):
            pT_v[:, g * 128:(g + 1) * 128] = _pack(jnp.where(same_head, pT[:, g * 128:(g + 1) * 128], 0.0))

        def fold(g, j):
            w = wqkv_v[:, j * D + g * 128: j * D + (g + 1) * 128]
            return _dot_nt(bg.operand(pT_v[:, g * 128:(g + 1) * 128]), w)

        def weight_terms(tag, make, refs, row, top, bot, scale=None):
            top, bot = top.astype(f32), bot.astype(f32)
            if scale is not None:
                top, bot = top * scale, bot * scale
            terms = make(top[:, :DH], top[:, DH:], bot[:, :DH], bot[:, DH:])
            for ref, term in zip(refs, terms):
                ref[row:row + WR // 2, :] = _pack(term)
            emitted.add((tag, row))
            return [term[-8:] for term in terms] if tag == "o" else [terms[-1][-8:, DH - 128:]]

        def terms_ready(tag, row):
            return lambda: all((tag, r) in emitted for r in range(row, row + 64, WR // 2))

        def prepare_kv(g):
            wk = fold(g, 1)
            wv = _pack(wqkv_v[:, 2 * D + g * 128: 2 * D + (g + 1) * 128].T)
            for r in range(0, 32, WR // 2):
                bg.add(8 * WR, weight_terms, "kv", _left_terms, wkv_v, g * 64 + 32 + r,
                       _unpack(wv[r:r + WR // 2]), _unpack(wv[32 + r:32 + r + WR // 2]))
            for r in range(0, 64, WR):
                bg.add(8 * WR, weight_terms, "kv", _left_terms, wkv_v, g * 64 + r // 2,
                       wk[r:r + WR], wk[64 + r:64 + r + WR], LOG2E, delay=delay)

        folded = []

        def prepare_q(g):
            folded.append(fold(g, 0))
            if g % 2 == 1:
                top, bot = folded[-2:]
                for r in range(0, 128, WR):
                    bg.add(8 * WR, weight_terms, "q", _left_terms, wq_v, (g - 1) * 32 + r // 2,
                           top[r:r + WR], bot[r:r + WR], LOG2E, delay=delay)

        def prepare_o():
            for b in range(NB):
                for r in range(0, 128, WR):
                    lo, hi = 2 * b * 128 + r, (2 * b + 1) * 128 + r
                    yield 8 * WR, weight_terms("o", _right_terms, wos_v, b * 64 + r // 2,
                                               wo_v[lo:lo + WR, :], wo_v[hi:hi + WR, :])

        sel = {"y": None}

        def route():
            r = _rb(r_v[...])
            key = jnp.where(r != r, -jnp.inf, r)
            best = jnp.max(jnp.max(jnp.max(key, axis=0), axis=0, keepdims=True), axis=1, keepdims=True)
            tile, sub = (lax.broadcasted_iota(i32, r.shape, k) for k in range(2))
            row = tile * T + ((lane >> 2) & 1) * TH + (lane >> 3) * 16 + ((lane >> 1) & 1) * 8 + sub
            idx = jnp.clip(jnp.min(jnp.min(jnp.where(key == best, row, S - 1), axis=0)), 0, S - 1)
            hit = (row == idx) & ((lane & 1) == 0)
            r_sel = jnp.sum(jnp.sum(jnp.sum(jnp.where(hit, r, 0.0), axis=0), axis=0, keepdims=True),
                            axis=1, keepdims=True)
            word = jnp.broadcast_to(xn_v[pl.ds(idx // 2, 1), :], (128, D))
            bits = jnp.where(idx % 2 == 1, word & jnp.uint32(0xFFFF0000), word << 16)
            xb = pltpu.bitcast(bits, f32).T
            xb_v[0:D, :] = xb
            sel.update(idx=idx, gate=_rb(1.0 / (1.0 + jnp.exp(-r_sel))))
            return [xb[-8:]]

        def swiglu():
            h_row = pl.multiple_of(D + nought * D, 8)
            for col in range(0, F, FP):
                ag = au = None
                for k in range(0, D, 8):
                    xb = jnp.tile(xb_v[k:k + 8, :], (1, FP // 128))
                    pg = wg_v[k:k + 8, col:col + FP].astype(f32) * xb
                    pu = wu_v[k:k + 8, col:col + FP].astype(f32) * xb
                    ag = pg if ag is None else ag + pg
                    au = pu if au is None else au + pu
                    if (k + 8) % UK == 0:
                        yield 105 * UK // 64, [ag[:, 0:128], ag[:, 128:256], au[:, 0:128], au[:, 128:256]]
                gate = _rb(jnp.sum(ag, axis=0, keepdims=True))
                up = _rb(jnp.sum(au, axis=0, keepdims=True))
                h = jnp.broadcast_to(_rb(_rb(_silu(gate)) * up), (128, FP)).T
                xb_v[pl.ds(h_row, FP), :] = h
                yield 100, [h[-8:]]
                for k in range(0, FP, 8):
                    hk = xb_v[pl.ds(h_row + k, 8), :]
                    pd = wd_v[col + k:col + k + 8, :].astype(f32) * jnp.tile(hk, (1, D // 128))
                    sel["y"] = pd if sel["y"] is None else sel["y"] + pd
                    if (k + 8) % UD == 0:
                        yield 105 * UD // 32, [sel["y"][:, c:c + 128] for c in range(0, D, 128)]

        kr = lax.broadcasted_iota(i32, (64, 128), 0)
        kc = lax.broadcasted_iota(i32, (64, 128), 1)
        same = (kr >> 5) == (kc & 1)

        def project(refs, row, t, l, at=None):
            def product(j):
                m = _dot_nt(bg.operand(refs[j][row:row + 64, :], at), _unpack(token_term(t, j, l)))
                bg.issue()
                return m
            return product

        def k_feature(i, pr, pv, state):
            ep, en = _dual_softmax(pv[:64])
            phi = jnp.concatenate([ep.reshape(64, 128), en.reshape(64, 128)], axis=0)
            if not state:
                state.update(parts=[], z=phi + z_v[pr] if i > 0 else phi)
            else:
                state["z"] = state["z"] + phi
            state["parts"].append((pv[64:].astype(bf16), phi.astype(bf16)))
            if len(state["parts"]) == T // 128:
                if i < NT - 1:
                    z_v[pr] = state["z"]
                else:
                    zb_v[pr] = jnp.broadcast_to(jnp.sum(state["z"], axis=1, keepdims=True), (128, 128))
                bg.matmuls.append((k_accumulate, (i, pr, state["parts"])))
            return [phi[120:]]

        def k_accumulate(i, pr, parts):
            kv = None
            for part in [_dot_nt(vT, phi) for vT, phi in parts]:
                kv = part if kv is None else kv + part
            if i > 0:
                kv = kv + kv_v[pr]
            if i < NT - 1:
                kv_v[pr] = kv
            else:
                kvT_v[pr] = _pack(jnp.where(same, kv, 0.0))
                emitted.add(("kvT", pr))

        wait_stage(0)
        prepare_kv(0)
        bg.drain()
        for i in range(NT):
            for g in range(NG):
                if 0 < i < NT - 1 and g == 0:
                    bg.fill(layernorm(i + 1, range(TH // 16)))
                bg.until(terms_ready("kv", g * 64))
                states = ({}, {})
                for l in range(0, TH, 128):
                    bg.budget = ((b_early if g < 3 else b_tile0), b_ln, b_ln2, b_free)[i]
                    _strassen(project(wkv_v, g * 64, i, l),
                              lambda rh, ch, c: bg.add(125, k_feature, i, 2 * g + rh, c, states[rh], delay=delay))
                    if (i, g, l) == (0, 0, 0):
                        wait_stage(1)
                        for _ in layernorm(0, range(128 // 16, TH // 16)):
                            pass
                        bg.drain()
                    if i == 0 and (g, l) in awaited:
                        wait_stage(awaited[g, l])
                    if (i, g, l) == (0, 3, 0):
                        bg.fill(layernorm(1, range(TH // 16)))
                    if i == 0 and (g, l) in prepared:
                        prepare_kv(prepared[g, l])
                    if (i, g, l) == route_at:
                        bg.add(100, route, delay=delay)
                    if i >= 2 and l == 0 and g % 2 == 0:
                        prepare_q(((i - 2) * NG + g) // 2)
            bg.finish_filler()
            if i == 1:
                wait_stage(6)
            if i == 2:
                bg.fill(prepare_o())

        bg.until(lambda: "idx" in sel)
        wait_stage(7)
        bg.fill(swiglu())
        idx = sel["idx"]
        t_sel = idx // T
        tiles = [lax.rem(t_sel + 1 + i, NT) for i in range(NT - 1)] + [t_sel]

        def q_feature(i, b, a, l, pq, state):
            ep, en = _dual_softmax(pq)
            zb = zb_v[4 * b + a]
            den = jnp.sum(ep * zb[0:64].reshape(8, 8, 128) + en * zb[64:128].reshape(8, 8, 128), axis=0)
            inv = _recip(_head_reduce(den, jnp.add) + 1e-6)
            phi = jnp.concatenate([ep.reshape(64, 128), en.reshape(64, 128)], axis=0)
            state.setdefault(a, {})[l] = (phi.astype(bf16), inv)
            if len(state[a]) == T // 128:
                bg.matmuls.append((q_attend, (i, b, a, state)))
            return [phi[120:]]

        def q_attend(i, b, a, state):
            parts = [state[a][l] for l in sorted(state[a])]
            kvT = _unpack(kvT_v[4 * b + a])
            num = jnp.concatenate([_dot(kvT, phi) for phi, _ in parts], axis=1)
            inv = jnp.concatenate([inv for _, inv in parts], axis=1)
            scale = jnp.concatenate([jnp.broadcast_to(inv[h:h + 1], (32, T)) for h in range(2)], axis=0)
            state.setdefault("o", {})[a] = num * scale
            if len(state["o"]) == 4:
                lo, hi = (jnp.concatenate([state["o"][k], state["o"][k + 1]], axis=0) for k in (0, 2))
                for js in ((0, 1), (2, 3, 4), (5, 6)):
                    bg.add(70 * len(js), o_terms, i, b, js, lo, hi, delay=delay + 2)

        def o_terms(i, b, js, lo, hi):
            terms = _left_terms(lo[:, :TH], hi[:, :TH], lo[:, TH:], hi[:, TH:])
            vals = []
            for j in js:
                packed = _pack(terms[j].astype(bf16).T)
                o_v[i, j, :, b * 128:(b + 1) * 128] = packed
                emitted.add(("ot", i, b, j))
                vals.append(packed[-8:])
            return vals

        out_ready, out_copies = [], []

        def residual(i, s, r0, c0):
            t, n, last = tiles[i], s.shape[0], i == NT - 1
            gin = _unpack(xn_v[pl.ds(pl.multiple_of(t * (T // 2) + r0 // 2, n // 2), n // 2), c0:c0 + 128]).astype(f32)
            if last:
                bg.finish_filler()
                upd = _rb(_rb(jnp.sum(sel["y"][:, c0:c0 + 128], axis=0, keepdims=True)) * sel["gate"])
                hit = lax.broadcasted_iota(i32, (n, 128), 0) == idx - t_sel * T - r0
                gin = jnp.where(hit, gin + upd, gin)
            row = pl.ds(pl.multiple_of(t * T + r0, n), n)
            res = x_v[row, c0:c0 + 128].astype(f32) + s * _silu(gin)
            out_v[row, c0:c0 + 128] = res.astype(bf16)
            if last and (r0 + n) % TH == 0:
                row = pl.ds(pl.multiple_of(t * T + r0 + n - TH, TH), TH)
                out_ready.append(dma(out_v.at[row, pl.ds(c0, 128)], out_hbm.at[row, pl.ds(c0, 128)]))
            elif not last and r0 + n == TH and c0 == DH - 128:
                row = pl.ds(pl.multiple_of(t * T, T), T)
                out_ready.append(dma(out_v.at[row, :], out_hbm.at[row, :]))
            return [res[-8:]]

        def send_ready():
            while out_ready:
                out_copies.append(out_ready.pop(0))
                out_copies[-1].start()

        def out_chunk(i, n):
            bg.until(lambda: all(("ot", i, b, j) in emitted for b in range(NB) for j in range(7)))

            def product(j):
                m = _dot(bg.operand(o_v[i, j]), _unpack(wos_v[j][:, n * 128:(n + 1) * 128]))
                send_ready()
                bg.issue()
                return m

            def done(rh, ch, c):
                for r in range(0, TH, 128):
                    bg.add(144, residual, i, c[r:r + 128], rh * TH + r, ch * DH + n * 128,
                           delay=tail_delay if (i, n) == (NT - 1, NB - 1) else delay)

            _strassen(product, done)

        chunks = [(i, n) for i in range(NT) for n in range(NB)]
        for i in range(NT):
            for b in range(NB):
                state = {}
                with_out = i * NB + b >= NB + olag
                bg.until(terms_ready("q", b * 64))
                bg.until(lambda: all(("kvT", pr) in emitted for pr in range(4 * b, 4 * b + 4)))
                bg.budget = b_both if with_out else b_alone
                for l in range(0, TH, 128):
                    def done(rh, ch, c):
                        for a in range(2):
                            bg.add(150, q_feature, i, b, 2 * rh + a, ch * TH + l, c[a * 64:(a + 1) * 64], state,
                                   delay=delay)

                    _strassen(project(wq_v, b * 64, tiles[i], l, 4), done)
                if with_out:
                    out_chunk(*chunks.pop(0))
        while chunks:
            out_chunk(*chunks.pop(0))
        bg.drain()
        send_ready()
        assert len(used) <= n_dma
        for c in out_copies:
            c.wait()

    scratch = [
        pltpu.VMEM((S, D), bf16),
        pltpu.VMEM((D, 3 * D), bf16),
        pltpu.VMEM((D, Dh), bf16),
        pltpu.VMEM((D, D), bf16),
        pltpu.VMEM((D,), bf16),
        pltpu.VMEM((D, F), bf16),
        pltpu.VMEM((D, F), bf16),
        pltpu.VMEM((F, D), bf16),
        pltpu.VMEM((S, D), bf16),
        pltpu.VMEM((S // 2, D), u32),
        [pltpu.VMEM((S // 4, DH), u32)] * 5,
        [pltpu.VMEM((D // 2, DH), u32)] * 7,
        [pltpu.VMEM((D // 4, DH), u32)] * 7,
        [pltpu.VMEM((D // 4, DH), u32)] * 7,
        pltpu.VMEM((64, D), u32),
        pltpu.VMEM((NP, 64, 128), f32),
        pltpu.VMEM((NP, 128, 128), f32),
        pltpu.VMEM((NP, 32, 128), u32),
        pltpu.VMEM((NP, 128, 128), f32),
        pltpu.VMEM((NT, 8, 128), f32),
        pltpu.VMEM((NT, 7, TH // 2, DH), u32),
        pltpu.VMEM((D + FP, 128), f32),
        pltpu.VMEM((8, D), f32),
        pltpu.SemaphoreType.DMA((n_dma,)),
    ]
    return kernel, scratch


@jax.jit
def pallas_recurrent_scan__linear_kernel_hedgehog__moe_arch_mod__prompt_kernel(
    A_x: jax.Array,
    A_wqkv: jax.Array,
    A_w_phi: jax.Array,
    A_wo: jax.Array,
    B_x: jax.Array,
    B_w_r: jax.Array,
    B_w_gate: jax.Array,
    B_w_up: jax.Array,
    B_w_down: jax.Array,
):
    del B_x
    B, S, D = A_x.shape
    H, Dh, _ = A_w_phi.shape
    F = B_w_gate.shape[1]
    assert B == 1
    kernel, scratch = make_kernel(S=S, D=D, H=H, F=F)
    out = pl.pallas_call(
        kernel,
        out_shape=jax.ShapeDtypeStruct((S, D), A_x.dtype),
        in_specs=[pl.BlockSpec(memory_space=pl.ANY)] * 8,
        out_specs=pl.BlockSpec(memory_space=pl.ANY),
        scratch_shapes=scratch,
        compiler_params=pltpu.CompilerParams(
            vmem_limit_bytes=110 * 1024 * 1024),
        name="hedgehog_mod",
    )(A_x.reshape(S, D), A_wqkv, A_w_phi.reshape(H * Dh, Dh), A_wo, B_w_r, B_w_gate, B_w_up, B_w_down)
    return out.reshape(B, S, D)
```

```python
import jax
import jax.numpy as jnp
import numpy as np
from jax import lax
import jax.experimental.pallas as pl
import jax.experimental.pallas.tpu as pltpu

bf16, f32, u32, i32 = jnp.bfloat16, jnp.float32, jnp.uint32, jnp.int32
LOG2E = 1.4426950408889634
LN_EPS = float(np.asarray(1e-5, dtype=bf16))


def _dot(a, b):
    return jnp.dot(a, b, preferred_element_type=f32)


def _dot_nt(a, b):
    return lax.dot_general(a, b, (((1,), (1,)), ((), ())), preferred_element_type=f32)


def _pack(x):
    return pltpu.bitcast(x.astype(bf16), u32)


def _unpack(x):
    return pltpu.bitcast(x, bf16)


def _rb(x):
    return x.astype(bf16).astype(f32)


def _recip(x):
    return pltpu.reciprocal(x, approx=False, full_range=False)


def _silu(x):
    h = 0.5 * x
    return h * jnp.tanh(h) + h


def _left_terms(a11, a12, a21, a22):
    return [a11 + a22, a21 + a22, a11, a22, a11 + a12, a21 - a11, a12 - a22]


def _right_terms(b11, b12, b21, b22):
    return [b11 + b22, b11, b12 - b22, b21 - b11, b22, b11 + b12, b21 + b22]


def _strassen(product, done):
    m1 = product(1)
    m3 = product(3)
    done(1, 0, m1 + m3)
    m2 = product(2)
    c22 = m2 - m1
    m4 = product(4)
    done(0, 1, m2 + m4)
    c11 = m3 - m4
    m0 = product(0)
    c22 = c22 + m0
    c11 = c11 + m0
    done(1, 1, c22 + product(5))
    done(0, 0, c11 + product(6))


def _head_reduce(v, op):
    v = op(v, pltpu.roll(v, 4, 0))
    return op(v, pltpu.roll(v, 2, 0))


def _dual_softmax(p):
    p3 = p.reshape(8, 8, p.shape[1])
    mx = _head_reduce(jnp.max(p3, axis=0), jnp.maximum)
    mn = _head_reduce(jnp.min(p3, axis=0), jnp.minimum)
    ep = jnp.exp2(p3 - mx[None])
    en = jnp.exp2(mn[None] - p3)
    sp = _head_reduce(jnp.sum(ep, axis=0), jnp.add)
    sn = _head_reduce(jnp.sum(en, axis=0), jnp.add)
    return ep * _recip(sp)[None], en * _recip(sn)[None]


def _zero_after(vals):
    parts = []
    for v in vals:
        b = pltpu.bitcast(v, u32)
        parts += [b[r:r + 8, c:c + 128] for r in range(0, b.shape[0], 8) for c in range(0, b.shape[1], 128)]
    while len(parts) > 1:
        parts = [parts[k] | parts[k + 1] if k + 1 < len(parts) else parts[k] for k in range(0, len(parts), 2)]
    return (parts[0] >> 16) >> 16


class _Interleaver:
    def __init__(self, at):
        self.at, self.slot, self.budget, self.credit = at, 0, 0, 0
        self.work, self.matmuls, self.filler = [], [], None

    def add(self, cost, fn, *args, delay=0):
        self.work.append((self.slot + delay, cost, fn, args))

    def fill(self, gen):
        self.finish_filler()
        self.filler = gen

    def finish_filler(self):
        for _ in self.filler or ():
            pass
        self.filler = None

    def tick(self):
        self.slot += 1
        self.credit = min(self.credit, 0) + self.budget
        vals = []
        while self.credit > 0 and self.work and self.work[0][0] < self.slot:
            _, cost, fn, args = self.work.pop(0)
            vals += fn(*args)
            self.credit -= cost
        while self.credit > 0 and self.filler:
            unit = next(self.filler, None)
            if unit is None:
                self.filler = None
            else:
                self.credit -= unit[0]
                vals += unit[1]
                if unit[0] >= 200:
                    break
        return _zero_after(vals) if vals else None

    def operand(self, op, at=None):
        parts, done = [], 0
        for r in range((self.at if at is None else at) * 8, op.shape[0], 64):
            zero = self.tick()
            if zero is not None:
                parts += [op[done:r]] if r > done else []
                parts.append(op[r:r + 8] | jnp.tile(zero, (1, op.shape[1] // 128)))
                done = r + 8
        parts += [op[done:]] if done < op.shape[0] else []
        return _unpack(parts[0] if len(parts) == 1 else jnp.concatenate(parts, axis=0))

    def issue(self):
        if self.matmuls:
            fn, args = self.matmuls.pop(0)
            fn(*args)

    def until(self, ready):
        while not ready():
            if self.matmuls:
                self.issue()
            else:
                _, _, fn, args = self.work.pop(0)
                fn(*args)

    def drain(self):
        self.until(lambda: not self.work and not self.matmuls)


def make_kernel(S, D, H, F, olag=2, delay=4, tail_delay=2, at=7, UK=128, UD=64, route_at=(3, 4, 0),
                b_early=170, b_tile0=220, b_ln=136, b_ln2=152, b_free=130, b_alone=200, b_both=240):
    T = 512
    Dh = D // H
    NT = S // T
    NG = D // 128
    NP = D // 64
    NB = NG // 2
    TH, DH = T // 2, D // 2
    FP = 256
    WR = 16
    assert (Dh, NT, NG) == (32, 4, 8) and F % FP == 0
    awaited = {(0, 0): 2, (1, 0): 3, (3, 0): 4, (5, 0): 5}
    prepared = {(0, 0): 1, (1, 0): 2, (1, 128): 3, (3, 0): 4, (3, 128): 5, (5, 0): 6, (5, 128): 7}

    def kernel(x_hbm, wqkv_hbm, wphi_hbm, wo_hbm, wr_hbm, wg_hbm, wu_hbm, wd_hbm, out_hbm,
               x_v, wqkv_v, wphi_v, wo_v, wr_v, wg_v, wu_v, wd_v, out_v,
               xn_v, xs_v, wkv_v, wq_v, wos_v, pT_v, kv_v, z_v, kvT_v, zb_v, r_v, o_v, xb_v, wrb_v, sem):

        def x_rows(r, n):
            return x_hbm.at[pl.ds(r, n), :], x_v.at[pl.ds(r, n), :]

        def w_cols(c, n):
            return wqkv_hbm.at[:, pl.ds(c, n)], wqkv_v.at[:, pl.ds(c, n)]

        def kv_cols(groups):
            return [w_cols(j * D + g * 128, 128) for g in groups for j in (1, 2)]

        stages = [kv_cols([0]),
                  [x_rows(128, TH - 128), x_rows(TH + 128, TH - 128)],
                  kv_cols([1]),
                  kv_cols([2, 3]),
                  [x_rows(T, T)] + kv_cols([4, 5]),
                  kv_cols([6, 7]) + [x_rows(2 * T, T)],
                  [x_rows(3 * T, T), w_cols(0, D), (wo_hbm, wo_v)],
                  [(wg_hbm, wg_v), (wu_hbm, wu_v), (wd_hbm, wd_v)],
                  [(wr_hbm, wr_v), (wphi_hbm, wphi_v), x_rows(0, 128), x_rows(TH, 128)]]
        stages = [[pltpu.make_async_copy(src, dst, sem.at[j]) for src, dst in stage] for j, stage in enumerate(stages)]
        for stage in stages[-1:] + stages[:-1]:
            for c in stage:
                c.start()

        def dma(src, dst):
            return pltpu.make_async_copy(src, dst, sem.at[len(stages)])

        bg = _Interleaver(at)
        emitted = set()

        def wait_stage(j):
            for c in stages[j]:
                c.wait()
            bg.credit = -bg.budget

        summed = (0, 2, 3, 5, 6)
        lane = lax.broadcasted_iota(i32, (8, 128), 1)

        def layernorm(i, pieces):
            scores = r_v[i] if pieces[0] else jnp.zeros((8, 128), f32)
            for p in pieces:
                starts = (i * T + p * 16, i * T + TH + p * 16)
                x = jnp.concatenate([x_v[r:r + 16, :] for r in starts], axis=0).astype(f32)
                m32 = jnp.sum(x, axis=1, keepdims=True) * (1.0 / D)
                yield 70, [jnp.broadcast_to(m32[24:], (8, 128))]
                m = _rb(m32)
                d = x - m
                v32 = jnp.sum(d * d, axis=1, keepdims=True) * (1.0 / D) - (m32 - m) * (m32 - m)
                inv = _recip(jnp.minimum(_rb(jnp.sqrt(_rb(_rb(v32) + LN_EPS))), 1e38))
                yield 170, [jnp.broadcast_to(inv[24:], (8, 128))]
                xn = d * inv
                a, b = xn[:16], xn[16:]
                for r, half in zip(starts, (a, b)):
                    xn_v[r // 2:r // 2 + 8, :] = _pack(half)
                score = jnp.sum(xn * jnp.tile(wrb_v[...], (4, 1)), axis=1, keepdims=True)
                for q in range(4):
                    scores = jnp.where((lane >> 1) == 4 * p + q, score[8 * q:8 * q + 8], scores)
                yield 110, [scores]
                terms = _right_terms(a[:, :DH], b[:, :DH], a[:, DH:], b[:, DH:])
                row = (i * TH + p * 16) // 2
                for n, j in enumerate(summed):
                    xs_v[n][row:row + 8, :] = _pack(terms[j])
                if p == pieces[-1]:
                    r_v[i] = scores
                yield 65, [terms[j][8:] for j in summed] if i == 2 else [terms[-1][8:, DH - 128:]]

        def token_term(t, j, l):
            def rows(start, stride):
                r = t * stride + start + l // 2
                return pl.ds(r if isinstance(r, int) else pl.multiple_of(r, 64), 64)
            if j == 1:
                return xn_v[rows(0, T // 2), :DH]
            if j == 4:
                return xn_v[rows(TH // 2, T // 2), DH:]
            return xs_v[summed.index(j)][rows(0, TH // 2), :]

        for c in stages[-1]:
            c.wait()
        wr = jnp.broadcast_to(wr_v[...].astype(f32).reshape(1, D), (8, D))
        wrb_v[...] = wr
        nought = jnp.max(pltpu.bitcast(wr[:, 0:128], i32) & 0xFFFF) >> 31
        for ref in (*wkv_v, *wq_v, *wos_v, o_v.at[0, 0]):
            ref[pl.ds(pl.multiple_of(nought * 8, 8), 8), 0:128] = jnp.zeros((8, 128), u32)
        for _ in layernorm(0, range(128 // 16)):
            pass

        er = lax.broadcasted_iota(i32, (128, Dh), 0)
        ec = lax.broadcasted_iota(i32, (128, Dh), 1)
        spread = jnp.where(((er & 63) >> 1) == ec, 1.0, 0.0).astype(bf16)
        pT = _dot_nt(spread, wphi_v[...])
        rr = lax.broadcasted_iota(i32, (128, 128), 0)
        cc = lax.broadcasted_iota(i32, (128, 128), 1)
        same_head = (rr >> 6) * 2 + (rr & 1) == (cc >> 5)
        for g in range(NG):
            pT_v[:, g * 128:(g + 1) * 128] = _pack(jnp.where(same_head, pT[:, g * 128:(g + 1) * 128], 0.0))

        def fold(g, j):
            w = wqkv_v[:, j * D + g * 128: j * D + (g + 1) * 128]
            return _dot_nt(bg.operand(pT_v[:, g * 128:(g + 1) * 128]), w)

        def weight_terms(tag, make, refs, row, top, bot, scale=None):
            top, bot = top.astype(f32), bot.astype(f32)
            if scale is not None:
                top, bot = top * scale, bot * scale
            terms = make(top[:, :DH], top[:, DH:], bot[:, :DH], bot[:, DH:])
            for ref, term in zip(refs, terms):
                ref[row:row + WR // 2, :] = _pack(term)
            emitted.add((tag, row))
            return [term[-8:] for term in terms] if tag == "o" else [terms[-1][-8:, DH - 128:]]

        def terms_ready(tag, row):
            return lambda: all((tag, r) in emitted for r in range(row, row + 64, WR // 2))

        def prepare_kv(g):
            wk = fold(g, 1)
            wv = _pack(wqkv_v[:, 2 * D + g * 128: 2 * D + (g + 1) * 128].T)
            for r in range(0, 32, WR // 2):
                bg.add(8 * WR, weight_terms, "kv", _left_terms, wkv_v, g * 64 + 32 + r,
                       _unpack(wv[r:r + WR // 2]), _unpack(wv[32 + r:32 + r + WR // 2]))
            for r in range(0, 64, WR):
                bg.add(8 * WR, weight_terms, "kv", _left_terms, wkv_v, g * 64 + r // 2,
                       wk[r:r + WR], wk[64 + r:64 + r + WR], LOG2E, delay=delay)

        folded = []

        def prepare_q(g):
            folded.append(fold(g, 0))
            if g % 2 == 1:
                top, bot = folded[-2:]
                for r in range(0, 128, WR):
                    bg.add(8 * WR, weight_terms, "q", _left_terms, wq_v, (g - 1) * 32 + r // 2,
                           top[r:r + WR], bot[r:r + WR], LOG2E, delay=delay)

        def prepare_o():
            for b in range(NB):
                for r in range(0, 128, WR):
                    lo, hi = 2 * b * 128 + r, (2 * b + 1) * 128 + r
                    yield 8 * WR, weight_terms("o", _right_terms, wos_v, b * 64 + r // 2,
                                               wo_v[lo:lo + WR, :], wo_v[hi:hi + WR, :])

        sel = {"y": None}

        def route():
            r = _rb(r_v[...])
            key = jnp.where(r != r, -jnp.inf, r)
            best = jnp.max(jnp.max(jnp.max(key, axis=0), axis=0, keepdims=True), axis=1, keepdims=True)
            tile, sub = (lax.broadcasted_iota(i32, r.shape, k) for k in range(2))
            row = tile * T + ((lane >> 2) & 1) * TH + (lane >> 3) * 16 + ((lane >> 1) & 1) * 8 + sub
            idx = jnp.clip(jnp.min(jnp.min(jnp.where(key == best, row, S - 1), axis=0)), 0, S - 1)
            hit = (row == idx) & ((lane & 1) == 0)
            r_sel = jnp.sum(jnp.sum(jnp.sum(jnp.where(hit, r, 0.0), axis=0), axis=0, keepdims=True),
                            axis=1, keepdims=True)
            word = jnp.broadcast_to(xn_v[pl.ds(idx // 2, 1), :], (128, D))
            bits = jnp.where(idx % 2 == 1, word & jnp.uint32(0xFFFF0000), word << 16)
            xb = pltpu.bitcast(bits, f32).T
            xb_v[0:D, :] = xb
            sel.update(idx=idx, gate=_rb(1.0 / (1.0 + jnp.exp(-r_sel))))
            return [xb[-8:]]

        def swiglu():
            h_row = pl.multiple_of(D + nought * D, 8)
            for col in range(0, F, FP):
                ag = au = None
                for k in range(0, D, 8):
                    xb = jnp.tile(xb_v[k:k + 8, :], (1, FP // 128))
                    pg = wg_v[k:k + 8, col:col + FP].astype(f32) * xb
                    pu = wu_v[k:k + 8, col:col + FP].astype(f32) * xb
                    ag = pg if ag is None else ag + pg
                    au = pu if au is None else au + pu
                    if (k + 8) % UK == 0:
                        yield 105 * UK // 64, [ag[:, 0:128], ag[:, 128:256], au[:, 0:128], au[:, 128:256]]
                gate = _rb(jnp.sum(ag, axis=0, keepdims=True))
                up = _rb(jnp.sum(au, axis=0, keepdims=True))
                h = jnp.broadcast_to(_rb(_rb(_silu(gate)) * up), (128, FP)).T
                xb_v[pl.ds(h_row, FP), :] = h
                yield 100, [h[-8:]]
                for k in range(0, FP, 8):
                    hk = xb_v[pl.ds(h_row + k, 8), :]
                    pd = wd_v[col + k:col + k + 8, :].astype(f32) * jnp.tile(hk, (1, D // 128))
                    sel["y"] = pd if sel["y"] is None else sel["y"] + pd
                    if (k + 8) % UD == 0:
                        yield 105 * UD // 32, [sel["y"][:, c:c + 128] for c in range(0, D, 128)]

        kr = lax.broadcasted_iota(i32, (64, 128), 0)
        kc = lax.broadcasted_iota(i32, (64, 128), 1)
        same = (kr >> 5) == (kc & 1)

        def project(refs, row, t, l, at=None):
            def product(j):
                m = _dot_nt(bg.operand(refs[j][row:row + 64, :], at), _unpack(token_term(t, j, l)))
                bg.issue()
                return m
            return product

        def k_feature(i, pr, pv, state):
            ep, en = _dual_softmax(pv[:64])
            phi = jnp.concatenate([ep.reshape(64, 128), en.reshape(64, 128)], axis=0)
            if not state:
                state.update(parts=[], z=phi + z_v[pr] if i > 0 else phi)
            else:
                state["z"] = state["z"] + phi
            state["parts"].append((pv[64:].astype(bf16), phi.astype(bf16)))
            if len(state["parts"]) == T // 128:
                if i < NT - 1:
                    z_v[pr] = state["z"]
                else:
                    zb_v[pr] = jnp.broadcast_to(jnp.sum(state["z"], axis=1, keepdims=True), (128, 128))
                bg.matmuls.append((k_accumulate, (i, pr, state["parts"])))
            return [phi[120:]]

        def k_accumulate(i, pr, parts):
            kv = None
            for part in [_dot_nt(vT, phi) for vT, phi in parts]:
                kv = part if kv is None else kv + part
            if i > 0:
                kv = kv + kv_v[pr]
            if i < NT - 1:
                kv_v[pr] = kv
            else:
                kvT_v[pr] = _pack(jnp.where(same, kv, 0.0))
                emitted.add(("kvT", pr))

        wait_stage(0)
        prepare_kv(0)
        bg.drain()
        for i in range(NT):
            for g in range(NG):
                if 0 < i < NT - 1 and g == 0:
                    bg.fill(layernorm(i + 1, range(TH // 16)))
                bg.until(terms_ready("kv", g * 64))
                states = ({}, {})
                for l in range(0, TH, 128):
                    bg.budget = ((b_early if g < 3 else b_tile0), b_ln, b_ln2, b_free)[i]
                    _strassen(project(wkv_v, g * 64, i, l),
                              lambda rh, ch, c: bg.add(125, k_feature, i, 2 * g + rh, c, states[rh], delay=delay))
                    if (i, g, l) == (0, 0, 0):
                        wait_stage(1)
                        for _ in layernorm(0, range(128 // 16, TH // 16)):
                            pass
                        bg.drain()
                    if i == 0 and (g, l) in awaited:
                        wait_stage(awaited[g, l])
                    if (i, g, l) == (0, 3, 0):
                        bg.fill(layernorm(1, range(TH // 16)))
                    if i == 0 and (g, l) in prepared:
                        prepare_kv(prepared[g, l])
                    if (i, g, l) == route_at:
                        bg.add(100, route, delay=delay)
                    if i >= 2 and l == 0 and g % 2 == 0:
                        prepare_q(((i - 2) * NG + g) // 2)
            bg.finish_filler()
            if i == 1:
                wait_stage(6)
            if i == 2:
                bg.fill(prepare_o())

        bg.until(lambda: "idx" in sel)
        wait_stage(7)
        bg.fill(swiglu())
        idx = sel["idx"]
        t_sel = idx // T
        tiles = [lax.rem(t_sel + 1 + i, NT) for i in range(NT - 1)] + [t_sel]

        def q_feature(i, b, a, l, pq, state):
            ep, en = _dual_softmax(pq)
            zb = zb_v[4 * b + a]
            den = jnp.sum(ep * zb[0:64].reshape(8, 8, 128) + en * zb[64:128].reshape(8, 8, 128), axis=0)
            inv = _recip(_head_reduce(den, jnp.add) + 1e-6)
            phi = jnp.concatenate([ep.reshape(64, 128), en.reshape(64, 128)], axis=0)
            state.setdefault(a, {})[l] = (phi.astype(bf16), inv)
            if len(state[a]) == T // 128:
                bg.matmuls.append((q_attend, (i, b, a, state)))
            return [phi[120:]]

        def q_attend(i, b, a, state):
            parts = [state[a][l] for l in sorted(state[a])]
            kvT = _unpack(kvT_v[4 * b + a])
            num = jnp.concatenate([_dot(kvT, phi) for phi, _ in parts], axis=1)
            inv = jnp.concatenate([inv for _, inv in parts], axis=1)
            scale = jnp.concatenate([jnp.broadcast_to(inv[h:h + 1], (32, T)) for h in range(2)], axis=0)
            state.setdefault("o", {})[a] = num * scale
            if len(state["o"]) == 4:
                lo, hi = (jnp.concatenate([state["o"][k], state["o"][k + 1]], axis=0) for k in (0, 2))
                for js in ((0, 1), (2, 3, 4), (5, 6)):
                    bg.add(70 * len(js), o_terms, i, b, js, lo, hi, delay=delay + 2)

        def o_terms(i, b, js, lo, hi):
            terms = _left_terms(lo[:, :TH], hi[:, :TH], lo[:, TH:], hi[:, TH:])
            vals = []
            for j in js:
                packed = _pack(terms[j].astype(bf16).T)
                o_v[i, j, :, b * 128:(b + 1) * 128] = packed
                emitted.add(("ot", i, b, j))
                vals.append(packed[-8:])
            return vals

        out_ready = []

        def residual(i, s, r0, c0, rows):
            t, n, last = tiles[i], s.shape[0], i == NT - 1
            gin = _unpack(xn_v[pl.ds(pl.multiple_of(t * (T // 2) + r0 // 2, n // 2), n // 2), c0:c0 + 128]).astype(f32)
            if last:
                bg.finish_filler()
                upd = _rb(_rb(jnp.sum(sel["y"][:, c0:c0 + 128], axis=0, keepdims=True)) * sel["gate"])
                hit = lax.broadcasted_iota(i32, (n, 128), 0) == idx - t_sel * T - r0
                gin = jnp.where(hit, gin + upd, gin)
            row = pl.ds(pl.multiple_of(t * T + r0, n), n)
            res = x_v[row, c0:c0 + 128].astype(f32) + s * _silu(gin)
            out_v[row, c0:c0 + 128] = res.astype(bf16)
            if last and (r0 + n) % rows == 0:
                row = pl.ds(pl.multiple_of(t * T + r0 + n - rows, rows), rows)
                out_ready.append(dma(out_v.at[row, pl.ds(c0, 128)], out_hbm.at[row, pl.ds(c0, 128)]))
            elif not last and r0 + n == TH and c0 == DH - 128:
                row = pl.ds(pl.multiple_of(t * T, T), T)
                out_ready.append(dma(out_v.at[row, :], out_hbm.at[row, :]))
            return [res[-8:]]

        def send_ready():
            while out_ready:
                out_ready.pop(0).start()

        def out_chunk(i, n):
            bg.until(lambda: all(("ot", i, b, j) in emitted for b in range(NB) for j in range(7)))

            final = (i, n) == (NT - 1, NB - 1)
            rows = TH // 2 if final else TH
            for r0 in range(0, TH, rows):
                def product(j):
                    m = _dot(bg.operand(o_v[i, j, r0 // 2:(r0 + rows) // 2, :]),
                             _unpack(wos_v[j][:, n * 128:(n + 1) * 128]))
                    send_ready()
                    bg.issue()
                    return m

                def done(rh, ch, c):
                    for r in range(0, rows, 128):
                        bg.add(144, residual, i, c[r:r + 128], rh * TH + r0 + r, ch * DH + n * 128, rows,
                               delay=tail_delay if final else delay)

                _strassen(product, done)

        chunks = [(i, n) for i in range(NT) for n in range(NB)]
        for i in range(NT):
            for b in range(NB):
                state = {}
                with_out = i * NB + b >= NB + olag
                bg.until(terms_ready("q", b * 64))
                bg.until(lambda: all(("kvT", pr) in emitted for pr in range(4 * b, 4 * b + 4)))
                bg.budget = b_both if with_out else b_alone
                for l in range(0, TH, 128):
                    def done(rh, ch, c):
                        for a in range(2):
                            bg.add(150, q_feature, i, b, 2 * rh + a, ch * TH + l, c[a * 64:(a + 1) * 64], state,
                                   delay=delay)

                    _strassen(project(wq_v, b * 64, tiles[i], l, 4), done)
                if with_out:
                    out_chunk(*chunks.pop(0))
        while chunks:
            out_chunk(*chunks.pop(0))
        bg.drain()
        send_ready()
        dma(out_v, out_hbm).wait()

    scratch = [
        pltpu.VMEM((S, D), bf16),
        pltpu.VMEM((D, 3 * D), bf16),
        pltpu.VMEM((D, Dh), bf16),
        pltpu.VMEM((D, D), bf16),
        pltpu.VMEM((D,), bf16),
        pltpu.VMEM((D, F), bf16),
        pltpu.VMEM((D, F), bf16),
        pltpu.VMEM((F, D), bf16),
        pltpu.VMEM((S, D), bf16),
        pltpu.VMEM((S // 2, D), u32),
        [pltpu.VMEM((S // 4, DH), u32)] * 5,
        [pltpu.VMEM((D // 2, DH), u32)] * 7,
        [pltpu.VMEM((D // 4, DH), u32)] * 7,
        [pltpu.VMEM((D // 4, DH), u32)] * 7,
        pltpu.VMEM((64, D), u32),
        pltpu.VMEM((NP, 64, 128), f32),
        pltpu.VMEM((NP, 128, 128), f32),
        pltpu.VMEM((NP, 32, 128), u32),
        pltpu.VMEM((NP, 128, 128), f32),
        pltpu.VMEM((NT, 8, 128), f32),
        pltpu.VMEM((NT, 7, TH // 2, DH), u32),
        pltpu.VMEM((D + FP, 128), f32),
        pltpu.VMEM((8, D), f32),
        pltpu.SemaphoreType.DMA((10,)),
    ]
    return kernel, scratch


@jax.jit
def pallas_recurrent_scan__linear_kernel_hedgehog__moe_arch_mod__prompt_kernel(
    A_x: jax.Array,
    A_wqkv: jax.Array,
    A_w_phi: jax.Array,
    A_wo: jax.Array,
    B_x: jax.Array,
    B_w_r: jax.Array,
    B_w_gate: jax.Array,
    B_w_up: jax.Array,
    B_w_down: jax.Array,
):
    del B_x
    B, S, D = A_x.shape
    H, Dh, _ = A_w_phi.shape
    F = B_w_gate.shape[1]
    assert B == 1
    kernel, scratch = make_kernel(S=S, D=D, H=H, F=F)
    out = pl.pallas_call(
        kernel,
        out_shape=jax.ShapeDtypeStruct((S, D), A_x.dtype),
        in_specs=[pl.BlockSpec(memory_space=pl.ANY)] * 8,
        out_specs=pl.BlockSpec(memory_space=pl.ANY),
        scratch_shapes=scratch,
        compiler_params=pltpu.CompilerParams(
            vmem_limit_bytes=110 * 1024 * 1024),
        name="hedgehog_mod",
    )(A_x.reshape(S, D), A_wqkv, A_w_phi.reshape(H * Dh, Dh), A_wo, B_w_r, B_w_gate, B_w_up, B_w_down)
    return out.reshape(B, S, D)
```
